```python
import jax
import jax.numpy as jnp

def _softmax(x, axis=-1):
    return jax.nn.softmax(x, axis=axis)
def _gelu(x):
    return jax.nn.gelu(x, approximate=True)
def _silu(x):
    return jax.nn.silu(x)
def _sigmoid(x):
    return jax.nn.sigmoid(x)
def _layernorm(x, axis=-1, eps=1e-5):
    m = jnp.mean(x, axis=axis, keepdims=True)
    v = jnp.var(x, axis=axis, keepdims=True)
    return (x - m) / jnp.sqrt(v + eps)
def _scatter_add(tgt, idx, src, axis=0):
    return tgt.at[idx].add(src)
def _segment_sum(src, seg, n):
    return jax.ops.segment_sum(src, seg, n)
class _Rng:
    def __init__(self, key):
        self._k = key
    def _next(self):
        self._k, sub = jax.random.split(self._k)
        return sub
    def normal(self, shape):
        return jax.random.normal(self._next(), shape, dtype=jnp.bfloat16)
    def randint(self, lo, hi, shape):
        return jax.random.randint(self._next(), shape, lo, hi, dtype=jnp.int32)
    def uniform(self, shape, lo=0.0, hi=1.0):
        return jax.random.uniform(self._next(), shape, jnp.bfloat16, lo, hi)
    def permutation(self, n):
        return jax.random.permutation(self._next(), n)


kernel_name = 'concat_heads__linear_attn_block__ssm_conv_h3__prompt'

def setup_inputs():
    _rng = _Rng(jax.random.key(int.from_bytes(__import__("os").urandom(4), "little")))
    _w = (lambda a: (lambda t: t.astype(jnp.bfloat16) if jnp.issubdtype(t.dtype, jnp.floating) else t)(jnp.asarray(a)))
    def _A_setup():
        B, S, D = 1, 2048, 1024
        return {
            "x": _w((lambda *s: _rng.normal(s) * 0.05)(B, S, D)),
            "wqkv": _w((lambda *s: _rng.normal(s) * 0.05)(D, 3 * D)),
            "wo": _w((lambda *s: _rng.normal(s) * 0.05)(D, D)),
        }
    _A_in = _A_setup()

    def _B_setup():
        B, S, D = 1, 2048, 1024
        ks = 4
        return {
            "q": _w((lambda *s: _rng.normal(s) * 0.05)(B, S, D)),
            "k": _w((lambda *s: _rng.normal(s) * 0.05)(B, S, D)),
            "v": _w((lambda *s: _rng.normal(s) * 0.05)(B, S, D)),
            "shift_k": _w((lambda *s: _rng.normal(s) * 0.05)(D, ks) * 0.5),
            "ssm_k": _w((lambda *s: _rng.normal(s) * 0.05)(D, S) * (1.0 / S ** 0.5)),
            "ssm_D": _w((lambda *s: _rng.normal(s) * 0.05)(D)),
        }
    _B_in = _B_setup()

    return {
        "A_x": _A_in["x"],
        "A_wqkv": _A_in["wqkv"],
        "A_wo": _A_in["wo"],
        "B_q": _B_in["q"],
        "B_k": _B_in["k"],
        "B_v": _B_in["v"],
        "B_shift_k": _B_in["shift_k"],
        "B_ssm_k": _B_in["ssm_k"],
        "B_ssm_D": _B_in["ssm_D"],
    }

def reference(A_x, A_wqkv, A_wo, B_q, B_k, B_v, B_shift_k, B_ssm_k, B_ssm_D):
    def _A_ref(x, wqkv, wo):
        B, S, D = x.shape
        H = 32; Dh = D // H
        qkv = (lambda x, *d: x.transpose(*d))((x @ wqkv).reshape(B, S, 3, H, Dh), 2, 0, 3, 1, 4)
        q, k, v = qkv[0], qkv[1], qkv[2]
        phi = lambda t: jnp.where(t > 0, t + 1, jnp.exp(t)) + 1e-6
        pq, pk = phi(q), phi(k)
        kv = jnp.einsum("bhsd,bhse->bhde", pk, v)
        z = jnp.einsum("bhsd->bhd", pk)
        num = jnp.einsum("bhqd,bhde->bhqe", pq, kv)
        den = jnp.einsum("bhqd,bhd->bhq", pq, z)[..., None] + 1e-6
        o = num / den
        return (lambda x, *d: x.transpose(*d))(o, 0, 2, 1, 3).reshape(B, S, D) @ wo

    def _B_ref(q, k, v, shift_k, ssm_k, ssm_D):
        B, S, D = q.shape
        ks = shift_k.shape[-1]
        k_pad = jnp.pad(k, ((0, 0), (ks - 1, 0), (0, 0)))
        k_shift = jnp.zeros_like(k)
        for t in range(ks):
            k_shift = k_shift + k_pad[:, t:t + S, :] * shift_k[:, ks - 1 - t][None, None, :]
        kv = k_shift * v
        L = 2 * S
        kv_pad = jnp.pad(kv, ((0, 0), (0, S), (0, 0)))
        kf_pad = jnp.pad(ssm_k, ((0, 0), (0, S)))
        kv_f = (lambda x, axes=(-2,-1): jnp.fft.rfft2(x.astype(jnp.float32), axes=axes))(kv_pad[:, None, :, :], axes=(1, 2))
        kf_f = (lambda x, axes=(-2,-1): jnp.fft.rfft2(x.astype(jnp.float32), axes=axes))(kf_pad[:, None, :], axes=(1, 2))
        kf_f = (lambda x, *d: x.transpose(*d))(kf_f, 1, 2, 0)
        y_f = kv_f * kf_f[None, :, :, :]
        y = (lambda x, s, axes=(-2,-1): jnp.fft.irfft2(x, s=s, axes=axes).astype(jnp.bfloat16))(y_f, (1, L), axes=(1, 2))[:, 0, :S, :]
        y = y + kv * ssm_D[None, None, :]
        return q * y

    a = _A_ref(A_x, A_wqkv, A_wo)
    b = _B_ref(B_q, B_k, B_v, B_shift_k, B_ssm_k, B_ssm_D)
    return jnp.concatenate([a, b], axis=-1)
```

```python
import jax
import jax.numpy as jnp
import numpy as np
import jax.experimental.pallas as pl
import jax.experimental.pallas.tpu as pltpu

S, D, H = 2048, 1024, 32
DH = D // H
CG = 128
NG = D // CG
T = 128
NC = S // T
KS = 4
RA = 256
RO = 512
F32, BF16 = jnp.float32, jnp.bfloat16


def _dft_matrices():
    k = np.concatenate([np.arange(0, T, 2), np.arange(1, T, 2)])
    ang = np.pi * (2 * k[:, None] + 1) / (2 * T) * np.arange(T)[None, :]
    re = np.cos(ang).reshape(T // 8, 1, 8, T)
    im = -np.sin(ang).reshape(T // 8, 1, 8, T)
    fwd = np.concatenate([re, im], axis=1).reshape(2 * T, T)
    inv = fwd.T / T
    return fwd.astype(BF16), inv.astype(BF16)


_FWD, _INV = _dft_matrices()


def _dot(a, b):
    return jnp.dot(a, b, preferred_element_type=F32)


def _dot_nt(a, b):
    return jax.lax.dot_general(a, b, (((1,), (1,)), ((), ())), preferred_element_type=F32)


def _dot_tn(a, b):
    return jax.lax.dot_general(a, b, (((0,), (0,)), ((), ())), preferred_element_type=F32)


def _phi(t):
    return jnp.where(t > 0, t + 1.0, jnp.exp(t)) + 1e-6


def _kernel(x_hbm, wqkv_hbm, wo_hbm, q_hbm, k_hbm, v_hbm, h_hbm, shk_ref, dd_ref, fwd_ref, inv_ref,
            out_hbm,
            x_buf, w_buf, wo_buf, q_buf, k_buf, v_buf, h_buf, kf_buf, kv_buf, xf_buf, hf_buf, yf_buf,
            pq_buf, m_buf, ob_buf, oa_buf, x_sem, in_sem, ob_sem, oa_sem):

    def in_copies(g, slot):
        c0 = pl.multiple_of(g * CG, CG)
        cps = [pltpu.make_async_copy(k_hbm.at[:, pl.ds(c0, CG)], k_buf.at[slot], in_sem.at[slot, 0]),
               pltpu.make_async_copy(v_hbm.at[:, pl.ds(c0, CG)], v_buf.at[slot], in_sem.at[slot, 1]),
               pltpu.make_async_copy(h_hbm.at[pl.ds(c0, CG), :], h_buf.at[slot], in_sem.at[slot, 2])]
        for p in range(3):
            cps.append(pltpu.make_async_copy(
                wqkv_hbm.at[:, pl.ds(pl.multiple_of(p * D + c0, CG), CG)],
                w_buf.at[slot, :, pl.ds(p * CG, CG)], in_sem.at[slot, 3 + p]))
        cps.append(pltpu.make_async_copy(q_hbm.at[:, pl.ds(c0, CG)], q_buf.at[slot], in_sem.at[slot, 6]))
        cps.append(pltpu.make_async_copy(wo_hbm.at[pl.ds(c0, CG), :], wo_buf.at[slot], in_sem.at[slot, 7]))
        return cps

    def ob_copy(g, slot):
        c0 = pl.multiple_of(D + g * CG, CG)
        return pltpu.make_async_copy(ob_buf.at[slot], out_hbm.at[:, pl.ds(c0, CG)], ob_sem.at[slot])

    def oa_copy(i, slot):
        r0 = pl.multiple_of(i * RO, RO)
        return pltpu.make_async_copy(oa_buf.at[slot], out_hbm.at[pl.ds(r0, RO), pl.ds(0, D)], oa_sem.at[slot])

    x_copy = pltpu.make_async_copy(x_hbm, x_buf, x_sem.at[0])
    for c in in_copies(0, 0):
        c.start()
    x_copy.start()
    kf_buf[0:8, :] = jnp.zeros((8, CG), F32)
    x_copy.wait()

    def group_step(g, carry):
        slot = g % 2
        for c in in_copies(g, slot):
            c.wait()

        @pl.when(g + 1 < NG)
        def _():
            for c in in_copies(g + 1, 1 - slot):
                c.start()

        @pl.when(g >= 2)
        def _():
            ob_copy(g - 2, slot).wait()

        shk = shk_ref[pl.ds(pl.multiple_of(g * CG, CG), CG), :].astype(F32)
        taps = [jnp.broadcast_to(shk[:, t:t + 1], (CG, CG)).T[0:8, :] for t in range(KS)]
        taps = [jnp.concatenate([tp] * (T // 8), axis=0) for tp in taps]
        row8 = jax.lax.broadcasted_iota(jnp.int32, (NG, CG), 0)
        dvec = jnp.sum(jnp.where(row8 == g, dd_ref[...].astype(F32), 0.0), axis=0, keepdims=True)

        st = {"z": None, "kv": None}

        def a_piece(c):
            rows = pl.ds(c * RA, RA)
            qkv = _dot(x_buf[rows, :], w_buf[slot])
            pq_buf[g, rows, :] = _phi(qkv[:, 0:CG]).astype(BF16)
            pk = _phi(qkv[:, CG:2 * CG])
            z = jnp.sum(pk.reshape(RA // 8, 8, CG), axis=0)
            kv = _dot_tn(pk.astype(BF16), qkv[:, 2 * CG:].astype(BF16))
            st["z"] = z if st["z"] is None else st["z"] + z
            st["kv"] = kv if st["kv"] is None else st["kv"] + kv

        def b_pre(j):
            rows = pl.ds(j * T, T)
            kf_buf[pl.ds(8 + j * T, T), :] = k_buf[slot, rows, :].astype(F32)
            acc = None
            for t in range(KS):
                term = kf_buf[pl.ds(8 + j * T - t, T), :] * taps[t]
                acc = term if acc is None else acc + term
            kv_buf[rows, :] = (acc * v_buf[slot, rows, :].astype(F32)).astype(BF16)

        def b_fwd_h(j):
            hf_buf[j] = _dot_nt(fwd_ref[...], h_buf[slot, :, pl.ds(j * T, T)])

        def b_fwd_x(j):
            xf_buf[j] = _dot(fwd_ref[...], kv_buf[pl.ds(j * T, T), :])

        def b_mac(r):
            re, im = pl.ds(16 * r, 8), pl.ds(16 * r + 8, 8)
            even = r < T // 16
            prev = None
            nb = 4
            for i0 in range(0, NC, nb):
                acc = [None] * nb
                hs = {}
                for j in range(i0 + nb):
                    xr, xi = xf_buf[j, re, :], xf_buf[j, im, :]
                    for a in range(nb):
                        m = i0 + a - j
                        if m < 0:
                            continue
                        if m not in hs:
                            hs[m] = (hf_buf[m, re, :], hf_buf[m, im, :])
                        hr, hi = hs[m]
                        pr = hr * xr - hi * xi
                        pi = hr * xi + hi * xr
                        acc[a] = (pr, pi) if acc[a] is None else (acc[a][0] + pr, acc[a][1] + pi)
                for a in range(nb):
                    yr, yi = acc[a]
                    if prev is not None:
                        if even:
                            yr, yi = yr - prev[1], yi + prev[0]
                        else:
                            yr, yi = yr + prev[1], yi - prev[0]
                    prev = acc[a]
                    yf_buf[i0 + a, pl.ds(16 * r, 16), :] = jnp.concatenate([yr, yi], axis=0).astype(BF16)

        def b_post(i):
            rows = pl.ds(i * T, T)
            y = _dot(inv_ref[...], yf_buf[i]) + kv_buf[rows, :].astype(F32) * dvec
            ob_buf[slot, rows, :] = (q_buf[slot, rows, :].astype(F32) * y).astype(BF16)

        def a_tail_m():
            hr = jax.lax.broadcasted_iota(jnp.int32, (CG, CG), 0) // DH
            hc = jax.lax.broadcasted_iota(jnp.int32, (CG, CG), 1) // DH
            same = hr == hc
            kvbd = jnp.where(same, st["kv"], 0.0).astype(BF16)
            m_buf[pl.ds(pl.multiple_of(g * CG, CG), CG), :] = _dot(kvbd, wo_buf[slot]).astype(BF16)
            z = jnp.sum(st["z"], axis=0, keepdims=True)
            st["zbd"] = jnp.where(same, z, 0.0).astype(BF16)

        def a_tail(c):
            rows = pl.ds(c * RA, RA)
            pq = pq_buf[g, rows, :]
            den = _dot_nt(pq, st["zbd"]) + 1e-6
            pq_buf[g, rows, :] = (pq.astype(F32) / den).astype(BF16)

        na = S // RA
        n0 = na // 4
        for c in range(n0):
            a_piece(c)
            for j in range(c * NC // n0, (c + 1) * NC // n0):
                b_pre(j)
                b_fwd_h(j)
        for j in range(NC):
            b_fwd_x(j)
        nr = T // 8
        for c in range(n0, na):
            a_piece(c)
            for r in range((c - n0) * nr // (na - n0), (c - n0 + 1) * nr // (na - n0)):
                b_mac(r)
        a_tail_m()
        for c in range(na):
            for i in range(c * NC // na, (c + 1) * NC // na):
                b_post(i)
            a_tail(c)
        ob_copy(g, slot).start()
        return carry

    jax.lax.fori_loop(0, NG, group_step, 0)

    def out_step(i, carry):
        slot = i % 2

        @pl.when(i >= 2)
        def _():
            oa_copy(i - 2, slot).wait()

        rows = pl.ds(pl.multiple_of(i * RO, RO), RO)
        pq = jnp.concatenate([pq_buf[g, rows, :] for g in range(NG)], axis=1)
        oa_buf[slot] = _dot(pq, m_buf[...]).astype(BF16)
        oa_copy(i, slot).start()
        return carry

    jax.lax.fori_loop(0, S // RO, out_step, 0)
    ob_copy(NG - 2, 0).wait()
    ob_copy(NG - 1, 1).wait()
    oa_copy(S // RO - 2, 0).wait()
    oa_copy(S // RO - 1, 1).wait()


@jax.jit
def pallas_concat_heads__linear_attn_block__ssm_conv_h3__prompt_kernel(
    A_x: jax.Array,
    A_wqkv: jax.Array,
    A_wo: jax.Array,
    B_q: jax.Array,
    B_k: jax.Array,
    B_v: jax.Array,
    B_shift_k: jax.Array,
    B_ssm_k: jax.Array,
    B_ssm_D: jax.Array,
):
    hbm = pl.BlockSpec(memory_space=pl.ANY)
    vmem = pl.BlockSpec(memory_space=pltpu.VMEM)
    out = pl.pallas_call(
        _kernel,
        out_shape=jax.ShapeDtypeStruct((S, 2 * D), BF16),
        in_specs=[hbm] * 7 + [vmem] * 4,
        out_specs=hbm,
        scratch_shapes=[
            pltpu.VMEM((S, D), BF16),
            pltpu.VMEM((2, D, 3 * CG), BF16),
            pltpu.VMEM((2, CG, D), BF16),
            pltpu.VMEM((2, S, CG), BF16),
            pltpu.VMEM((2, S, CG), BF16),
            pltpu.VMEM((2, S, CG), BF16),
            pltpu.VMEM((2, CG, S), BF16),
            pltpu.VMEM((S + 8, CG), F32),
            pltpu.VMEM((S, CG), BF16),
            pltpu.VMEM((NC, 2 * T, CG), F32),
            pltpu.VMEM((NC, 2 * T, CG), F32),
            pltpu.VMEM((NC, 2 * T, CG), BF16),
            pltpu.VMEM((NG, S, CG), BF16),
            pltpu.VMEM((D, D), BF16),
            pltpu.VMEM((2, S, CG), BF16),
            pltpu.VMEM((2, RO, D), BF16),
            pltpu.SemaphoreType.DMA((1,)),
            pltpu.SemaphoreType.DMA((2, 8)),
            pltpu.SemaphoreType.DMA((2,)),
            pltpu.SemaphoreType.DMA((2,)),
        ],
        compiler_params=pltpu.CompilerParams(vmem_limit_bytes=96 * 1024 * 1024),
    )(A_x.reshape(S, D), A_wqkv, A_wo, B_q.reshape(S, D), B_k.reshape(S, D), B_v.reshape(S, D),
      B_ssm_k, B_shift_k, B_ssm_D.reshape(NG, CG), _FWD, _INV)
    return out.reshape(1, S, 2 * D)
```

```python
import jax
import jax.numpy as jnp
import numpy as np
import jax.experimental.pallas as pl
import jax.experimental.pallas.tpu as pltpu

S, D, H = 2048, 1024, 32
DH = D // H
CG = 128
NG = D // CG
T = 128
NC = S // T
KS = 4
RA = 128
NSA = 1
NB = 2
RP = 32
LAG_X = 2
LAG_KV = 1536
MAC_RATE = 1.0
FLAGS = None
RO = 128
XC = 4
F32, BF16, U32 = jnp.float32, jnp.bfloat16, jnp.uint32


def _dft_matrices():
    k = np.concatenate([np.arange(0, T, 2), np.arange(1, T, 2)])
    ang = np.pi * (2 * k[:, None] + 1) / (2 * T) * np.arange(T)[None, :]
    re = np.cos(ang).reshape(T // 8, 1, 8, T)
    im = -np.sin(ang).reshape(T // 8, 1, 8, T)
    fwd = np.concatenate([re, im], axis=1).reshape(2 * T, T)
    inv = fwd.T / T
    inv = np.stack([inv[:, :T], inv[:, T:]])
    return fwd.astype(BF16), inv.astype(BF16)


_FWD, _INV = _dft_matrices()


def _dot(a, b):
    return jnp.dot(a, b, preferred_element_type=F32)


def _dot_nt(a, b):
    return jax.lax.dot_general(a, b, (((1,), (1,)), ((), ())), preferred_element_type=F32)


def _dot_tn(a, b):
    return jax.lax.dot_general(a, b, (((0,), (0,)), ((), ())), preferred_element_type=F32)


def _phi(t):
    return jnp.where(t > 0, t + 1.0, jnp.exp(t)) + 1e-6


def _ld(ref, lead, r0, n):
    return pltpu.bitcast(ref.bitcast(U32)[lead + (pl.ds(r0 // 2, n // 2), slice(None))], BF16)


def _merge(*streams):
    done = [0.0] * len(streams)
    live = list(range(len(streams)))
    while live:
        i = min(live, key=lambda s: done[s] / streams[s][1])
        cost = next(streams[i][0], None)
        if cost is None:
            live.remove(i)
        else:
            done[i] += cost


def _kernel(x_hbm, wqkv_hbm, wo_hbm, q_hbm, k_hbm, v_hbm, h_hbm, shk_ref, dd_ref, fwd_ref, inv_ref,
            out_hbm,
            x_buf, w_buf, wo_buf, q_buf, k_buf, v_buf, h_buf, tap_buf, kf_buf, kv_buf, xf_buf, hf_buf,
            yf_buf, pk_buf, pv_buf, z_buf, zbd_buf, kvs_buf, kvbd_buf, pq_buf, m_buf, ob_buf, oa_buf, x_sem, in_sem, ob_sem, oa_sem, fence_sem):

    def rows_of(i, n):
        return i * n if isinstance(i, int) else pl.multiple_of(i * n, n)

    def col_copy(hbm, c0, dst, sem):
        return pltpu.make_async_copy(hbm.at[:, pl.ds(c0, CG)], dst, sem)

    def in_copies(g, slot, which):
        c0 = rows_of(g, CG)
        sem = in_sem.at[slot, which]
        if which == 0:
            return [pltpu.make_async_copy(h_hbm.at[pl.ds(c0, CG), pl.ds(j * T, T)], h_buf.at[slot, j], sem)
                    for j in range(NC)]
        if which == 1:
            return [col_copy(k_hbm, c0, k_buf.at[slot], sem)]
        if which == 2:
            return [col_copy(v_hbm, c0, v_buf.at[slot], sem)]
        if which == 3:
            return [col_copy(wqkv_hbm, rows_of(p * NG + g, CG), w_buf.at[slot, p], sem) for p in range(3)]
        if which == 4:
            return [col_copy(q_hbm, c0, q_buf.at[slot], sem)]
        return [pltpu.make_async_copy(wo_hbm.at[pl.ds(c0, CG), pl.ds(n * CG, CG)], wo_buf.at[slot, n], sem)
                for n in range(NG)]

    def in_wait(slot, which):
        buf = (h_buf, k_buf, v_buf, w_buf, q_buf, wo_buf)[which].at[slot]
        pltpu.make_async_copy(buf, buf, in_sem.at[slot, which]).wait()

    def in_start(g, slot, whiches):
        for which in whiches:
            for c in in_copies(g, slot, which):
                c.start()

    RX = S // XC

    def x_start(c):
        for kb in range(NG):
            pltpu.make_async_copy(x_hbm.at[pl.ds(c * RX, RX), pl.ds(kb * CG, CG)],
                                  x_buf.at[c, kb], x_sem.at[c]).start()

    def x_wait(c):
        pltpu.make_async_copy(x_buf.at[c], x_buf.at[c], x_sem.at[c]).wait()

    def ob_copy(g):
        return pltpu.make_async_copy(ob_buf.at[g], out_hbm.at[:, pl.ds(rows_of(NG + g, CG), CG)], ob_sem.at[g])

    def oa_copy(i):
        return pltpu.make_async_copy(oa_buf.at[pl.ds(i * RO, RO)],
                                     out_hbm.at[pl.ds(i * RO, RO), pl.ds(0, D)], oa_sem.at[i])

    def kv_block(b):
        kv = _dot_tn(_ld(pk_buf, (), b * CG, CG), _ld(pv_buf, (), b * CG, CG))
        kvs_buf[...] = kv if b == 0 else kvs_buf[...] + kv

    def b_filter(g):
        for j in range(NC):
            hf_buf[j] = _dot_nt(_ld(fwd_ref, (), 0, 2 * T), _ld(h_buf, (g % 2, j), 0, CG))
            yield 1

    def b_pre(g):
        slot = g % 2
        taps = [jnp.concatenate([tap_buf[g, t]] * (RP // 8), axis=0) for t in range(KS)]
        for r0 in range(0, S, RP):
            kf = _ld(k_buf, (slot,), r0, RP).astype(F32)
            kf_buf[pl.ds(8 + r0, RP), :] = kf
            acc = kf * taps[0]
            for t in range(1, KS):
                acc = acc + kf_buf[pl.ds(8 + r0 - t, RP), :] * taps[t]
            kv_buf[slot, pl.ds(r0, RP), :] = (acc * _ld(v_buf, (slot,), r0, RP).astype(F32)).astype(BF16)
            yield RP

    def b_signal(g):
        for j in range(NC):
            xf_buf[j] = _dot(_ld(fwd_ref, (), 0, 2 * T), _ld(kv_buf, (g % 2,), j * T, T))
            yield 1

    def a_main(g, first):
        slot = g % 2
        todo = []
        n = 0
        zs = None
        for r0 in range(0, S, RA):
            if first and r0 == 0:
                in_wait(slot, 3)
            if first and r0 % RX == 0:
                x_wait(r0 // RX)
                fence()
            cols = []
            for p0 in range(0, 3, NSA):
                acc = None
                for kb in range(NG):
                    w = jnp.concatenate([_ld(w_buf, (slot, p), kb * CG, CG) for p in range(p0, p0 + NSA)], axis=1)
                    part = _dot(_ld(x_buf, (r0 // RX, kb), r0 % RX, RA), w)
                    acc = part if acc is None else acc + part
                    n += RA * NSA
                    yield RA * NSA
                    if todo and todo[0][0] <= n:
                        kv_block(todo.pop(0)[1])
                        yield CG
                cols += [acc[:, p * CG:(p + 1) * CG] for p in range(NSA)]
            rows = pl.ds(r0, RA)
            pq_buf[g, rows, :] = _phi(cols[0]).astype(BF16)
            pk = _phi(cols[1])
            z = jnp.sum(pk.reshape(RA // 8, 8, CG), axis=0)
            zs = z if zs is None else zs + z
            pk_buf[rows, :] = pk.astype(BF16)
            pv_buf[rows, :] = cols[2].astype(BF16)
            if (r0 + RA) % CG == 0 and r0 + RA < S:
                todo.append((n + LAG_KV, (r0 + RA) // CG - 1))
        for _, b in todo:
            kv_block(b)
        z_buf[...] = zs

    def b_mac():
        for r in range(T // 8):
            re, im = pl.ds(16 * r, 8), pl.ds(16 * r + 8, 8)
            even = r < T // 16
            prev = None
            for i0 in range(0, NC, NB):
                acc = [None] * NB
                hs = {}
                for j in range(i0 + NB):
                    xr, xi = xf_buf[j, re, :], xf_buf[j, im, :]
                    n = 0
                    for a in range(NB):
                        m = i0 + a - j
                        if m < 0:
                            continue
                        if m not in hs:
                            hs[m] = (hf_buf[m, re, :], hf_buf[m, im, :])
                        hr, hi = hs[m]
                        pr = hr * xr - hi * xi
                        pi = hr * xi + hi * xr
                        acc[a] = (pr, pi) if acc[a] is None else (acc[a][0] + pr, acc[a][1] + pi)
                        n += 1
                    yield n
                for a in range(NB):
                    yr, yi = acc[a]
                    if prev is not None:
                        yr, yi = (yr - prev[1], yi + prev[0]) if even else (yr + prev[1], yi - prev[0])
                    prev = acc[a]
                    yf_buf[i0 + a, pl.ds(16 * r, 16), :] = jnp.concatenate([yr, yi], axis=0).astype(BF16)

    def b_post(g):
        slot = g % 2
        dvec = jnp.concatenate([tap_buf[g, KS]] * (T // 8), axis=0)
        for i in range(NC):
            inv = jnp.concatenate([_ld(inv_ref, (0,), 0, T), _ld(inv_ref, (1,), 0, T)], axis=1)
            y = _dot(inv, _ld(yf_buf, (i,), 0, 2 * T)) + _ld(kv_buf, (slot,), i * T, T).astype(F32) * dvec
            ob_buf[g, pl.ds(i * T, T), :] = (_ld(q_buf, (slot,), i * T, T).astype(F32) * y).astype(BF16)
            yield 1

    def a_heads():
        kv_block(S // CG - 1)
        same = (jax.lax.broadcasted_iota(jnp.int32, (CG, CG), 0) // DH
                == jax.lax.broadcasted_iota(jnp.int32, (CG, CG), 1) // DH)
        z = jnp.sum(z_buf[...], axis=0, keepdims=True)
        zbd_buf[...] = jnp.where(same, z, 0.0).T.astype(BF16)
        kvbd_buf[...] = jnp.where(same, kvs_buf[...], 0.0).astype(BF16)

    def a_norm(g):
        for r0 in range(0, S, CG):
            pq = _ld(pq_buf, (g,), r0, CG)
            den = _dot(pq, _ld(zbd_buf, (), 0, CG)) + 1e-6
            rcp = pl.reciprocal(den, approx=True)
            rcp = rcp * (2.0 - den * rcp)
            pq_buf[g, pl.ds(r0, CG), :] = (pq.astype(F32) * rcp).astype(BF16)
            yield 1

    def a_mix(g):
        for n in range(NG):
            m_buf[n, pl.ds(rows_of(g, CG), CG), :] = _dot(
                _ld(kvbd_buf, (), 0, CG), _ld(wo_buf, (g % 2, n), 0, CG)).astype(BF16)
            yield 1

    def fence():
        pl.semaphore_signal(fence_sem, 1)
        pl.semaphore_wait(fence_sem, 1)

    MAIN_COST = S * (3 * NG + 1)
    MAC_COST = MAC_RATE * (T // 8) * NC * (NC + 1) / 2

    def group_step(g, first):
        slot = g % 2
        if first:
            in_wait(slot, 0)
            _merge((b_filter(g), NC))
            in_wait(slot, 1)
            in_wait(slot, 2)
            in_start(1, 1, range(4))
            in_start(0, 0, range(4, 6))
            _merge((b_pre(g), S))
            fence()
            _merge((b_signal(g), NC))
        else:
            for which in range(4):
                in_wait(slot, which)
            for which in range(4, 6):
                in_wait(1 - slot, which)
            in_start(g, slot, range(4, 6))

            @pl.when(g + 1 < NG)
            def _():
                in_start(g + 1, 1 - slot, range(4))

            a_heads()
            _merge((b_filter(g), NC), (b_post(g - 1), NC), (b_pre(g), S))
            ob_copy(g - 1).start()
            fence()
            _merge((b_signal(g), NC), (a_norm(g - 1), S // CG), (a_mix(g - 1), NG))
        fence()
        _merge((a_main(g, first), MAIN_COST), (b_mac(), MAC_COST))
        fence()

    in_start(0, 0, range(4))
    for c in range(XC):
        x_start(c)
    kf_buf[0:8, :] = jnp.zeros((8, CG), F32)
    shk = shk_ref[...].astype(F32)
    dd = dd_ref[...].astype(F32)
    for g in range(NG):
        for t in range(KS):
            tap_buf[g, t] = jnp.broadcast_to(shk[t:t + 1, g * CG:(g + 1) * CG], (8, CG))
        tap_buf[g, KS] = jnp.broadcast_to(dd[g:g + 1, :], (8, CG))

    group_step(0, True)

    def loop_body(g, carry):
        group_step(g, False)
        return carry

    jax.lax.fori_loop(1, NG, loop_body, 0)

    for which in range(4, 6):
        in_wait((NG - 1) % 2, which)
    a_heads()
    _merge((b_post(NG - 1), NC))
    ob_copy(NG - 1).start()
    fence()
    _merge((a_norm(NG - 1), S // CG), (a_mix(NG - 1), NG))
    fence()

    for i in range(S // RO):
        pq = jnp.concatenate([_ld(pq_buf, (g,), i * RO, RO) for g in range(NG)], axis=1)
        m = jnp.concatenate([_ld(m_buf, (n,), 0, D) for n in range(NG)], axis=1)
        oa_buf[pl.ds(i * RO, RO), :] = _dot(pq, m).astype(BF16)
        oa_copy(i).start()
    for g in range(NG):
        ob_copy(g).wait()
    for i in range(S // RO):
        oa_copy(i).wait()


@jax.jit
def pallas_concat_heads__linear_attn_block__ssm_conv_h3__prompt_kernel(
    A_x: jax.Array,
    A_wqkv: jax.Array,
    A_wo: jax.Array,
    B_q: jax.Array,
    B_k: jax.Array,
    B_v: jax.Array,
    B_shift_k: jax.Array,
    B_ssm_k: jax.Array,
    B_ssm_D: jax.Array,
):
    hbm = pl.BlockSpec(memory_space=pl.ANY)
    vmem = pl.BlockSpec(memory_space=pltpu.VMEM)
    out = pl.pallas_call(
        _kernel,
        out_shape=jax.ShapeDtypeStruct((S, 2 * D), BF16),
        in_specs=[hbm] * 7 + [vmem] * 4,
        out_specs=hbm,
        scratch_shapes=[
            pltpu.VMEM((XC, NG, S // XC, CG), BF16),
            pltpu.VMEM((2, 3, D, CG), BF16),
            pltpu.VMEM((2, NG, CG, CG), BF16),
            pltpu.VMEM((2, S, CG), BF16),
            pltpu.VMEM((2, S, CG), BF16),
            pltpu.VMEM((2, S, CG), BF16),
            pltpu.VMEM((2, NC, CG, T), BF16),
            pltpu.VMEM((NG, KS + 1, 8, CG), F32),
            pltpu.VMEM((S + 8, CG), F32),
            pltpu.VMEM((2, S, CG), BF16),
            pltpu.VMEM((NC, 2 * T, CG), F32),
            pltpu.VMEM((NC, 2 * T, CG), F32),
            pltpu.VMEM((NC, 2 * T, CG), BF16),
            pltpu.VMEM((S, CG), BF16),
            pltpu.VMEM((S, CG), BF16),
            pltpu.VMEM((8, CG), F32),
            pltpu.VMEM((CG, CG), BF16),
            pltpu.VMEM((CG, CG), F32),
            pltpu.VMEM((CG, CG), BF16),
            pltpu.VMEM((NG, S, CG), BF16),
            pltpu.VMEM((NG, D, CG), BF16),
            pltpu.VMEM((NG, S, CG), BF16),
            pltpu.VMEM((S, D), BF16),
            pltpu.SemaphoreType.DMA((XC,)),
            pltpu.SemaphoreType.DMA((2, 6)),
            pltpu.SemaphoreType.DMA((NG,)),
            pltpu.SemaphoreType.DMA((S // RO,)),
            pltpu.SemaphoreType.REGULAR,
        ],
        compiler_params=pltpu.CompilerParams(vmem_limit_bytes=96 * 1024 * 1024, flags=FLAGS),
    )(A_x.reshape(S, D), A_wqkv, A_wo, B_q.reshape(S, D), B_k.reshape(S, D), B_v.reshape(S, D),
      B_ssm_k, B_shift_k.T, B_ssm_D.reshape(NG, CG), _FWD, _INV)
    return out.reshape(1, S, 2 * D)
```

```python
import jax
import jax.numpy as jnp
import numpy as np
import jax.experimental.pallas as pl
import jax.experimental.pallas.tpu as pltpu

S, D, H = 2048, 1024, 32
DH = D // H
CG = 128
NG = D // CG
T = 128
NC = S // T
KS = 4
RA = 128
NSA = 1
NB = 2
RP = 32
PRE_CHUNKS = 3
NSO = 1
LAG_KV = 1536
MAC_RATE = 1.0
FLAGS = None
RO = 128
XC = 8
F32, BF16, U32 = jnp.float32, jnp.bfloat16, jnp.uint32


def _dft_matrices():
    k = np.concatenate([np.arange(0, T, 2), np.arange(1, T, 2)])
    ang = np.pi * (2 * k[:, None] + 1) / (2 * T) * np.arange(T)[None, :]
    re = np.cos(ang).reshape(T // 8, 1, 8, T)
    im = -np.sin(ang).reshape(T // 8, 1, 8, T)
    fwd = np.concatenate([re, im], axis=1).reshape(2 * T, T)
    inv = fwd.T / T
    inv = np.stack([inv[:, :T], inv[:, T:]])
    return fwd.astype(BF16), inv.astype(BF16)


_FWD, _INV = _dft_matrices()


def _dot(a, b):
    return jnp.dot(a, b, preferred_element_type=F32)


def _dot_nt(a, b):
    return jax.lax.dot_general(a, b, (((1,), (1,)), ((), ())), preferred_element_type=F32)


def _dot_tn(a, b):
    return jax.lax.dot_general(a, b, (((0,), (0,)), ((), ())), preferred_element_type=F32)


def _phi(t):
    return jnp.where(t > 0, t + 1.0, jnp.exp(t)) + 1e-6


def _ld(ref, lead, r0, n):
    return pltpu.bitcast(ref.bitcast(U32)[lead + (pl.ds(r0 // 2, n // 2), slice(None))], BF16)


def _merge(*streams):
    done = [0.0] * len(streams)
    live = list(range(len(streams)))
    while live:
        i = min(live, key=lambda s: done[s] / streams[s][1])
        cost = next(streams[i][0], None)
        if cost is None:
            live.remove(i)
        else:
            done[i] += cost


def _kernel(x_hbm, wqkv_hbm, wo_hbm, q_hbm, k_hbm, v_hbm, h_hbm, shk_ref, dd_ref, fwd_ref, inv_ref,
            out_hbm,
            x_buf, w_buf, wo_buf, q_buf, k_buf, v_buf, h_buf, tap_buf, kf_buf, kv_buf, xf_buf, hf_buf,
            yf_buf, pk_buf, pv_buf, z_buf, zbd_buf, kvs_buf, kvbd_buf, pq_buf, m_buf, ob_buf, oa_buf, x_sem, in_sem, ob_sem, oa_sem, fence_sem):

    def rows_of(i, n):
        return i * n if isinstance(i, int) else pl.multiple_of(i * n, n)

    def col_copy(hbm, c0, dst, sem):
        return pltpu.make_async_copy(hbm.at[:, pl.ds(c0, CG)], dst, sem)

    H_IN, K_IN, V_IN, W_IN, Q_IN, WO_IN = range(6)

    def in_copies(g, which):
        c0 = rows_of(g, CG)
        sem = in_sem.at[g, which]
        if which == H_IN:
            return [pltpu.make_async_copy(h_hbm.at[pl.ds(c0, CG), pl.ds(j * T, T)], h_buf.at[g, j], sem)
                    for j in range(NC)]
        if which == W_IN:
            return [col_copy(wqkv_hbm, rows_of(p * NG + g, CG), w_buf.at[g, p], sem) for p in range(3)]
        if which == WO_IN:
            return [pltpu.make_async_copy(wo_hbm.at[pl.ds(c0, CG), pl.ds(n * CG, CG)], wo_buf.at[g, n], sem)
                    for n in range(NG)]
        hbm, buf = {K_IN: (k_hbm, k_buf), V_IN: (v_hbm, v_buf), Q_IN: (q_hbm, q_buf)}[which]
        return [col_copy(hbm, c0, buf.at[g], sem)]

    def in_start(g, *whiches):
        for which in whiches:
            for c in in_copies(g, which):
                c.start()

    def in_wait(g, *whiches):
        for which in whiches:
            buf = (h_buf, k_buf, v_buf, w_buf, q_buf, wo_buf)[which].at[g]
            pltpu.make_async_copy(buf, buf, in_sem.at[g, which]).wait()

    RX = S // XC

    def x_start(c):
        for kb in range(NG):
            pltpu.make_async_copy(x_hbm.at[pl.ds(c * RX, RX), pl.ds(kb * CG, CG)],
                                  x_buf.at[c, kb], x_sem.at[c]).start()

    def x_wait(c):
        pltpu.make_async_copy(x_buf.at[c], x_buf.at[c], x_sem.at[c]).wait()

    def ob_copy(g):
        return pltpu.make_async_copy(ob_buf.at[g], out_hbm.at[:, pl.ds(rows_of(NG + g, CG), CG)], ob_sem.at[g])

    def oa_copy(i):
        return pltpu.make_async_copy(oa_buf.at[pl.ds(i * RO, RO)],
                                     out_hbm.at[pl.ds(i * RO, RO), pl.ds(0, D)], oa_sem.at[i])

    def kv_block(b):
        kv = _dot_tn(_ld(pk_buf, (), b * CG, CG), _ld(pv_buf, (), b * CG, CG))
        kvs_buf[...] = kv if b == 0 else kvs_buf[...] + kv

    def b_filter(g):
        for j in range(NC):
            hf_buf[j] = _dot_nt(_ld(fwd_ref, (), 0, 2 * T), _ld(h_buf, (g, j), 0, CG))
            yield 1

    def b_pre(g):
        slot = g % 2
        taps = [jnp.concatenate([tap_buf[g, t]] * (RP // 8), axis=0) for t in range(KS)]
        for r0 in range(0, S, RP):
            kf = _ld(k_buf, (g,), r0, RP).astype(F32)
            kf_buf[pl.ds(8 + r0, RP), :] = kf
            acc = kf * taps[0]
            for t in range(1, KS):
                acc = acc + kf_buf[pl.ds(8 + r0 - t, RP), :] * taps[t]
            kv_buf[slot, pl.ds(r0, RP), :] = (acc * _ld(v_buf, (g,), r0, RP).astype(F32)).astype(BF16)
            yield RP

    def b_signal(g):
        for j in range(NC):
            xf_buf[j] = _dot(_ld(fwd_ref, (), 0, 2 * T), _ld(kv_buf, (g % 2,), j * T, T))
            yield 1

    def a_main(g, before_rows=None):
        todo = []
        n = 0
        zs = None
        for r0 in range(0, S, RA):
            if before_rows is not None:
                before_rows(r0)
            cols = []
            for p0 in range(0, 3, NSA):
                acc = None
                for kb in range(NG):
                    w = jnp.concatenate([_ld(w_buf, (g, p), kb * CG, CG) for p in range(p0, p0 + NSA)], axis=1)
                    part = _dot(_ld(x_buf, (r0 // RX, kb), r0 % RX, RA), w)
                    acc = part if acc is None else acc + part
                    n += RA * NSA
                    yield RA * NSA
                    if todo and todo[0][0] <= n:
                        kv_block(todo.pop(0)[1])
                        yield CG
                cols += [acc[:, p * CG:(p + 1) * CG] for p in range(NSA)]
            rows = pl.ds(r0, RA)
            pq_buf[g, rows, :] = _phi(cols[0]).astype(BF16)
            pk = _phi(cols[1])
            z = jnp.sum(pk.reshape(RA // 8, 8, CG), axis=0)
            zs = z if zs is None else zs + z
            pk_buf[rows, :] = pk.astype(BF16)
            pv_buf[rows, :] = cols[2].astype(BF16)
            if (r0 + RA) % CG == 0 and r0 + RA < S:
                todo.append((n + LAG_KV, (r0 + RA) // CG - 1))
        for _, b in todo:
            kv_block(b)
        z_buf[...] = zs

    def b_mac():
        for r in range(T // 8):
            re, im = pl.ds(16 * r, 8), pl.ds(16 * r + 8, 8)
            even = r < T // 16
            prev = None
            for i0 in range(0, NC, NB):
                acc = [None] * NB
                hs = {}
                for j in range(i0 + NB):
                    xr, xi = xf_buf[j, re, :], xf_buf[j, im, :]
                    n = 0
                    for a in range(NB):
                        m = i0 + a - j
                        if m < 0:
                            continue
                        if m not in hs:
                            hs[m] = (hf_buf[m, re, :], hf_buf[m, im, :])
                        hr, hi = hs[m]
                        pr = hr * xr - hi * xi
                        pi = hr * xi + hi * xr
                        acc[a] = (pr, pi) if acc[a] is None else (acc[a][0] + pr, acc[a][1] + pi)
                        n += 1
                    yield n
                for a in range(NB):
                    yr, yi = acc[a]
                    if prev is not None:
                        yr, yi = (yr - prev[1], yi + prev[0]) if even else (yr + prev[1], yi - prev[0])
                    prev = acc[a]
                    yf_buf[i0 + a, pl.ds(16 * r, 16), :] = jnp.concatenate([yr, yi], axis=0).astype(BF16)

    def b_post(g):
        slot = g % 2
        dvec = jnp.concatenate([tap_buf[g, KS]] * (T // 8), axis=0)
        for i in range(NC):
            inv = jnp.concatenate([_ld(inv_ref, (0,), 0, T), _ld(inv_ref, (1,), 0, T)], axis=1)
            y = _dot(inv, _ld(yf_buf, (i,), 0, 2 * T)) + _ld(kv_buf, (slot,), i * T, T).astype(F32) * dvec
            ob_buf[g, pl.ds(i * T, T), :] = (_ld(q_buf, (g,), i * T, T).astype(F32) * y).astype(BF16)
            yield 1

    def a_heads():
        kv_block(S // CG - 1)
        same = (jax.lax.broadcasted_iota(jnp.int32, (CG, CG), 0) // DH
                == jax.lax.broadcasted_iota(jnp.int32, (CG, CG), 1) // DH)
        z = jnp.sum(z_buf[...], axis=0, keepdims=True)
        zbd_buf[...] = jnp.where(same, z, 0.0).T.astype(BF16)
        kvbd_buf[...] = jnp.where(same, kvs_buf[...], 0.0).astype(BF16)

    def a_norm(g):
        for r0 in range(0, S, CG):
            pq = _ld(pq_buf, (g,), r0, CG)
            den = _dot(pq, _ld(zbd_buf, (), 0, CG)) + 1e-6
            rcp = pl.reciprocal(den, approx=True)
            rcp = rcp * (2.0 - den * rcp)
            pq_buf[g, pl.ds(r0, CG), :] = (pq.astype(F32) * rcp).astype(BF16)
            yield 1

    def a_mix(g):
        for n in range(NG):
            m_buf[n, pl.ds(rows_of(g, CG), CG), :] = _dot(
                _ld(kvbd_buf, (), 0, CG), _ld(wo_buf, (g, n), 0, CG)).astype(BF16)
            yield 1

    def fence():
        pl.semaphore_signal(fence_sem, 1)
        pl.semaphore_wait(fence_sem, 1)

    def take(stream, cost):
        while cost > 0:
            c = next(stream, None)
            if c is None:
                return
            cost -= c
            yield c

    def a_out(i0, i1):
        for i in range(i0, i1):
            for n0 in range(0, NG, NSO):
                acc = None
                for g in range(NG):
                    m = jnp.concatenate([_ld(m_buf, (n,), g * CG, CG) for n in range(n0, n0 + NSO)], axis=1)
                    part = _dot(_ld(pq_buf, (g,), i * RO, RO), m)
                    acc = part if acc is None else acc + part
                    yield NSO
                oa_buf[pl.ds(i * RO, RO), pl.ds(n0 * CG, NSO * CG)] = acc.astype(BF16)
            oa_copy(i).start()

    MAIN_COST = S * (3 * NG + 1)
    MAC_COST = (T // 8) * NC * (NC + 1) // 2

    def front(g):
        a_heads()
        _merge((b_filter(g), NC), (b_signal(g), NC))

    def back(g):
        in_wait(g, Q_IN)
        _merge((b_post(g), NC))
        ob_copy(g).start()

    in_start(0, W_IN)
    x_start(0)
    x_start(1)
    kf_buf[0:8, :] = jnp.zeros((8, CG), F32)
    shk = shk_ref[...].astype(F32)
    dd = dd_ref[...].astype(F32)
    for g in range(NG):
        for t in range(KS):
            tap_buf[g, t] = jnp.broadcast_to(shk[t:t + 1, g * CG:(g + 1) * CG], (8, CG))
        tap_buf[g, KS] = jnp.broadcast_to(dd[g:g + 1, :], (8, CG))
    extra = [(0, K_IN), (0, V_IN), (0, H_IN), (0, WO_IN), (1, W_IN), (1, K_IN), (1, V_IN)]

    def fetch_rows(r0):
        if r0 % RX == 0:
            c = r0 // RX
            if c == 0:
                in_wait(0, W_IN)
            x_wait(c)
            if c + 2 < XC:
                x_start(c + 2)
            for item in extra[c * len(extra) // XC:(c + 1) * len(extra) // XC]:
                in_start(*item)
            if c == XC - PRE_CHUNKS:
                in_wait(0, K_IN, V_IN)
            fence()

    main0 = a_main(0, fetch_rows)
    _merge((take(main0, MAIN_COST * (XC - PRE_CHUNKS) // XC + LAG_KV), 1))
    _merge((main0, MAIN_COST * PRE_CHUNKS // XC - LAG_KV), (b_pre(0), S))
    fence()

    def group_step(g, carry):
        @pl.when(g + 1 < NG)
        def _():
            in_start(g + 1, W_IN, K_IN, V_IN)

        in_start(g, H_IN, WO_IN)
        in_start(g - 1, Q_IN)
        in_wait(g - 1, H_IN)
        front(g - 1)

        @pl.when(g >= 2)
        def _():
            back(g - 2)

        in_wait(g, W_IN, K_IN, V_IN)
        in_wait(g - 1, WO_IN)
        fence()
        _merge((a_main(g), MAIN_COST), (b_mac(), MAC_RATE * MAC_COST), (b_pre(g), S),
               (a_norm(g - 1), S // CG), (a_mix(g - 1), NG))
        return carry

    jax.lax.fori_loop(1, NG, group_step, 0)

    in_start(NG - 1, Q_IN)
    in_wait(NG - 1, H_IN, WO_IN)
    front(NG - 1)
    back(NG - 2)
    fence()
    mac = b_mac()
    _merge((a_norm(NG - 1), S // CG), (a_mix(NG - 1), NG), (take(mac, MAC_COST // 12), MAC_COST // 12))
    fence()
    n_out = S // RO
    n_mac = n_out * 5 // 8
    _merge((a_out(0, n_mac), n_mac * NG * NG), (mac, MAC_COST * 11 / 12))
    fence()
    in_wait(NG - 1, Q_IN)
    _merge((b_post(NG - 1), NC), (a_out(n_mac, n_mac + 2), 2 * NG * NG))
    ob_copy(NG - 1).start()
    _merge((a_out(n_mac + 2, n_out), 1))
    for g in range(NG):
        ob_copy(g).wait()
    for i in range(n_out):
        oa_copy(i).wait()


@jax.jit
def pallas_concat_heads__linear_attn_block__ssm_conv_h3__prompt_kernel(
    A_x: jax.Array,
    A_wqkv: jax.Array,
    A_wo: jax.Array,
    B_q: jax.Array,
    B_k: jax.Array,
    B_v: jax.Array,
    B_shift_k: jax.Array,
    B_ssm_k: jax.Array,
    B_ssm_D: jax.Array,
):
    hbm = pl.BlockSpec(memory_space=pl.ANY)
    vmem = pl.BlockSpec(memory_space=pltpu.VMEM)
    out = pl.pallas_call(
        _kernel,
        out_shape=jax.ShapeDtypeStruct((S, 2 * D), BF16),
        in_specs=[hbm] * 7 + [vmem] * 4,
        out_specs=hbm,
        scratch_shapes=[
            pltpu.VMEM((XC, NG, S // XC, CG), BF16),
            pltpu.VMEM((NG, 3, D, CG), BF16),
            pltpu.VMEM((NG, NG, CG, CG), BF16),
            pltpu.VMEM((NG, S, CG), BF16),
            pltpu.VMEM((NG, S, CG), BF16),
            pltpu.VMEM((NG, S, CG), BF16),
            pltpu.VMEM((NG, NC, CG, T), BF16),
            pltpu.VMEM((NG, KS + 1, 8, CG), F32),
            pltpu.VMEM((S + 8, CG), F32),
            pltpu.VMEM((2, S, CG), BF16),
            pltpu.VMEM((NC, 2 * T, CG), F32),
            pltpu.VMEM((NC, 2 * T, CG), F32),
            pltpu.VMEM((NC, 2 * T, CG), BF16),
            pltpu.VMEM((S, CG), BF16),
            pltpu.VMEM((S, CG), BF16),
            pltpu.VMEM((8, CG), F32),
            pltpu.VMEM((CG, CG), BF16),
            pltpu.VMEM((CG, CG), F32),
            pltpu.VMEM((CG, CG), BF16),
            pltpu.VMEM((NG, S, CG), BF16),
            pltpu.VMEM((NG, D, CG), BF16),
            pltpu.VMEM((NG, S, CG), BF16),
            pltpu.VMEM((S, D), BF16),
            pltpu.SemaphoreType.DMA((XC,)),
            pltpu.SemaphoreType.DMA((NG, 6)),
            pltpu.SemaphoreType.DMA((NG,)),
            pltpu.SemaphoreType.DMA((S // RO,)),
            pltpu.SemaphoreType.REGULAR,
        ],
        compiler_params=pltpu.CompilerParams(vmem_limit_bytes=96 * 1024 * 1024, flags=FLAGS),
    )(A_x.reshape(S, D), A_wqkv, A_wo, B_q.reshape(S, D), B_k.reshape(S, D), B_v.reshape(S, D),
      B_ssm_k, B_shift_k.T, B_ssm_D.reshape(NG, CG), _FWD, _INV)
    return out.reshape(1, S, 2 * D)
```

```python
import jax
import jax.numpy as jnp
import numpy as np
import jax.experimental.pallas as pl
import jax.experimental.pallas.tpu as pltpu

S, D, H = 2048, 1024, 32
DH = D // H
CG = 128
NG = D // CG
T = 128
NC = S // T
KS = 4
RA = 64
NSA = 1
NB = 2
RP = 32
EX_ROW = 1216
EX_STEP = 64
NSO = 1
LAG_KV = 3072
MAC_RATE = 1.0
FLAGS = None
RO = 128
XB = (0, 256, 640, 1216, 2048)
F32, BF16, U32 = jnp.float32, jnp.bfloat16, jnp.uint32


def _dft_matrices():
    k = np.concatenate([np.arange(0, T, 2), np.arange(1, T, 2)])
    ang = np.pi * (2 * k[:, None] + 1) / (2 * T) * np.arange(T)[None, :]
    re = np.cos(ang).reshape(T // 8, 1, 8, T)
    im = -np.sin(ang).reshape(T // 8, 1, 8, T)
    fwd = np.concatenate([re, im], axis=1).reshape(2 * T, T)
    inv = fwd.T / T
    inv = np.stack([inv[:, :T], inv[:, T:]])
    return fwd.astype(BF16), inv.astype(BF16)


_FWD, _INV = _dft_matrices()


def _dot(a, b):
    return jnp.dot(a, b, preferred_element_type=F32)


def _dot_nt(a, b):
    return jax.lax.dot_general(a, b, (((1,), (1,)), ((), ())), preferred_element_type=F32)


def _dot_tn(a, b):
    return jax.lax.dot_general(a, b, (((0,), (0,)), ((), ())), preferred_element_type=F32)


def _phi(t):
    return jnp.where(t > 0, t + 1.0, jnp.exp(t)) + 1e-6


def _ld(ref, lead, r0, n):
    return pltpu.bitcast(ref.bitcast(U32)[lead + (pl.ds(r0 // 2, n // 2), slice(None))], BF16)


def _merge(*streams):
    done = [0.0] * len(streams)
    live = list(range(len(streams)))
    while live:
        i = min(live, key=lambda s: done[s] / streams[s][1])
        cost = next(streams[i][0], None)
        if cost is None:
            live.remove(i)
        else:
            done[i] += cost


def _kernel(x_hbm, wqkv_hbm, wo_hbm, q_hbm, k_hbm, v_hbm, h_hbm, shk_ref, dd_ref, fwd_ref, inv_ref,
            out_hbm,
            xw_buf, x_buf, w_buf, wo_buf, q_buf, k_buf, v_buf, h_buf, tap_buf, kf_buf, kv_buf, xf_buf, hf_buf,
            yf_buf, pk_buf, pv_buf, z_buf, zbd_buf, kvs_buf, kvbd_buf, pq_buf, m_buf, ob_buf, oa_buf, x_sem, in_sem, ob_sem, oa_sem, fence_sem):

    def rows_of(i, n):
        return i * n if isinstance(i, int) else pl.multiple_of(i * n, n)

    def col_copy(hbm, c0, dst, sem):
        return pltpu.make_async_copy(hbm.at[:, pl.ds(c0, CG)], dst, sem)

    H_IN, K_IN, V_IN, W_IN, Q_IN, WO_IN = range(6)

    def in_copies(g, which):
        c0 = rows_of(g, CG)
        sem = in_sem.at[g, which]
        if which == H_IN:
            return [pltpu.make_async_copy(h_hbm.at[pl.ds(c0, CG)], h_buf.at[g], sem)]
        if which == WO_IN:
            return [pltpu.make_async_copy(wo_hbm.at[pl.ds(c0, CG)], wo_buf.at[g], sem)]
        if which == W_IN:
            return [col_copy(wqkv_hbm, rows_of(p * NG + g, CG), w_buf.at[g, p], sem) for p in range(3)]
        hbm, buf = {K_IN: (k_hbm, k_buf), V_IN: (v_hbm, v_buf), Q_IN: (q_hbm, q_buf)}[which]
        return [col_copy(hbm, c0, buf.at[g], sem)]

    def in_start(g, *whiches):
        for which in whiches:
            for c in in_copies(g, which):
                c.start()

    def in_wait(g, *whiches):
        for which in whiches:
            buf = (h_buf, k_buf, v_buf, w_buf, q_buf, wo_buf)[which].at[g]
            pltpu.make_async_copy(buf, buf, in_sem.at[g, which]).wait()

    def x_copy(c):
        rows = pl.ds(XB[c], XB[c + 1] - XB[c])
        return pltpu.make_async_copy(x_hbm.at[rows], xw_buf.at[rows], x_sem.at[c])

    def ob_copy(g):
        return pltpu.make_async_copy(ob_buf.at[g], out_hbm.at[:, pl.ds(rows_of(NG + g, CG), CG)], ob_sem.at[g])

    def oa_copy(i):
        return pltpu.make_async_copy(oa_buf.at[pl.ds(i * RO, RO)],
                                     out_hbm.at[pl.ds(i * RO, RO), pl.ds(0, D)], oa_sem.at[i])

    def kv_block(b):
        kv = _dot_tn(_ld(pk_buf, (), b * CG, CG), _ld(pv_buf, (), b * CG, CG))
        kvs_buf[...] = kv if b == 0 else kvs_buf[...] + kv

    def b_filter(g):
        for j in range(NC):
            hf_buf[j] = _dot_nt(_ld(fwd_ref, (), 0, 2 * T), h_buf[g, :, pl.ds(j * T, T)])
            yield 1

    def b_pre(g):
        slot = g % 2
        taps = [jnp.concatenate([tap_buf[g, t]] * (RP // 8), axis=0) for t in range(KS)]
        for r0 in range(0, S, RP):
            kf = _ld(k_buf, (g,), r0, RP).astype(F32)
            kf_buf[pl.ds(8 + r0, RP), :] = kf
            acc = kf * taps[0]
            for t in range(1, KS):
                acc = acc + kf_buf[pl.ds(8 + r0 - t, RP), :] * taps[t]
            kv_buf[slot, pl.ds(r0, RP), :] = (acc * _ld(v_buf, (g,), r0, RP).astype(F32)).astype(BF16)
            yield RP

    def b_signal(g):
        for j in range(NC):
            xf_buf[j] = _dot(_ld(fwd_ref, (), 0, 2 * T), _ld(kv_buf, (g % 2,), j * T, T))
            yield 1

    def a_main(g, before_rows=None):
        first = before_rows is not None
        todo = []
        n = 0
        zs = None
        for r0 in range(0, S, RA):
            if first:
                yield from before_rows(r0)
            cols = []
            for p0 in range(0, 3, NSA):
                acc = None
                for kb in range(NG):
                    w = jnp.concatenate([_ld(w_buf, (g, p), kb * CG, CG) for p in range(p0, p0 + NSA)], axis=1)
                    if first and p0 == 0:
                        xs = xw_buf[pl.ds(r0, RA), pl.ds(kb * CG, CG)]
                        x_buf[kb, pl.ds(r0, RA), :] = xs
                    elif first:
                        xs = xw_buf[pl.ds(r0, RA), pl.ds(kb * CG, CG)]
                    else:
                        xs = _ld(x_buf, (kb,), r0, RA)
                    part = _dot(xs, w)
                    acc = part if acc is None else acc + part
                    n += RA * NSA
                    yield RA * NSA
                    if todo and todo[0][0] <= n:
                        kv_block(todo.pop(0)[1])
                        yield CG
                cols += [acc[:, p * CG:(p + 1) * CG] for p in range(NSA)]
            rows = pl.ds(r0, RA)
            pq_buf[g, rows, :] = _phi(cols[0]).astype(BF16)
            pk = _phi(cols[1])
            z = jnp.sum(pk.reshape(RA // 8, 8, CG), axis=0)
            zs = z if zs is None else zs + z
            pk_buf[rows, :] = pk.astype(BF16)
            pv_buf[rows, :] = cols[2].astype(BF16)
            if (r0 + RA) % CG == 0 and r0 + RA < S:
                todo.append((n + LAG_KV, (r0 + RA) // CG - 1))
        for _, b in todo:
            kv_block(b)
        z_buf[...] = zs

    def b_mac():
        for r in range(T // 8):
            re, im = pl.ds(16 * r, 8), pl.ds(16 * r + 8, 8)
            even = r < T // 16
            prev = None
            for i0 in range(0, NC, NB):
                acc = [None] * NB
                hs = {}
                for j in range(i0 + NB):
                    xr, xi = xf_buf[j, re, :], xf_buf[j, im, :]
                    n = 0
                    for a in range(NB):
                        m = i0 + a - j
                        if m < 0:
                            continue
                        if m not in hs:
                            hs[m] = (hf_buf[m, re, :], hf_buf[m, im, :])
                        hr, hi = hs[m]
                        pr = hr * xr - hi * xi
                        pi = hr * xi + hi * xr
                        acc[a] = (pr, pi) if acc[a] is None else (acc[a][0] + pr, acc[a][1] + pi)
                        n += 1
                    yield n
                for a in range(NB):
                    yr, yi = acc[a]
                    if prev is not None:
                        yr, yi = (yr - prev[1], yi + prev[0]) if even else (yr + prev[1], yi - prev[0])
                    prev = acc[a]
                    yf_buf[i0 + a, pl.ds(16 * r, 16), :] = jnp.concatenate([yr, yi], axis=0).astype(BF16)

    def b_post(g):
        slot = g % 2
        dvec = jnp.concatenate([tap_buf[g, KS]] * (T // 8), axis=0)
        for i in range(NC):
            inv = jnp.concatenate([_ld(inv_ref, (0,), 0, T), _ld(inv_ref, (1,), 0, T)], axis=1)
            y = _dot(inv, _ld(yf_buf, (i,), 0, 2 * T)) + _ld(kv_buf, (slot,), i * T, T).astype(F32) * dvec
            ob_buf[g, pl.ds(i * T, T), :] = (_ld(q_buf, (g,), i * T, T).astype(F32) * y).astype(BF16)
            yield 1

    def a_heads():
        kv_block(S // CG - 1)
        same = (jax.lax.broadcasted_iota(jnp.int32, (CG, CG), 0) // DH
                == jax.lax.broadcasted_iota(jnp.int32, (CG, CG), 1) // DH)
        z = jnp.sum(z_buf[...], axis=0, keepdims=True)
        zbd_buf[...] = jnp.where(same, z, 0.0).T.astype(BF16)
        kvbd_buf[...] = jnp.where(same, kvs_buf[...], 0.0).astype(BF16)

    def a_norm(g):
        for r0 in range(0, S, CG):
            pq = _ld(pq_buf, (g,), r0, CG)
            den = _dot(pq, _ld(zbd_buf, (), 0, CG)) + 1e-6
            rcp = pl.reciprocal(den, approx=True)
            rcp = rcp * (2.0 - den * rcp)
            pq_buf[g, pl.ds(r0, CG), :] = (pq.astype(F32) * rcp).astype(BF16)
            yield 1

    def a_mix(g):
        for n in range(NG):
            m_buf[n, pl.ds(rows_of(g, CG), CG), :] = _dot(
                _ld(kvbd_buf, (), 0, CG), wo_buf[g, :, pl.ds(n * CG, CG)]).astype(BF16)
            yield 1

    def fence():
        pl.semaphore_signal(fence_sem, 1)
        pl.semaphore_wait(fence_sem, 1)

    def take(stream, cost):
        while cost > 0:
            c = next(stream, None)
            if c is None:
                return
            cost -= c
            yield c

    def a_out(i0, i1):
        for i in range(i0, i1):
            for n0 in range(0, NG, NSO):
                acc = None
                for g in range(NG):
                    m = jnp.concatenate([_ld(m_buf, (n,), g * CG, CG) for n in range(n0, n0 + NSO)], axis=1)
                    part = _dot(_ld(pq_buf, (g,), i * RO, RO), m)
                    acc = part if acc is None else acc + part
                    yield NSO
                oa_buf[pl.ds(i * RO, RO), pl.ds(n0 * CG, NSO * CG)] = acc.astype(BF16)
            oa_copy(i).start()

    MAIN_COST = S * (3 * NG + 1)
    MAC_COST = (T // 8) * NC * (NC + 1) // 2

    x_copy(0).start()
    in_start(0, W_IN)
    x_copy(1).start()
    extra = [(0, K_IN), (0, V_IN), (0, H_IN), (1, W_IN), (0, WO_IN), (1, K_IN), (1, V_IN), (1, H_IN), (0, Q_IN)]
    extra = dict(zip(range(EX_ROW, S, EX_STEP), extra))
    assert len(extra) == 9

    def fetch_rows(r0):
        if r0 in XB:
            c = XB.index(r0)
            x_copy(c).wait()
            if c == 0:
                in_wait(0, W_IN)
        if r0 - RA in XB and XB.index(r0 - RA) + 2 < len(XB) - 1:
            x_copy(XB.index(r0 - RA) + 2).start()
        if r0 in extra:
            in_start(*extra[r0])
        yield 0

    _merge((a_main(0, fetch_rows), 1))
    kf_buf[0:8, :] = jnp.zeros((8, CG), F32)
    shk = shk_ref[...].astype(F32)
    dd = dd_ref[...].astype(F32)
    for g in range(NG):
        for t in range(KS):
            tap_buf[g, t] = jnp.broadcast_to(shk[t:t + 1, g * CG:(g + 1) * CG], (8, CG))
        tap_buf[g, KS] = jnp.broadcast_to(dd[g:g + 1, :], (8, CG))
    in_wait(0, K_IN, V_IN, H_IN)
    fence()
    a_heads()
    _merge((b_filter(0), NC), (b_pre(0), S))
    fence()
    _merge((b_signal(0), NC))

    def group_step(g, carry):
        @pl.when(g + 1 < NG)
        def _():
            in_start(g + 1, W_IN, K_IN, V_IN, H_IN)

        in_start(g, WO_IN, Q_IN)
        in_wait(g, W_IN, K_IN, V_IN)
        in_wait(g - 1, WO_IN)
        fence()
        _merge((a_main(g), MAIN_COST), (b_mac(), MAC_RATE * MAC_COST), (b_pre(g), S),
               (a_norm(g - 1), S // CG), (a_mix(g - 1), NG))
        in_wait(g, H_IN)
        in_wait(g - 1, Q_IN)
        fence()
        a_heads()
        _merge((b_filter(g), NC), (b_signal(g), NC), (b_post(g - 1), NC))
        ob_copy(g - 1).start()
        return carry

    jax.lax.fori_loop(1, NG, group_step, 0)

    in_wait(NG - 1, WO_IN)
    fence()
    mac = b_mac()
    _merge((a_norm(NG - 1), S // CG), (a_mix(NG - 1), NG), (take(mac, MAC_COST // 12), MAC_COST // 12))
    fence()
    n_out = S // RO
    n_mac = n_out * 5 // 8
    _merge((a_out(0, n_mac), n_mac * NG * NG), (mac, MAC_COST * 11 / 12))
    fence()
    in_wait(NG - 1, Q_IN)
    _merge((b_post(NG - 1), NC), (a_out(n_mac, n_mac + 2), 2 * NG * NG))
    ob_copy(NG - 1).start()
    _merge((a_out(n_mac + 2, n_out), 1))
    for g in range(NG):
        ob_copy(g).wait()
    for i in range(n_out):
        oa_copy(i).wait()


@jax.jit
def pallas_concat_heads__linear_attn_block__ssm_conv_h3__prompt_kernel(
    A_x: jax.Array,
    A_wqkv: jax.Array,
    A_wo: jax.Array,
    B_q: jax.Array,
    B_k: jax.Array,
    B_v: jax.Array,
    B_shift_k: jax.Array,
    B_ssm_k: jax.Array,
    B_ssm_D: jax.Array,
):
    hbm = pl.BlockSpec(memory_space=pl.ANY)
    vmem = pl.BlockSpec(memory_space=pltpu.VMEM)
    out = pl.pallas_call(
        _kernel,
        out_shape=jax.ShapeDtypeStruct((S, 2 * D), BF16),
        in_specs=[hbm] * 7 + [vmem] * 4,
        out_specs=hbm,
        scratch_shapes=[
            pltpu.VMEM((S, D), BF16),
            pltpu.VMEM((NG, S, CG), BF16),
            pltpu.VMEM((NG, 3, D, CG), BF16),
            pltpu.VMEM((NG, CG, D), BF16),
            pltpu.VMEM((NG, S, CG), BF16),
            pltpu.VMEM((NG, S, CG), BF16),
            pltpu.VMEM((NG, S, CG), BF16),
            pltpu.VMEM((NG, CG, S), BF16),
            pltpu.VMEM((NG, KS + 1, 8, CG), F32),
            pltpu.VMEM((S + 8, CG), F32),
            pltpu.VMEM((2, S, CG), BF16),
            pltpu.VMEM((NC, 2 * T, CG), F32),
            pltpu.VMEM((NC, 2 * T, CG), F32),
            pltpu.VMEM((NC, 2 * T, CG), BF16),
            pltpu.VMEM((S, CG), BF16),
            pltpu.VMEM((S, CG), BF16),
            pltpu.VMEM((8, CG), F32),
            pltpu.VMEM((CG, CG), BF16),
            pltpu.VMEM((CG, CG), F32),
            pltpu.VMEM((CG, CG), BF16),
            pltpu.VMEM((NG, S, CG), BF16),
            pltpu.VMEM((NG, D, CG), BF16),
            pltpu.VMEM((NG, S, CG), BF16),
            pltpu.VMEM((S, D), BF16),
            pltpu.SemaphoreType.DMA((len(XB) - 1,)),
            pltpu.SemaphoreType.DMA((NG, 6)),
            pltpu.SemaphoreType.DMA((NG,)),
            pltpu.SemaphoreType.DMA((S // RO,)),
            pltpu.SemaphoreType.REGULAR,
        ],
        compiler_params=pltpu.CompilerParams(vmem_limit_bytes=96 * 1024 * 1024, flags=FLAGS),
    )(A_x.reshape(S, D), A_wqkv, A_wo, B_q.reshape(S, D), B_k.reshape(S, D), B_v.reshape(S, D),
      B_ssm_k, B_shift_k.T, B_ssm_D.reshape(NG, CG), _FWD, _INV)
    return out.reshape(1, S, 2 * D)
```

```python
import jax
import jax.numpy as jnp
import numpy as np
import jax.experimental.pallas as pl
import jax.experimental.pallas.tpu as pltpu

S, D, H = 2048, 1024, 32
DH = D // H
CG = 128
NG = D // CG
T = 128
NC = S // T
KS = 4
NP = NG // 2
HS = S // 2
KH = NG // 2
RA = 64
NB = 2
RP = 32
RO = 512
XB = (0, 256, 512, 1024, 2048)
LAG_KV = 2048
MAC_RATE = 1.0
FLAGS = None
F32, BF16, U32 = jnp.float32, jnp.bfloat16, jnp.uint32


def _dft_matrices():
    k = np.concatenate([np.arange(0, T, 2), np.arange(1, T, 2)])
    ang = np.pi * (2 * k[:, None] + 1) / (2 * T) * np.arange(T)[None, :]
    re = np.cos(ang).reshape(T // 8, 1, 8, T)
    im = -np.sin(ang).reshape(T // 8, 1, 8, T)
    fwd = np.concatenate([re, im], axis=1).reshape(2 * T, T)
    inv = fwd.T / T
    inv = np.stack([inv[:, :T], inv[:, T:]])
    return fwd.astype(BF16), inv.astype(BF16)


_FWD, _INV = _dft_matrices()


def _dot(a, b):
    return jnp.dot(a, b, preferred_element_type=F32)


def _dot_nt(a, b):
    return jax.lax.dot_general(a, b, (((1,), (1,)), ((), ())), preferred_element_type=F32)


def _dot_tn(a, b):
    return jax.lax.dot_general(a, b, (((0,), (0,)), ((), ())), preferred_element_type=F32)


def _phi(t):
    return jnp.where(t > 0, t + 1.0, jnp.exp(t)) + 1e-6


def _ld(ref, lead, r0, n):
    return pltpu.bitcast(ref.bitcast(U32)[lead + (pl.ds(r0 // 2, n // 2), slice(None))], BF16)


def _merge(*streams):
    done = [0.0] * len(streams)
    live = list(range(len(streams)))
    while live:
        i = min(live, key=lambda s: done[s] / streams[s][1])
        cost = next(streams[i][0], None)
        if cost is None:
            live.remove(i)
        else:
            done[i] += cost


def _take(stream, cost):
    while cost > 0:
        c = next(stream, None)
        if c is None:
            return
        cost -= c
        yield c


def _lhs_terms(a11, a12, a21, a22):
    return a11 + a22, a21 + a22, a11, a22, a11 + a12, a21 - a11, a12 - a22


def _rhs_terms(b11, b12, b21, b22):
    return b11 + b22, b11, b12 - b22, b21 - b11, b22, b11 + b12, b21 + b22


def _strassen(lhs, rhs, emit):
    def prod(i, acc=None):
        for kb in range(KH):
            part = _dot(lhs(i, kb), rhs(i, kb))
            acc = part if acc is None else acc + part
        return acc

    m1 = prod(0)
    yield 1
    m2 = prod(1)
    c22 = m1 - m2
    yield 1
    m4 = prod(3)
    emit(1, 0, m2 + m4)
    c11 = m1 + m4
    yield 1
    m3 = prod(2)
    c22 = c22 + m3
    yield 1
    emit(1, 1, prod(5, c22))
    yield 1
    m5 = prod(4)
    emit(0, 1, m3 + m5)
    c11 = c11 - m5
    yield 1
    emit(0, 0, prod(6, c11))
    yield 1


def _kernel(x_hbm, wqkv_hbm, wo_hbm, q_hbm, k_hbm, v_hbm, h_hbm, shk_ref, dd_ref, fwd_ref, inv_ref,
            out_hbm,
            x_buf, xs_buf, w_buf, ws_buf, wo_buf, q_buf, k_buf, v_buf, h_buf, tap_buf, kf_buf, kv_buf,
            xf_buf, hf_buf, yf_buf, pk_buf, pv_buf, z_buf, kvs_buf, zs_buf, kvbd_buf, pq_buf, ps_buf,
            m_buf, ms_buf, ob_buf, oa_buf, x_sem, in_sem, ob_sem, oa_sem, fence_sem):

    def rows_of(i, n):
        return i * n if isinstance(i, int) else pl.multiple_of(i * n, n)

    H_IN, K_IN, V_IN, Q_IN, WO_IN, WQ_IN, WK_IN, WV_IN = range(8)
    W_IN = (WQ_IN, WK_IN, WV_IN)

    def in_copy(g, which):
        if which in W_IN:
            t = which - WQ_IN
            src, dst = wqkv_hbm.at[:, :, pl.ds(rows_of(t * NG + g, CG), CG)], w_buf.at[g, t]
        elif which in (H_IN, WO_IN):
            hbm, buf = (h_hbm, h_buf) if which == H_IN else (wo_hbm, wo_buf)
            src, dst = hbm.at[pl.ds(rows_of(g, CG), CG)], buf.at[g]
        else:
            hbm, buf = {K_IN: (k_hbm, k_buf), V_IN: (v_hbm, v_buf), Q_IN: (q_hbm, q_buf)}[which]
            src, dst = hbm.at[:, pl.ds(rows_of(g, CG), CG)], buf.at[g]
        return pltpu.make_async_copy(src, dst, in_sem.at[g, which])

    def in_start(g, *whiches):
        for which in whiches:
            in_copy(g, which).start()

    def in_wait(g, *whiches):
        for which in whiches:
            in_copy(g, which).wait()

    def x_copy(c):
        rows = pl.ds(XB[c], XB[c + 1] - XB[c])
        return pltpu.make_async_copy(x_hbm.at[rows], x_buf.at[rows], x_sem.at[c])

    def ob_copy(g):
        return pltpu.make_async_copy(ob_buf.at[g], out_hbm.at[:, pl.ds(rows_of(NG + g, CG), CG)], ob_sem.at[g])

    def oa_copy(i):
        rows = pl.ds(i * 2 * RA, 2 * RA)
        return pltpu.make_async_copy(oa_buf.at[rows], out_hbm.at[rows, pl.ds(0, D)], oa_sem.at[i])

    def fence():
        pl.semaphore_signal(fence_sem, 1)
        pl.semaphore_wait(fence_sem, 1)

    def x_terms(r_lo, r_hi):
        for r0 in range(r_lo, r_hi, 2 * RA):
            for kb in range(KH):
                for r in range(0, RA, RP):
                    blocks = [x_buf[pl.ds(r0 + a * RA + r, RP), pl.ds((b * KH + kb) * CG, CG)].astype(F32)
                              for a in range(2) for b in range(2)]
                    for i, term in enumerate(_lhs_terms(*blocks)):
                        xs_buf[r0 // HS, i, kb, pl.ds(r0 % HS // 2 + r, RP), :] = term.astype(BF16)
                    yield 1

    def w_terms(p, tiles, kbs):
        for t in tiles:
            for kb in kbs:
                for r in range(0, CG, RP):
                    blocks = [_ld(w_buf, (2 * p + b, t, a * KH + kb), r, RP).astype(F32)
                              for a in range(2) for b in range(2)]
                    for i, term in enumerate(_rhs_terms(*blocks)):
                        if i not in (1, 4):
                            ws_buf[p % 2, t, i, kb, pl.ds(r, RP), :] = term.astype(BF16)
                    yield 1

    def kv_block(s, j, b):
        kv = _dot_tn(_ld(pk_buf, (j,), b * CG, CG), _ld(pv_buf, (j,), b * CG, CG))
        kvs_buf[s, j] = kv if b == 0 else kvs_buf[s, j] + kv

    def a_main(s, tiles=(0, 1, 2), r_lo=0, r_hi=HS):
        p, half = s // 2, s % 2
        todo = []
        n = 0
        zs = [None, None]
        for r0 in range(r_lo, r_hi, 2 * RA):
            for t in tiles:
                def lhs(i, kb):
                    return _ld(xs_buf, (half, i, kb), r0 // 2, RA)

                def rhs(i, kb):
                    if i == 1:
                        return _ld(w_buf, (2 * p, t, kb), 0, CG)
                    if i == 4:
                        return _ld(w_buf, (2 * p + 1, t, KH + kb), 0, CG)
                    return _ld(ws_buf, (p % 2, t, i, kb), 0, CG)

                def emit(a, j, val):
                    rows = pl.ds(r0 + a * RA, RA)
                    if t == 0:
                        pq_buf[2 * p + j, half, rows, :] = _phi(val).astype(BF16)
                    elif t == 1:
                        pk = _phi(val)
                        z = jnp.sum(pk.reshape(RA // 8, 8, CG), axis=0)
                        zs[j] = z if zs[j] is None else zs[j] + z
                        pk_buf[j, rows, :] = pk.astype(BF16)
                    else:
                        pv_buf[j, rows, :] = val.astype(BF16)

                for _ in _strassen(lhs, rhs, emit):
                    n += KH * RA
                    yield KH * RA
                    if todo and todo[0][0] <= n:
                        kv_block(s, *todo.pop(0)[1:])
                        yield CG
            if 2 in tiles and (r0 + 2 * RA) % CG == 0 and r0 + 2 * RA < HS:
                todo += [(n + LAG_KV, j, (r0 + 2 * RA) // CG - 1) for j in range(2)]
        for _, j, b in todo:
            kv_block(s, j, b)
        if 1 in tiles:
            for j in range(2):
                z_buf[s, j] = zs[j]

    def a_last(s):
        for j in range(2):
            kv_block(s, j, HS // CG - 1)

    def a_heads(g):
        s0, j, slot = g // 2 * 2, g % 2, g % 2
        col_head = jax.lax.broadcasted_iota(jnp.int32, (CG, CG), 1) // DH
        row_head = jax.lax.broadcasted_iota(jnp.int32, (CG, CG), 0) // DH
        kvbd_buf[slot] = jnp.where(row_head == col_head, kvs_buf[s0, j] + kvs_buf[s0 + 1, j], 0.0).astype(BF16)
        z = jnp.sum(z_buf[s0, j] + z_buf[s0 + 1, j], axis=0, keepdims=True)
        sel = (jax.lax.broadcasted_iota(jnp.int32, (8 * CG // DH, CG), 0) // 8
               == jax.lax.broadcasted_iota(jnp.int32, (8 * CG // DH, CG), 1) // DH)
        zs_buf[slot] = jnp.where(sel, z, 0.0).astype(BF16)

    def a_norm(g):
        for half in range(2):
            for r0 in range(0, HS, CG):
                pq = _ld(pq_buf, (g, half), r0, CG)
                den = _dot_nt(_ld(zs_buf, (g % 2,), 0, 8 * CG // DH), pq) + 1e-6
                rcp = pl.reciprocal(den, approx=True)
                rcp = rcp * (2.0 - den * rcp)
                rcp = jnp.concatenate([rcp[8 * (c // DH):8 * (c // DH) + 8] for c in range(0, CG, 8)], axis=0)
                pq_buf[g, half, pl.ds(r0, CG), :] = (pq.astype(F32) * rcp.T).astype(BF16)
                yield 1

    def a_mix(g):
        for n in range(NG):
            m_buf[n, g] = _dot(_ld(kvbd_buf, (g % 2,), 0, CG), wo_buf[g, :, pl.ds(n * CG, CG)]).astype(BF16)
            yield 1

    def m_terms():
        for t in range(KH):
            for kb in range(KH):
                for r in range(0, CG, RP):
                    blocks = [_ld(m_buf, (b * KH + t, a * KH + kb), r, RP).astype(F32)
                              for a in range(2) for b in range(2)]
                    for i, term in enumerate(_rhs_terms(*blocks)):
                        if i not in (1, 4):
                            ms_buf[t, i, kb, pl.ds(r, RP), :] = term.astype(BF16)
                    yield 1

    def p_terms(sec):
        for r0 in range(sec * RO, (sec + 1) * RO, 2 * RA):
            for kb in range(KH):
                for r in range(0, RA, RP):
                    blocks = [_ld(pq_buf, (b * KH + kb, r0 // HS), r0 % HS + a * RA + r, RP).astype(F32)
                              for a in range(2) for b in range(2)]
                    for i, term in enumerate(_lhs_terms(*blocks)):
                        if i not in (2, 3):
                            ps_buf[sec % 2, i, kb, pl.ds(r0 % RO // 2 + r, RP), :] = term.astype(BF16)
                    yield 1

    def a_out(sec):
        for r0 in range(sec * RO, (sec + 1) * RO, 2 * RA):
            for t in range(KH):
                def lhs(i, kb):
                    if i == 2:
                        return _ld(pq_buf, (kb, r0 // HS), r0 % HS, RA)
                    if i == 3:
                        return _ld(pq_buf, (KH + kb, r0 // HS), r0 % HS + RA, RA)
                    return _ld(ps_buf, (sec % 2, i, kb), r0 % RO // 2, RA)

                def rhs(i, kb):
                    if i == 1:
                        return _ld(m_buf, (t, kb), 0, CG)
                    if i == 4:
                        return _ld(m_buf, (KH + t, KH + kb), 0, CG)
                    return _ld(ms_buf, (t, i, kb), 0, CG)

                def emit(a, b, val):
                    oa_buf[pl.ds(r0 + a * RA, RA), pl.ds((b * KH + t) * CG, CG)] = val.astype(BF16)

                yield from _strassen(lhs, rhs, emit)
            oa_copy(r0 // (2 * RA)).start()

    def b_pre(g):
        taps = [jnp.concatenate([tap_buf[g, t]] * (RP // 8), axis=0) for t in range(KS)]
        for r0 in range(0, S, RP):
            kf = _ld(k_buf, (g,), r0, RP).astype(F32)
            kf_buf[pl.ds(8 + r0, RP), :] = kf
            acc = kf * taps[0]
            for t in range(1, KS):
                acc = acc + kf_buf[pl.ds(8 + r0 - t, RP), :] * taps[t]
            kv_buf[g % 2, pl.ds(r0, RP), :] = (acc * _ld(v_buf, (g,), r0, RP).astype(F32)).astype(BF16)
            yield 1

    def b_filter(g):
        for j in range(NC):
            hf_buf[j] = _dot_nt(_ld(fwd_ref, (), 0, 2 * T), h_buf[g, :, pl.ds(j * T, T)])
            yield 1

    def b_signal(g):
        for j in range(NC):
            xf_buf[j] = _dot(_ld(fwd_ref, (), 0, 2 * T), _ld(kv_buf, (g % 2,), j * T, T))
            yield 1

    def b_mac():
        for r in range(T // 8):
            re, im = pl.ds(16 * r, 8), pl.ds(16 * r + 8, 8)
            even = r < T // 16
            prev = None
            for i0 in range(0, NC, NB):
                acc = [None] * NB
                hs = {}
                for j in range(i0 + NB):
                    xr, xi = xf_buf[j, re, :], xf_buf[j, im, :]
                    n = 0
                    for a in range(NB):
                        m = i0 + a - j
                        if m < 0:
                            continue
                        if m not in hs:
                            hs[m] = (hf_buf[m, re, :], hf_buf[m, im, :])
                        hr, hi = hs[m]
                        pr = hr * xr - hi * xi
                        pi = hr * xi + hi * xr
                        acc[a] = (pr, pi) if acc[a] is None else (acc[a][0] + pr, acc[a][1] + pi)
                        n += 1
                    yield n
                for a in range(NB):
                    yr, yi = acc[a]
                    if prev is not None:
                        yr, yi = (yr - prev[1], yi + prev[0]) if even else (yr + prev[1], yi - prev[0])
                    prev = acc[a]
                    yf_buf[i0 + a, pl.ds(16 * r, 16), :] = jnp.concatenate([yr, yi], axis=0).astype(BF16)

    def b_post(g):
        dvec = jnp.concatenate([tap_buf[g, KS]] * (T // 8), axis=0)
        for i in range(NC):
            inv = jnp.concatenate([_ld(inv_ref, (0,), 0, T), _ld(inv_ref, (1,), 0, T)], axis=1)
            y = _dot(inv, _ld(yf_buf, (i,), 0, 2 * T)) + _ld(kv_buf, (g % 2,), i * T, T).astype(F32) * dvec
            ob_buf[g, pl.ds(i * T, T), :] = (_ld(q_buf, (g,), i * T, T).astype(F32) * y).astype(BF16)
            yield 1

    TILE_COST = 7 * KH * HS // 2
    MAIN_COST = 3 * TILE_COST + 2 * HS
    MAC_COST = (T // 8) * NC * (NC + 1) // 2
    PRE_COST = S // RP
    NORM_COST = S // CG
    KB_COST = CG // RP
    all_kb = range(KH)

    x_copy(0).start()
    in_start(0, WQ_IN)
    in_start(1, WQ_IN)
    x_copy(0).wait()
    x_copy(1).start()
    _merge((x_terms(XB[0], XB[1]), 1))
    in_wait(0, WQ_IN)
    in_wait(1, WQ_IN)
    x_copy(2).start()
    _merge((w_terms(0, (0,), all_kb), 1))
    x_copy(1).wait()
    fence()
    _merge((a_main(0, (0,), XB[0], XB[1]), 7 * KH * (XB[1] - XB[0]) // 2),
           (x_terms(XB[1], XB[2]), (XB[2] - XB[1]) * KH / (2 * RP)))
    in_start(0, WK_IN, WV_IN)
    in_start(1, WK_IN, WV_IN)
    x_copy(2).wait()
    fence()
    _merge((a_main(0, (0,), XB[1], XB[2]), 7 * KH * (XB[2] - XB[1]) // 2),
           (x_terms(XB[2], XB[3]), (XB[3] - XB[2]) * KH / (2 * RP)))
    x_copy(3).start()
    in_wait(0, WK_IN, WV_IN)
    in_wait(1, WK_IN, WV_IN)
    fence()
    _merge((a_main(0, (0,), XB[2], XB[3]), 7 * KH * (XB[3] - XB[2]) // 2),
           (w_terms(0, (1, 2), all_kb), 2 * KH * KB_COST))
    in_start(0, K_IN, V_IN, H_IN)
    kf_buf[0:8, :] = jnp.zeros((8, CG), F32)
    shk = shk_ref[...].astype(F32)
    dd = dd_ref[...].astype(F32)
    for g in range(NG):
        for t in range(KS):
            tap_buf[g, t] = jnp.broadcast_to(shk[t:t + 1, g * CG:(g + 1) * CG], (8, CG))
        tap_buf[g, KS] = jnp.broadcast_to(dd[g:g + 1, :], (8, CG))
    fence()
    kv0 = a_main(0, (1, 2))
    _merge((_take(kv0, TILE_COST), 1))
    x_copy(3).wait()
    in_start(1, K_IN, V_IN)
    in_start(2, *W_IN)
    fence()
    _merge((kv0, TILE_COST + 2 * HS), (x_terms(HS, S), HS * KH / (2 * RP)))
    in_wait(0, K_IN, V_IN, H_IN)
    in_start(3, *W_IN)
    fence()
    a_last(0)
    _merge((b_filter(0), NC), (b_pre(0), PRE_COST))
    fence()
    _merge((b_signal(0), NC))

    def step(s, first=False):
        in_start(s, H_IN)
        in_start(s - 1, Q_IN, WO_IN)
        if first:
            in_start(s + 1, K_IN, V_IN)
        else:
            @pl.when(s + 1 < NG)
            def _():
                in_start(s + 1, K_IN, V_IN)

            in_wait(s - 2, WO_IN)
        in_wait(s, K_IN, V_IN)
        fence()
        streams = [(a_main(s), MAIN_COST), (b_mac(), MAC_RATE * MAC_COST), (b_pre(s), PRE_COST)]
        if not first:
            streams += [(a_norm(s - 2), NORM_COST), (a_mix(s - 2), NG)]
        _merge(*streams)
        in_wait(s, H_IN)
        in_wait(s - 1, Q_IN)
        if first:
            in_wait(2, *W_IN)
            in_wait(3, *W_IN)
            in_start(4, *W_IN)
            in_start(5, *W_IN)
            terms = (w_terms(1, range(3), all_kb), 3 * KH * KB_COST)
        else:
            @pl.when(jnp.logical_and(s % 2 == 0, s + 2 < NG))
            def _():
                in_wait(s + 2, *W_IN)
                in_wait(s + 3, *W_IN)

            @pl.when(jnp.logical_and(s % 2 == 1, s + 3 < NG))
            def _():
                in_start(s + 3, *W_IN)
                in_start(s + 4, *W_IN)

            kbs = [s % 2 * (KH // 2) + i for i in range(KH // 2)]
            terms = (w_terms((s // 2 + 1) % NP, range(3), kbs), 3 * KH // 2 * KB_COST)
        fence()
        a_last(s)
        a_heads(s - 1)
        _merge((b_filter(s), NC), (b_signal(s), NC), (b_post(s - 1), NC), terms)
        ob_copy(s - 1).start()

    step(1, first=True)

    def loop_body(s, carry):
        step(s)
        return carry

    jax.lax.fori_loop(2, NG, loop_body, 0)

    in_start(NG - 1, Q_IN, WO_IN)
    in_wait(NG - 2, WO_IN)
    a_heads(NG - 1)
    mac = b_mac()
    fence()
    _merge((a_norm(NG - 2), NORM_COST), (a_mix(NG - 2), NG), (a_norm(NG - 1), NORM_COST))
    in_wait(NG - 1, WO_IN)
    _merge((a_mix(NG - 1), NG))
    fence()
    _merge((m_terms(), KH * KH * KB_COST), (p_terms(0), RO * KH / (2 * RP)))
    n_sec = S // RO
    for sec in range(n_sec):
        fence()
        streams = [(a_out(sec), RO // (2 * RA) * KH * 7)]
        if sec + 1 < n_sec:
            streams += [(p_terms(sec + 1), RO * KH / (2 * RP)),
                        (_take(mac, MAC_COST / (n_sec - 1) + 1), MAC_COST / (n_sec - 1))]
            _merge(*streams)
            if sec + 2 == n_sec:
                _merge((mac, 1))
                in_wait(NG - 1, Q_IN)
        else:
            _merge((b_post(NG - 1), NC), (_take(streams[0][0], streams[0][1] // 2), streams[0][1] // 2))
            ob_copy(NG - 1).start()
            _merge(streams[0])
    for g in range(NG):
        ob_copy(g).wait()
    for i in range(S // (2 * RA)):
        oa_copy(i).wait()


@jax.jit
def pallas_concat_heads__linear_attn_block__ssm_conv_h3__prompt_kernel(
    A_x: jax.Array,
    A_wqkv: jax.Array,
    A_wo: jax.Array,
    B_q: jax.Array,
    B_k: jax.Array,
    B_v: jax.Array,
    B_shift_k: jax.Array,
    B_ssm_k: jax.Array,
    B_ssm_D: jax.Array,
):
    hbm = pl.BlockSpec(memory_space=pl.ANY)
    vmem = pl.BlockSpec(memory_space=pltpu.VMEM)
    out = pl.pallas_call(
        _kernel,
        out_shape=jax.ShapeDtypeStruct((S, 2 * D), BF16),
        in_specs=[hbm] * 7 + [vmem] * 4,
        out_specs=hbm,
        scratch_shapes=[
            pltpu.VMEM((S, D), BF16),
            pltpu.VMEM((2, 7, KH, HS // 2, CG), BF16),
            pltpu.VMEM((NG, 3, NG, CG, CG), BF16),
            pltpu.VMEM((2, 3, 7, KH, CG, CG), BF16),
            pltpu.VMEM((NG, CG, D), BF16),
            pltpu.VMEM((NG, S, CG), BF16),
            pltpu.VMEM((NG, S, CG), BF16),
            pltpu.VMEM((NG, S, CG), BF16),
            pltpu.VMEM((NG, CG, S), BF16),
            pltpu.VMEM((NG, KS + 1, 8, CG), F32),
            pltpu.VMEM((S + 8, CG), F32),
            pltpu.VMEM((2, S, CG), BF16),
            pltpu.VMEM((NC, 2 * T, CG), F32),
            pltpu.VMEM((NC, 2 * T, CG), F32),
            pltpu.VMEM((NC, 2 * T, CG), BF16),
            pltpu.VMEM((2, HS, CG), BF16),
            pltpu.VMEM((2, HS, CG), BF16),
            pltpu.VMEM((NG, 2, 8, CG), F32),
            pltpu.VMEM((NG, 2, CG, CG), F32),
            pltpu.VMEM((2, 8 * CG // DH, CG), BF16),
            pltpu.VMEM((2, CG, CG), BF16),
            pltpu.VMEM((NG, 2, HS, CG), BF16),
            pltpu.VMEM((2, 7, KH, RO // 2, CG), BF16),
            pltpu.VMEM((NG, NG, CG, CG), BF16),
            pltpu.VMEM((KH, 7, KH, CG, CG), BF16),
            pltpu.VMEM((NG, S, CG), BF16),
            pltpu.VMEM((S, D), BF16),
            pltpu.SemaphoreType.DMA((len(XB) - 1,)),
            pltpu.SemaphoreType.DMA((NG, 8)),
            pltpu.SemaphoreType.DMA((NG,)),
            pltpu.SemaphoreType.DMA((S // (2 * RA),)),
            pltpu.SemaphoreType.REGULAR,
        ],
        compiler_params=pltpu.CompilerParams(vmem_limit_bytes=100 * 1024 * 1024, flags=FLAGS),
    )(A_x.reshape(S, D), A_wqkv.reshape(NG, CG, 3 * D), A_wo, B_q.reshape(S, D), B_k.reshape(S, D),
      B_v.reshape(S, D), B_ssm_k, B_shift_k.T, B_ssm_D.reshape(NG, CG), _FWD, _INV)
    return out.reshape(1, S, 2 * D)
```

```python
import jax
import jax.numpy as jnp
import numpy as np
import jax.experimental.pallas as pl
import jax.experimental.pallas.tpu as pltpu

S, D, H = 2048, 1024, 32
DH = D // H
CG = 128
NG = D // CG
T = 128
NC = S // T
KS = 4
NP = NG // 2
HS = S // 2
KH = NG // 2
RA = 64
NB = 2
RP = 32
RO = 512
XB = (0, 256, 512, 1024, 2048)
LAG_KV = 2048
MAC_RATE = 1.0
FLAGS = None
F32, BF16, U32 = jnp.float32, jnp.bfloat16, jnp.uint32


def _dft_matrices():
    k = np.concatenate([np.arange(0, T, 2), np.arange(1, T, 2)])
    ang = np.pi * (2 * k[:, None] + 1) / (2 * T) * np.arange(T)[None, :]
    re = np.cos(ang).reshape(T // 8, 1, 8, T)
    im = -np.sin(ang).reshape(T // 8, 1, 8, T)
    fwd = np.concatenate([re, im], axis=1).reshape(2 * T, T)
    inv = fwd.T / T
    inv = np.stack([inv[:, :T], inv[:, T:]])
    return fwd.astype(BF16), inv.astype(BF16)


_FWD, _INV = _dft_matrices()


def _dot(a, b):
    return jnp.dot(a, b, preferred_element_type=F32)


def _dot_nt(a, b):
    return jax.lax.dot_general(a, b, (((1,), (1,)), ((), ())), preferred_element_type=F32)


def _dot_tn(a, b):
    return jax.lax.dot_general(a, b, (((0,), (0,)), ((), ())), preferred_element_type=F32)


def _phi(t):
    return jnp.where(t > 0, t + 1.0, jnp.exp(t)) + 1e-6


def _ld(ref, lead, r0, n):
    return pltpu.bitcast(ref.bitcast(U32)[lead + (pl.ds(r0 // 2, n // 2), slice(None))], BF16)


def _merge(*streams):
    done = [0.0] * len(streams)
    live = list(range(len(streams)))
    while live:
        i = min(live, key=lambda s: done[s] / streams[s][1])
        cost = next(streams[i][0], None)
        if cost is None:
            live.remove(i)
        else:
            done[i] += cost


def _take(stream, cost):
    while cost > 0:
        c = next(stream, None)
        if c is None:
            return
        cost -= c
        yield c


def _lhs_terms(a11, a12, a21, a22):
    return a11 + a22, a21 + a22, a11, a22, a11 + a12, a21 - a11, a12 - a22


def _rhs_terms(b11, b12, b21, b22):
    return b11 + b22, b11, b12 - b22, b21 - b11, b22, b11 + b12, b21 + b22


def _strassen(lhs, rhs, emit):
    def prod(i, acc=None):
        for kb in range(KH):
            part = _dot(lhs(i, kb), rhs(i, kb))
            acc = part if acc is None else acc + part
        return acc

    m1 = prod(0)
    yield 1
    m2 = prod(1)
    c22 = m1 - m2
    yield 1
    m4 = prod(3)
    emit(1, 0, m2 + m4)
    c11 = m1 + m4
    yield 1
    m3 = prod(2)
    c22 = c22 + m3
    yield 1
    emit(1, 1, prod(5, c22))
    yield 1
    m5 = prod(4)
    emit(0, 1, m3 + m5)
    c11 = c11 - m5
    yield 1
    emit(0, 0, prod(6, c11))
    yield 1


def _kernel(x_hbm, wqkv_hbm, wo_hbm, q_hbm, k_hbm, v_hbm, h_hbm, shk_ref, dd_ref, fwd_ref, inv_ref,
            out_hbm,
            x_buf, xs_buf, w_buf, ws_buf, wo_buf, q_buf, k_buf, v_buf, h_buf, tap_buf, kf_buf, kv_buf,
            xf_buf, hf_buf, yf_buf, pk_buf, pv_buf, z_buf, kvs_buf, zs_buf, kvbd_buf, pq_buf, ps_buf,
            m_buf, ms_buf, ob_buf, oa_buf, x_sem, in_sem, ob_sem, oa_sem, fence_sem):

    def rows_of(i, n):
        return i * n if isinstance(i, int) else pl.multiple_of(i * n, n)

    H_IN, K_IN, V_IN, Q_IN, WO_IN, WQ_IN, WK_IN, WV_IN = range(8)
    W_IN = (WQ_IN, WK_IN, WV_IN)

    def in_copy(g, which):
        if which in W_IN:
            t = which - WQ_IN
            src, dst = wqkv_hbm.at[:, :, pl.ds(rows_of(t * NG + g, CG), CG)], w_buf.at[g, t]
        elif which in (H_IN, WO_IN):
            hbm, buf = (h_hbm, h_buf) if which == H_IN else (wo_hbm, wo_buf)
            src, dst = hbm.at[pl.ds(rows_of(g, CG), CG)], buf.at[g]
        else:
            hbm, buf = {K_IN: (k_hbm, k_buf), V_IN: (v_hbm, v_buf), Q_IN: (q_hbm, q_buf)}[which]
            src, dst = hbm.at[:, pl.ds(rows_of(g, CG), CG)], buf.at[g]
        return pltpu.make_async_copy(src, dst, in_sem.at[g, which])

    def in_start(g, *whiches):
        for which in whiches:
            in_copy(g, which).start()

    def in_wait(g, *whiches):
        for which in whiches:
            in_copy(g, which).wait()

    def x_copy(c):
        rows = pl.ds(XB[c], XB[c + 1] - XB[c])
        return pltpu.make_async_copy(x_hbm.at[rows], x_buf.at[rows], x_sem.at[c])

    def ob_copy(g):
        return pltpu.make_async_copy(ob_buf.at[g], out_hbm.at[:, pl.ds(rows_of(NG + g, CG), CG)], ob_sem.at[g])

    def oa_copy(i):
        rows = pl.ds(i * 2 * RA, 2 * RA)
        return pltpu.make_async_copy(oa_buf.at[rows], out_hbm.at[rows, pl.ds(0, D)], oa_sem.at[i])

    def fence():
        pl.semaphore_signal(fence_sem, 1)
        pl.semaphore_wait(fence_sem, 1)

    def x_terms(r_lo, r_hi):
        for r0 in range(r_lo, r_hi, 2 * RA):
            for kb in range(KH):
                for r in range(0, RA, RP):
                    blocks = [x_buf[pl.ds(r0 + a * RA + r, RP), pl.ds((b * KH + kb) * CG, CG)].astype(F32)
                              for a in range(2) for b in range(2)]
                    for i, term in enumerate(_lhs_terms(*blocks)):
                        xs_buf[r0 // HS, i, kb, pl.ds(r0 % HS // 2 + r, RP), :] = term.astype(BF16)
                    yield 1

    def w_terms(p, tiles, kbs):
        for t in tiles:
            for kb in kbs:
                for r in range(0, CG, RP):
                    blocks = [_ld(w_buf, (2 * p + b, t, a * KH + kb), r, RP).astype(F32)
                              for a in range(2) for b in range(2)]
                    for i, term in enumerate(_rhs_terms(*blocks)):
                        if i not in (1, 4):
                            ws_buf[p % 2, t, i, kb, pl.ds(r, RP), :] = term.astype(BF16)
                    yield 1

    def kv_block(s, j, b):
        kv = _dot_tn(_ld(pk_buf, (j,), b * CG, CG), _ld(pv_buf, (j,), b * CG, CG))
        kvs_buf[s, j] = kv if b == 0 else kvs_buf[s, j] + kv

    def a_main(s, tiles=(0, 1, 2), r_lo=0, r_hi=HS, state=None):
        p, half = s // 2, s % 2
        state = state or {"todo": [], "n": 0, "zs": [None, None]}
        todo, zs = state["todo"], state["zs"]
        for r0 in range(r_lo, r_hi, 2 * RA):
            for t in tiles:
                def lhs(i, kb):
                    return _ld(xs_buf, (half, i, kb), r0 // 2, RA)

                def rhs(i, kb):
                    if i == 1:
                        return _ld(w_buf, (2 * p, t, kb), 0, CG)
                    if i == 4:
                        return _ld(w_buf, (2 * p + 1, t, KH + kb), 0, CG)
                    return _ld(ws_buf, (p % 2, t, i, kb), 0, CG)

                def emit(a, j, val):
                    rows = pl.ds(r0 + a * RA, RA)
                    if t == 0:
                        pq_buf[2 * p + j, half, rows, :] = _phi(val).astype(BF16)
                    elif t == 1:
                        pk = _phi(val)
                        z = jnp.sum(pk.reshape(RA // 8, 8, CG), axis=0)
                        zs[j] = z if zs[j] is None else zs[j] + z
                        pk_buf[j, rows, :] = pk.astype(BF16)
                    else:
                        pv_buf[j, rows, :] = val.astype(BF16)

                for _ in _strassen(lhs, rhs, emit):
                    state["n"] += KH * RA
                    yield KH * RA
                    if todo and todo[0][0] <= state["n"]:
                        kv_block(s, *todo.pop(0)[1:])
                        yield CG
            if 2 in tiles and (r0 + 2 * RA) % CG == 0 and r0 + 2 * RA < HS:
                todo += [(state["n"] + LAG_KV, j, (r0 + 2 * RA) // CG - 1) for j in range(2)]
        if r_hi == HS:
            for _, j, b in todo:
                kv_block(s, j, b)
            for j in range(2):
                z_buf[s, j] = zs[j]

    def a_last(s):
        for j in range(2):
            kv_block(s, j, HS // CG - 1)

    def a_heads(g):
        s0, j, slot = g // 2 * 2, g % 2, g % 2
        col_head = jax.lax.broadcasted_iota(jnp.int32, (CG, CG), 1) // DH
        row_head = jax.lax.broadcasted_iota(jnp.int32, (CG, CG), 0) // DH
        kvbd_buf[slot] = jnp.where(row_head == col_head, kvs_buf[s0, j] + kvs_buf[s0 + 1, j], 0.0).astype(BF16)
        z = jnp.sum(z_buf[s0, j] + z_buf[s0 + 1, j], axis=0, keepdims=True)
        sel = (jax.lax.broadcasted_iota(jnp.int32, (8 * CG // DH, CG), 0) // 8
               == jax.lax.broadcasted_iota(jnp.int32, (8 * CG // DH, CG), 1) // DH)
        zs_buf[slot] = jnp.where(sel, z, 0.0).astype(BF16)

    def a_norm(g):
        for half in range(2):
            for r0 in range(0, HS, CG):
                pq = _ld(pq_buf, (g, half), r0, CG)
                den = _dot_nt(_ld(zs_buf, (g % 2,), 0, 8 * CG // DH), pq) + 1e-6
                rcp = pl.reciprocal(den, approx=True)
                rcp = rcp * (2.0 - den * rcp)
                rcp = jnp.concatenate([rcp[8 * (c // DH):8 * (c // DH) + 8] for c in range(0, CG, 8)], axis=0)
                pq_buf[g, half, pl.ds(r0, CG), :] = (pq.astype(F32) * rcp.T).astype(BF16)
                yield 1

    def a_mix(g):
        for n in range(NG):
            m_buf[n, g] = _dot(_ld(kvbd_buf, (g % 2,), 0, CG), wo_buf[g, :, pl.ds(n * CG, CG)]).astype(BF16)
            yield 1

    def m_terms():
        for t in range(KH):
            for kb in range(KH):
                for r in range(0, CG, RP):
                    blocks = [_ld(m_buf, (b * KH + t, a * KH + kb), r, RP).astype(F32)
                              for a in range(2) for b in range(2)]
                    for i, term in enumerate(_rhs_terms(*blocks)):
                        if i not in (1, 4):
                            ms_buf[t, i, kb, pl.ds(r, RP), :] = term.astype(BF16)
                    yield 1

    def p_terms(sec):
        for r0 in range(sec * RO, (sec + 1) * RO, 2 * RA):
            for kb in range(KH):
                for r in range(0, RA, RP):
                    blocks = [_ld(pq_buf, (b * KH + kb, r0 // HS), r0 % HS + a * RA + r, RP).astype(F32)
                              for a in range(2) for b in range(2)]
                    for i, term in enumerate(_lhs_terms(*blocks)):
                        if i not in (2, 3):
                            ps_buf[sec % 2, i, kb, pl.ds(r0 % RO // 2 + r, RP), :] = term.astype(BF16)
                    yield 1

    def a_out(sec):
        for r0 in range(sec * RO, (sec + 1) * RO, 2 * RA):
            for t in range(KH):
                def lhs(i, kb):
                    if i == 2:
                        return _ld(pq_buf, (kb, r0 // HS), r0 % HS, RA)
                    if i == 3:
                        return _ld(pq_buf, (KH + kb, r0 // HS), r0 % HS + RA, RA)
                    return _ld(ps_buf, (sec % 2, i, kb), r0 % RO // 2, RA)

                def rhs(i, kb):
                    if i == 1:
                        return _ld(m_buf, (t, kb), 0, CG)
                    if i == 4:
                        return _ld(m_buf, (KH + t, KH + kb), 0, CG)
                    return _ld(ms_buf, (t, i, kb), 0, CG)

                def emit(a, b, val):
                    oa_buf[pl.ds(r0 + a * RA, RA), pl.ds((b * KH + t) * CG, CG)] = val.astype(BF16)

                yield from _strassen(lhs, rhs, emit)
            oa_copy(r0 // (2 * RA)).start()

    def b_pre(g):
        taps = [jnp.concatenate([tap_buf[g, t]] * (RP // 8), axis=0) for t in range(KS)]
        for r0 in range(0, S, RP):
            kf = _ld(k_buf, (g,), r0, RP).astype(F32)
            kf_buf[pl.ds(8 + r0, RP), :] = kf
            acc = kf * taps[0]
            for t in range(1, KS):
                acc = acc + kf_buf[pl.ds(8 + r0 - t, RP), :] * taps[t]
            kv_buf[g, pl.ds(r0, RP), :] = (acc * _ld(v_buf, (g,), r0, RP).astype(F32)).astype(BF16)
            yield 1

    def b_filter(g):
        for j in range(NC):
            hf_buf[j] = _dot_nt(_ld(fwd_ref, (), 0, 2 * T), h_buf[g, :, pl.ds(j * T, T)])
            yield 1

    def b_signal(g):
        for j in range(NC):
            xf_buf[j] = _dot(_ld(fwd_ref, (), 0, 2 * T), _ld(kv_buf, (g,), j * T, T))
            yield 1

    def b_mac():
        for r in range(T // 8):
            re, im = pl.ds(16 * r, 8), pl.ds(16 * r + 8, 8)
            even = r < T // 16
            prev = None
            for i0 in range(0, NC, NB):
                acc = [None] * NB
                hs = {}
                for j in range(i0 + NB):
                    xr, xi = xf_buf[j, re, :], xf_buf[j, im, :]
                    n = 0
                    for a in range(NB):
                        m = i0 + a - j
                        if m < 0:
                            continue
                        if m not in hs:
                            hs[m] = (hf_buf[m, re, :], hf_buf[m, im, :])
                        hr, hi = hs[m]
                        pr = hr * xr - hi * xi
                        pi = hr * xi + hi * xr
                        acc[a] = (pr, pi) if acc[a] is None else (acc[a][0] + pr, acc[a][1] + pi)
                        n += 1
                    yield n
                for a in range(NB):
                    yr, yi = acc[a]
                    if prev is not None:
                        yr, yi = (yr - prev[1], yi + prev[0]) if even else (yr + prev[1], yi - prev[0])
                    prev = acc[a]
                    yf_buf[i0 + a, pl.ds(16 * r, 16), :] = jnp.concatenate([yr, yi], axis=0).astype(BF16)

    def b_post(g):
        dvec = jnp.concatenate([tap_buf[g, KS]] * (T // 8), axis=0)
        for i in range(NC):
            inv = jnp.concatenate([_ld(inv_ref, (0,), 0, T), _ld(inv_ref, (1,), 0, T)], axis=1)
            y = _dot(inv, _ld(yf_buf, (i,), 0, 2 * T)) + _ld(kv_buf, (g,), i * T, T).astype(F32) * dvec
            ob_buf[g, pl.ds(i * T, T), :] = (_ld(q_buf, (g,), i * T, T).astype(F32) * y).astype(BF16)
            yield 1

    TILE_COST = 7 * KH * HS // 2
    MAIN_COST = 3 * TILE_COST + 2 * HS
    MAC_COST = (T // 8) * NC * (NC + 1) // 2
    PRE_COST = S // RP
    NORM_COST = S // CG
    KB_COST = CG // RP
    all_kb = range(KH)

    def rows_cost(c, n_tiles):
        return n_tiles * 7 * KH * (XB[c + 1] - XB[c]) // 2

    def x_cost(c):
        return (XB[c + 1] - XB[c]) * KH / (2 * RP)

    state = {"todo": [], "n": 0, "zs": [None, None]}
    x_copy(0).start()
    in_start(0, WQ_IN)
    in_start(1, WQ_IN)
    x_copy(0).wait()
    in_start(0, WK_IN, WV_IN)
    in_start(1, WK_IN, WV_IN)
    _merge((x_terms(XB[0], XB[1]), 1))
    in_wait(0, WQ_IN)
    in_wait(1, WQ_IN)
    _merge((w_terms(0, (0,), all_kb), 1))
    fence()
    x_copy(1).start()
    _merge((a_main(0, (0,), XB[0], XB[1], state), 1))
    in_wait(0, WK_IN, WV_IN)
    in_wait(1, WK_IN, WV_IN)
    x_copy(2).start()
    fence()
    _merge((w_terms(0, (1,), all_kb), 1))
    fence()
    _merge((a_main(0, (1,), XB[0], XB[1], state), rows_cost(0, 1)), (w_terms(0, (2,), all_kb), KH * KB_COST))
    x_copy(1).wait()
    fence()
    _merge((a_main(0, (2,), XB[0], XB[1], state), rows_cost(0, 1)), (x_terms(XB[1], XB[2]), x_cost(1)))
    x_copy(3).start()
    x_copy(2).wait()
    fence()
    _merge((a_main(0, (0, 1, 2), XB[1], XB[2], state), rows_cost(1, 3)), (x_terms(XB[2], XB[3]), x_cost(2)))
    in_start(0, K_IN, V_IN, H_IN)
    x_copy(3).wait()
    fence()
    _merge((a_main(0, (0, 1, 2), XB[2], XB[3], state), rows_cost(2, 3)), (x_terms(XB[3], XB[4]), x_cost(3)))
    in_start(1, K_IN, V_IN)
    kf_buf[0:8, :] = jnp.zeros((8, CG), F32)
    shk = shk_ref[...].astype(F32)
    dd = dd_ref[...].astype(F32)
    for g in range(NG):
        for t in range(KS):
            tap_buf[g, t] = jnp.broadcast_to(shk[t:t + 1, g * CG:(g + 1) * CG], (8, CG))
        tap_buf[g, KS] = jnp.broadcast_to(dd[g:g + 1, :], (8, CG))
    in_wait(0, K_IN, V_IN, H_IN)
    fence()
    a_last(0)
    _merge((b_filter(0), NC), (b_pre(0), PRE_COST))
    in_start(2, *W_IN)
    in_start(3, *W_IN)
    fence()
    _merge((b_signal(0), NC))

    def step(s, first=False):
        in_start(s, H_IN, Q_IN, WO_IN)
        if first:
            in_start(0, Q_IN, WO_IN)
            in_start(2, K_IN, V_IN)
            in_wait(1, K_IN, V_IN)
        else:
            in_start((s + 1) % NG, K_IN, V_IN)
        fence()
        streams = [(a_main(s), MAIN_COST), (b_mac(), MAC_RATE * MAC_COST)]
        if first:
            streams.append((b_pre(1), PRE_COST))
        _merge(*streams)
        in_wait(s, H_IN)
        in_wait(s - 1, Q_IN)
        in_wait((s + 1) % NG, K_IN, V_IN)
        if first:
            in_wait(2, *W_IN)
            in_wait(3, *W_IN)
            in_start(4, *W_IN)
            in_start(5, *W_IN)
            terms = (w_terms(1, range(3), all_kb), 3 * KH * KB_COST)
        else:
            @pl.when(jnp.logical_and(s % 2 == 0, s + 2 < NG))
            def _():
                in_wait(s + 2, *W_IN)
                in_wait(s + 3, *W_IN)

            @pl.when(jnp.logical_and(s % 2 == 1, s + 3 < NG))
            def _():
                in_start(s + 3, *W_IN)
                in_start(s + 4, *W_IN)

            in_wait(s - 2, WO_IN)
            kbs = [s % 2 * (KH // 2) + i for i in range(KH // 2)]
            terms = (w_terms((s // 2 + 1) % NP, range(3), kbs), 3 * KH // 2 * KB_COST)
        fence()
        a_last(s)
        a_heads(s - 1)
        streams = [(b_filter(s), NC), (b_signal(s), NC), (b_post(s - 1), NC), terms,
                   (b_pre((s + 1) % NG), PRE_COST)]
        if not first:
            streams += [(a_norm(s - 2), NORM_COST), (a_mix(s - 2), NG)]
        _merge(*streams)
        ob_copy(s - 1).start()

    step(1, first=True)

    def loop_body(s, carry):
        step(s)
        return carry

    jax.lax.fori_loop(2, NG, loop_body, 0)

    in_wait(NG - 2, WO_IN)
    in_wait(NG - 1, Q_IN, WO_IN)
    a_heads(NG - 1)
    mac = b_mac()
    fence()
    _merge((a_norm(NG - 2), NORM_COST), (a_mix(NG - 2), NG), (a_norm(NG - 1), NORM_COST), (a_mix(NG - 1), NG))
    fence()
    _merge((m_terms(), KH * KH * KB_COST), (p_terms(0), RO * KH / (2 * RP)))
    n_sec = S // RO
    for sec in range(n_sec):
        fence()
        streams = [(a_out(sec), RO // (2 * RA) * KH * 7)]
        if sec + 1 < n_sec:
            streams += [(p_terms(sec + 1), RO * KH / (2 * RP)),
                        (_take(mac, MAC_COST / (n_sec - 1) + 1), MAC_COST / (n_sec - 1))]
            _merge(*streams)
            if sec + 2 == n_sec:
                _merge((mac, 1))
        else:
            _merge((b_post(NG - 1), NC), (_take(streams[0][0], streams[0][1] // 2), streams[0][1] // 2))
            ob_copy(NG - 1).start()
            _merge(streams[0])
    for g in range(NG):
        ob_copy(g).wait()
    for i in range(S // (2 * RA)):
        oa_copy(i).wait()


@jax.jit
def pallas_concat_heads__linear_attn_block__ssm_conv_h3__prompt_kernel(
    A_x: jax.Array,
    A_wqkv: jax.Array,
    A_wo: jax.Array,
    B_q: jax.Array,
    B_k: jax.Array,
    B_v: jax.Array,
    B_shift_k: jax.Array,
    B_ssm_k: jax.Array,
    B_ssm_D: jax.Array,
):
    hbm = pl.BlockSpec(memory_space=pl.ANY)
    vmem = pl.BlockSpec(memory_space=pltpu.VMEM)
    out = pl.pallas_call(
        _kernel,
        out_shape=jax.ShapeDtypeStruct((S, 2 * D), BF16),
        in_specs=[hbm] * 7 + [vmem] * 4,
        out_specs=hbm,
        scratch_shapes=[
            pltpu.VMEM((S, D), BF16),
            pltpu.VMEM((2, 7, KH, HS // 2, CG), BF16),
            pltpu.VMEM((NG, 3, NG, CG, CG), BF16),
            pltpu.VMEM((2, 3, 7, KH, CG, CG), BF16),
            pltpu.VMEM((NG, CG, D), BF16),
            pltpu.VMEM((NG, S, CG), BF16),
            pltpu.VMEM((NG, S, CG), BF16),
            pltpu.VMEM((NG, S, CG), BF16),
            pltpu.VMEM((NG, CG, S), BF16),
            pltpu.VMEM((NG, KS + 1, 8, CG), F32),
            pltpu.VMEM((S + 8, CG), F32),
            pltpu.VMEM((NG, S, CG), BF16),
            pltpu.VMEM((NC, 2 * T, CG), F32),
            pltpu.VMEM((NC, 2 * T, CG), F32),
            pltpu.VMEM((NC, 2 * T, CG), BF16),
            pltpu.VMEM((2, HS, CG), BF16),
            pltpu.VMEM((2, HS, CG), BF16),
            pltpu.VMEM((NG, 2, 8, CG), F32),
            pltpu.VMEM((NG, 2, CG, CG), F32),
            pltpu.VMEM((2, 8 * CG // DH, CG), BF16),
            pltpu.VMEM((2, CG, CG), BF16),
            pltpu.VMEM((NG, 2, HS, CG), BF16),
            pltpu.VMEM((2, 7, KH, RO // 2, CG), BF16),
            pltpu.VMEM((NG, NG, CG, CG), BF16),
            pltpu.VMEM((KH, 7, KH, CG, CG), BF16),
            pltpu.VMEM((NG, S, CG), BF16),
            pltpu.VMEM((S, D), BF16),
            pltpu.SemaphoreType.DMA((len(XB) - 1,)),
            pltpu.SemaphoreType.DMA((NG, 8)),
            pltpu.SemaphoreType.DMA((NG,)),
            pltpu.SemaphoreType.DMA((S // (2 * RA),)),
            pltpu.SemaphoreType.REGULAR,
        ],
        compiler_params=pltpu.CompilerParams(vmem_limit_bytes=100 * 1024 * 1024, flags=FLAGS),
    )(A_x.reshape(S, D), A_wqkv.reshape(NG, CG, 3 * D), A_wo, B_q.reshape(S, D), B_k.reshape(S, D),
      B_v.reshape(S, D), B_ssm_k, B_shift_k.T, B_ssm_D.reshape(NG, CG), _FWD, _INV)
    return out.reshape(1, S, 2 * D)
```

```python
import jax
import jax.numpy as jnp
import numpy as np
import jax.experimental.pallas as pl
import jax.experimental.pallas.tpu as pltpu

S, D, H = 2048, 1024, 32
DH = D // H
CG = 128
NG = D // CG
T = 128
NC = S // T
KS = 4
NP = NG // 2
HS = S // 2
KH = NG // 2
RA = 64
NB = 2
RP = 32
RO = 512
XB = (0, 256, 512, 1024, 2048)
LAG_KV = 2048
MAC_RATE = 1.0
NORM_SPLIT = 0
MIX_SPLIT = 0
FLAGS = None
F32, BF16, U32 = jnp.float32, jnp.bfloat16, jnp.uint32


def _dft_matrices():
    k = np.concatenate([np.arange(0, T, 2), np.arange(1, T, 2)])
    ang = np.pi * (2 * k[:, None] + 1) / (2 * T) * np.arange(T)[None, :]
    re = np.cos(ang).reshape(T // 8, 1, 8, T)
    im = -np.sin(ang).reshape(T // 8, 1, 8, T)
    fwd = np.concatenate([re, im], axis=1).reshape(2 * T, T)
    inv = fwd.T / T
    inv = np.stack([inv[:, :T], inv[:, T:]])
    return fwd.astype(BF16), inv.astype(BF16)


_FWD, _INV = _dft_matrices()


def _dot(a, b):
    return jnp.dot(a, b, preferred_element_type=F32)


def _dot_nt(a, b):
    return jax.lax.dot_general(a, b, (((1,), (1,)), ((), ())), preferred_element_type=F32)


def _dot_tn(a, b):
    return jax.lax.dot_general(a, b, (((0,), (0,)), ((), ())), preferred_element_type=F32)


def _phi(t):
    return jnp.where(t > 0, t + 1.0, jnp.exp(t)) + 1e-6


def _ld(ref, lead, r0, n):
    return pltpu.bitcast(ref.bitcast(U32)[lead + (pl.ds(r0 // 2, n // 2), slice(None))], BF16)


def _merge(*streams):
    done = [0.0] * len(streams)
    live = list(range(len(streams)))
    while live:
        i = min(live, key=lambda s: done[s] / streams[s][1])
        cost = next(streams[i][0], None)
        if cost is None:
            live.remove(i)
        else:
            done[i] += cost


def _take(stream, cost):
    while cost > 0:
        c = next(stream, None)
        if c is None:
            return
        cost -= c
        yield c


def _lhs_terms(a11, a12, a21, a22):
    return a11 + a22, a21 + a22, a11, a22, a11 + a12, a21 - a11, a12 - a22


def _rhs_terms(b11, b12, b21, b22):
    return b11 + b22, b11, b12 - b22, b21 - b11, b22, b11 + b12, b21 + b22


def _strassen(lhs, rhs, emit):
    def prod(i, acc=None):
        for kb in range(KH):
            part = _dot(lhs(i, kb), rhs(i, kb))
            acc = part if acc is None else acc + part
        return acc

    m1 = prod(0)
    yield 1
    m2 = prod(1)
    c22 = m1 - m2
    yield 1
    m4 = prod(3)
    emit(1, 0, m2 + m4)
    c11 = m1 + m4
    yield 1
    m3 = prod(2)
    c22 = c22 + m3
    yield 1
    emit(1, 1, prod(5, c22))
    yield 1
    m5 = prod(4)
    emit(0, 1, m3 + m5)
    c11 = c11 - m5
    yield 1
    emit(0, 0, prod(6, c11))
    yield 1


def _kernel(x_hbm, wqkv_hbm, wo_hbm, q_hbm, k_hbm, v_hbm, h_hbm, shk_ref, dd_ref, fwd_ref, inv_ref,
            out_hbm,
            x_buf, xs_buf, w_buf, ws_buf, wo_buf, q_buf, k_buf, v_buf, h_buf, tap_buf, kf_buf, kv_buf,
            xf_buf, hf_buf, yf_buf, pk_buf, pv_buf, z_buf, kvs_buf, zs_buf, kvbd_buf, pq_buf, ps_buf,
            m_buf, ms_buf, ob_buf, oa_buf, x_sem, in_sem, ob_sem, oa_sem, fence_sem):

    def rows_of(i, n):
        return i * n if isinstance(i, int) else pl.multiple_of(i * n, n)

    H_IN, K_IN, V_IN, Q_IN, WO_IN, WQ_IN, WK_IN, WV_IN = range(8)
    W_IN = (WQ_IN, WK_IN, WV_IN)

    def in_copy(g, which):
        if which in W_IN:
            t = which - WQ_IN
            src, dst = wqkv_hbm.at[:, :, pl.ds(rows_of(t * NG + g, CG), CG)], w_buf.at[g, t]
        elif which in (H_IN, WO_IN):
            hbm, buf = (h_hbm, h_buf) if which == H_IN else (wo_hbm, wo_buf)
            src, dst = hbm.at[pl.ds(rows_of(g, CG), CG)], buf.at[g]
        else:
            hbm, buf = {K_IN: (k_hbm, k_buf), V_IN: (v_hbm, v_buf), Q_IN: (q_hbm, q_buf)}[which]
            src, dst = hbm.at[:, pl.ds(rows_of(g, CG), CG)], buf.at[g]
        return pltpu.make_async_copy(src, dst, in_sem.at[g, which])

    def in_start(g, *whiches):
        for which in whiches:
            in_copy(g, which).start()

    def in_wait(g, *whiches):
        for which in whiches:
            in_copy(g, which).wait()

    def x_copy(c):
        rows = pl.ds(XB[c], XB[c + 1] - XB[c])
        return pltpu.make_async_copy(x_hbm.at[rows], x_buf.at[rows], x_sem.at[c])

    def ob_copy(g):
        return pltpu.make_async_copy(ob_buf.at[g], out_hbm.at[:, pl.ds(rows_of(NG + g, CG), CG)], ob_sem.at[g])

    def oa_copy(i):
        rows = pl.ds(i * 2 * RA, 2 * RA)
        return pltpu.make_async_copy(oa_buf.at[rows], out_hbm.at[rows, pl.ds(0, D)], oa_sem.at[i])

    def fence():
        pl.semaphore_signal(fence_sem, 1)
        pl.semaphore_wait(fence_sem, 1)

    def x_terms(r_lo, r_hi):
        for r0 in range(r_lo, r_hi, 2 * RA):
            for kb in range(KH):
                for r in range(0, RA, RP):
                    blocks = [x_buf[pl.ds(r0 + a * RA + r, RP), pl.ds((b * KH + kb) * CG, CG)].astype(F32)
                              for a in range(2) for b in range(2)]
                    for i, term in enumerate(_lhs_terms(*blocks)):
                        xs_buf[r0 // HS, i, kb, pl.ds(r0 % HS // 2 + r, RP), :] = term.astype(BF16)
                    yield 1

    def w_terms(p, tiles, kbs):
        for t in tiles:
            for kb in kbs:
                for r in range(0, CG, RP):
                    blocks = [_ld(w_buf, (2 * p + b, t, a * KH + kb), r, RP).astype(F32)
                              for a in range(2) for b in range(2)]
                    for i, term in enumerate(_rhs_terms(*blocks)):
                        if i not in (1, 4):
                            ws_buf[p % 2, t, i, kb, pl.ds(r, RP), :] = term.astype(BF16)
                    yield 1

    def kv_block(s, j, b):
        kv = _dot_tn(_ld(pk_buf, (j,), b * CG, CG), _ld(pv_buf, (j,), b * CG, CG))
        kvs_buf[s, j] = kv if b == 0 else kvs_buf[s, j] + kv

    def a_main(s, tiles=(0, 1, 2), r_lo=0, r_hi=HS, state=None):
        p, half = s // 2, s % 2
        state = state or {"todo": [], "n": 0, "zs": [None, None]}
        todo, zs = state["todo"], state["zs"]
        for r0 in range(r_lo, r_hi, 2 * RA):
            for t in tiles:
                def lhs(i, kb):
                    return _ld(xs_buf, (half, i, kb), r0 // 2, RA)

                def rhs(i, kb):
                    if i == 1:
                        return _ld(w_buf, (2 * p, t, kb), 0, CG)
                    if i == 4:
                        return _ld(w_buf, (2 * p + 1, t, KH + kb), 0, CG)
                    return _ld(ws_buf, (p % 2, t, i, kb), 0, CG)

                def emit(a, j, val):
                    rows = pl.ds(r0 + a * RA, RA)
                    if t == 0:
                        pq_buf[2 * p + j, half, rows, :] = _phi(val).astype(BF16)
                    elif t == 1:
                        pk = _phi(val)
                        z = jnp.sum(pk.reshape(RA // 8, 8, CG), axis=0)
                        zs[j] = z if zs[j] is None else zs[j] + z
                        pk_buf[j, rows, :] = pk.astype(BF16)
                    else:
                        pv_buf[j, rows, :] = val.astype(BF16)

                for _ in _strassen(lhs, rhs, emit):
                    state["n"] += KH * RA
                    yield KH * RA
                    if todo and todo[0][0] <= state["n"]:
                        kv_block(s, *todo.pop(0)[1:])
                        yield CG
            if 2 in tiles and (r0 + 2 * RA) % CG == 0 and r0 + 2 * RA < HS:
                todo += [(state["n"] + LAG_KV, j, (r0 + 2 * RA) // CG - 1) for j in range(2)]
        if r_hi == HS:
            for _, j, b in todo:
                kv_block(s, j, b)
            for j in range(2):
                z_buf[s, j] = zs[j]

    def a_last(s):
        for j in range(2):
            kv_block(s, j, HS // CG - 1)

    def a_heads(g):
        s0, j, slot = g // 2 * 2, g % 2, g % 2
        col_head = jax.lax.broadcasted_iota(jnp.int32, (CG, CG), 1) // DH
        row_head = jax.lax.broadcasted_iota(jnp.int32, (CG, CG), 0) // DH
        kvbd_buf[slot] = jnp.where(row_head == col_head, kvs_buf[s0, j] + kvs_buf[s0 + 1, j], 0.0).astype(BF16)
        z = jnp.sum(z_buf[s0, j] + z_buf[s0 + 1, j], axis=0, keepdims=True)
        sel = (jax.lax.broadcasted_iota(jnp.int32, (8 * CG // DH, CG), 0) // 8
               == jax.lax.broadcasted_iota(jnp.int32, (8 * CG // DH, CG), 1) // DH)
        zs_buf[slot] = jnp.where(sel, z, 0.0).astype(BF16)

    def a_norm(g):
        for half in range(2):
            for r0 in range(0, HS, CG):
                pq = _ld(pq_buf, (g, half), r0, CG)
                den = _dot_nt(_ld(zs_buf, (g % 2,), 0, 8 * CG // DH), pq) + 1e-6
                rcp = pl.reciprocal(den, approx=True)
                rcp = rcp * (2.0 - den * rcp)
                rcp = jnp.concatenate([rcp[8 * (c // DH):8 * (c // DH) + 8] for c in range(0, CG, 8)], axis=0)
                pq_buf[g, half, pl.ds(r0, CG), :] = (pq.astype(F32) * rcp.T).astype(BF16)
                yield 1

    def a_mix(g):
        for n in range(NG):
            m_buf[n, g] = _dot(_ld(kvbd_buf, (g % 2,), 0, CG), wo_buf[g, :, pl.ds(n * CG, CG)]).astype(BF16)
            yield 1

    def m_terms():
        for t in range(KH):
            for kb in range(KH):
                for r in range(0, CG, RP):
                    blocks = [_ld(m_buf, (b * KH + t, a * KH + kb), r, RP).astype(F32)
                              for a in range(2) for b in range(2)]
                    for i, term in enumerate(_rhs_terms(*blocks)):
                        if i not in (1, 4):
                            ms_buf[t, i, kb, pl.ds(r, RP), :] = term.astype(BF16)
                    yield 1

    def p_terms(sec):
        for r0 in range(max(sec * RO, 2 * RA), (sec + 1) * RO, 2 * RA):
            for kb in range(KH):
                for r in range(0, RA, RP):
                    blocks = [_ld(pq_buf, (b * KH + kb, r0 // HS), r0 % HS + a * RA + r, RP).astype(F32)
                              for a in range(2) for b in range(2)]
                    for i, term in enumerate(_lhs_terms(*blocks)):
                        if i not in (2, 3):
                            ps_buf[sec % 2, i, kb, pl.ds(r0 % RO // 2 + r, RP), :] = term.astype(BF16)
                    yield 1

    def a_out_plain():
        for n in range(NG):
            acc = None
            for g in range(NG):
                part = _dot(_ld(pq_buf, (g, 0), 0, 2 * RA), _ld(m_buf, (n, g), 0, CG))
                acc = part if acc is None else acc + part
                yield 1
            oa_buf[pl.ds(0, 2 * RA), pl.ds(n * CG, CG)] = acc.astype(BF16)
        oa_copy(0).start()

    def a_out(sec):
        for r0 in range(max(sec * RO, 2 * RA), (sec + 1) * RO, 2 * RA):
            for t in range(KH):
                def lhs(i, kb):
                    if i == 2:
                        return _ld(pq_buf, (kb, r0 // HS), r0 % HS, RA)
                    if i == 3:
                        return _ld(pq_buf, (KH + kb, r0 // HS), r0 % HS + RA, RA)
                    return _ld(ps_buf, (sec % 2, i, kb), r0 % RO // 2, RA)

                def rhs(i, kb):
                    if i == 1:
                        return _ld(m_buf, (t, kb), 0, CG)
                    if i == 4:
                        return _ld(m_buf, (KH + t, KH + kb), 0, CG)
                    return _ld(ms_buf, (t, i, kb), 0, CG)

                def emit(a, b, val):
                    oa_buf[pl.ds(r0 + a * RA, RA), pl.ds((b * KH + t) * CG, CG)] = val.astype(BF16)

                yield from _strassen(lhs, rhs, emit)
            oa_copy(r0 // (2 * RA)).start()

    def b_pre(g):
        taps = [jnp.concatenate([tap_buf[g, t]] * (RP // 8), axis=0) for t in range(KS)]
        for r0 in range(0, S, RP):
            kf = _ld(k_buf, (g,), r0, RP).astype(F32)
            kf_buf[pl.ds(8 + r0, RP), :] = kf
            acc = kf * taps[0]
            for t in range(1, KS):
                acc = acc + kf_buf[pl.ds(8 + r0 - t, RP), :] * taps[t]
            kv_buf[g % 2, pl.ds(r0, RP), :] = (acc * _ld(v_buf, (g,), r0, RP).astype(F32)).astype(BF16)
            yield 1

    def b_filter(g):
        for j in range(NC):
            hf_buf[j] = _dot_nt(_ld(fwd_ref, (), 0, 2 * T), h_buf[g, :, pl.ds(j * T, T)])
            yield 1

    def b_signal(g):
        for j in range(NC):
            xf_buf[j] = _dot(_ld(fwd_ref, (), 0, 2 * T), _ld(kv_buf, (g % 2,), j * T, T))
            yield 1

    def b_mac():
        for r in range(T // 8):
            re, im = pl.ds(16 * r, 8), pl.ds(16 * r + 8, 8)
            even = r < T // 16
            prev = None
            for i0 in range(0, NC, NB):
                acc = [None] * NB
                hs = {}
                for j in range(i0 + NB):
                    xr, xi = xf_buf[j, re, :], xf_buf[j, im, :]
                    n = 0
                    for a in range(NB):
                        m = i0 + a - j
                        if m < 0:
                            continue
                        if m not in hs:
                            hs[m] = (hf_buf[m, re, :], hf_buf[m, im, :])
                        hr, hi = hs[m]
                        pr = hr * xr - hi * xi
                        pi = hr * xi + hi * xr
                        acc[a] = (pr, pi) if acc[a] is None else (acc[a][0] + pr, acc[a][1] + pi)
                        n += 1
                    yield n
                for a in range(NB):
                    yr, yi = acc[a]
                    if prev is not None:
                        yr, yi = (yr - prev[1], yi + prev[0]) if even else (yr + prev[1], yi - prev[0])
                    prev = acc[a]
                    yf_buf[i0 + a, pl.ds(16 * r, 16), :] = jnp.concatenate([yr, yi], axis=0).astype(BF16)

    def b_post(g):
        dvec = jnp.concatenate([tap_buf[g, KS]] * (T // 8), axis=0)
        for i in range(NC):
            inv = jnp.concatenate([_ld(inv_ref, (0,), 0, T), _ld(inv_ref, (1,), 0, T)], axis=1)
            y = _dot(inv, _ld(yf_buf, (i,), 0, 2 * T)) + _ld(kv_buf, (g % 2,), i * T, T).astype(F32) * dvec
            ob_buf[g, pl.ds(i * T, T), :] = (_ld(q_buf, (g,), i * T, T).astype(F32) * y).astype(BF16)
            yield 1

    TILE_COST = 7 * KH * HS // 2
    MAIN_COST = 3 * TILE_COST + 2 * HS
    MAC_COST = (T // 8) * NC * (NC + 1) // 2
    PRE_COST = S // RP
    NORM_COST = S // CG
    KB_COST = CG // RP
    all_kb = range(KH)

    def rows_cost(c, n_tiles):
        return n_tiles * 7 * KH * (XB[c + 1] - XB[c]) // 2

    def x_cost(c):
        return (XB[c + 1] - XB[c]) * KH / (2 * RP)

    state = {"todo": [], "n": 0, "zs": [None, None]}
    x_copy(0).start()
    in_start(0, WQ_IN)
    in_start(1, WQ_IN)
    x_copy(0).wait()
    in_start(0, WK_IN)
    in_start(1, WK_IN)
    _merge((x_terms(XB[0], XB[1]), 1))
    in_wait(0, WQ_IN)
    in_wait(1, WQ_IN)
    in_start(0, WV_IN)
    in_start(1, WV_IN)
    _merge((w_terms(0, (0,), all_kb), 1))
    fence()
    _merge((a_main(0, (0,), XB[0], XB[1], state), 1))
    in_wait(0, WK_IN)
    in_wait(1, WK_IN)
    x_copy(1).start()
    _merge((w_terms(0, (1,), all_kb), 1))
    in_wait(0, WV_IN)
    in_wait(1, WV_IN)
    x_copy(2).start()
    fence()
    _merge((a_main(0, (1,), XB[0], XB[1], state), rows_cost(0, 1)), (w_terms(0, (2,), all_kb), KH * KB_COST))
    x_copy(1).wait()
    fence()
    _merge((a_main(0, (2,), XB[0], XB[1], state), rows_cost(0, 1)), (x_terms(XB[1], XB[2]), x_cost(1)))
    x_copy(2).wait()
    in_start(0, K_IN, V_IN, H_IN)
    fence()
    _merge((a_main(0, (0, 1, 2), XB[1], XB[2], state), rows_cost(1, 3)), (x_terms(XB[2], XB[3]), x_cost(2)))
    x_copy(3).start()
    fence()
    _merge((a_main(0, (0, 1, 2), XB[2], XB[3], state), 1))
    in_start(1, K_IN, V_IN)
    kf_buf[0:8, :] = jnp.zeros((8, CG), F32)
    shk = shk_ref[...].astype(F32)
    dd = dd_ref[...].astype(F32)
    for g in range(NG):
        for t in range(KS):
            tap_buf[g, t] = jnp.broadcast_to(shk[t:t + 1, g * CG:(g + 1) * CG], (8, CG))
        tap_buf[g, KS] = jnp.broadcast_to(dd[g:g + 1, :], (8, CG))
    in_wait(0, K_IN, V_IN, H_IN)
    fence()
    a_last(0)
    _merge((b_filter(0), NC), (b_pre(0), PRE_COST))
    x_copy(3).wait()
    in_start(2, *W_IN)
    in_start(3, *W_IN)
    fence()
    _merge((b_signal(0), NC), (x_terms(XB[3], XB[4]), x_cost(3)))

    def step(s, first=False):
        in_start(s, H_IN, Q_IN, WO_IN)
        if first:
            in_start(0, Q_IN, WO_IN)
            in_start(2, K_IN, V_IN)
        else:
            @pl.when(s + 1 < NG)
            def _():
                in_start(s + 1, K_IN, V_IN)

            in_wait(s - 2, WO_IN)
        in_wait(s, K_IN, V_IN)
        fence()
        streams = [(a_main(s), MAIN_COST), (b_mac(), MAC_RATE * MAC_COST)]
        streams.append((b_pre(s), PRE_COST))
        if not first:
            norm, mix = a_norm(s - 2), a_mix(s - 2)
            streams += [(_take(norm, NORM_SPLIT), NORM_SPLIT + 1e-3), (_take(mix, MIX_SPLIT), MIX_SPLIT + 1e-3)]
        _merge(*streams)
        in_wait(s, H_IN)
        in_wait(s - 1, Q_IN)
        if first:
            in_wait(2, *W_IN)
            in_wait(3, *W_IN)
            in_start(4, *W_IN)
            in_start(5, *W_IN)
            terms = (w_terms(1, range(3), all_kb), 3 * KH * KB_COST)
        else:
            @pl.when(jnp.logical_and(s % 2 == 0, s + 2 < NG))
            def _():
                in_wait(s + 2, *W_IN)
                in_wait(s + 3, *W_IN)

            @pl.when(jnp.logical_and(s % 2 == 1, s + 3 < NG))
            def _():
                in_start(s + 3, *W_IN)
                in_start(s + 4, *W_IN)

            kbs = [s % 2 * (KH // 2) + i for i in range(KH // 2)]
            terms = (w_terms((s // 2 + 1) % NP, range(3), kbs), 3 * KH // 2 * KB_COST)
        fence()
        a_last(s)
        a_heads(s - 1)
        streams = [(b_filter(s), NC), (b_signal(s), NC), (b_post(s - 1), NC), terms]
        if not first:
            streams += [(norm, NORM_COST - NORM_SPLIT + 1e-3), (mix, NG - MIX_SPLIT + 1e-3)]
        _merge(*streams)
        ob_copy(s - 1).start()

    step(1, first=True)

    def loop_body(s, carry):
        step(s)
        return carry

    jax.lax.fori_loop(2, NG, loop_body, 0)

    in_wait(NG - 2, WO_IN)
    in_wait(NG - 1, Q_IN, WO_IN)
    a_heads(NG - 1)
    mac = b_mac()
    fence()
    _merge((a_norm(NG - 2), NORM_COST), (a_mix(NG - 2), NG), (a_norm(NG - 1), NORM_COST), (a_mix(NG - 1), NG))
    fence()
    _merge((a_out_plain(), NG * NG), (m_terms(), KH * KH * KB_COST), (p_terms(0), (RO - 2 * RA) * KH / (2 * RP)))
    n_sec = S // RO
    mac_rows = S - RO - 2 * RA
    for sec in range(n_sec - 1):
        fence()
        rows = RO - (2 * RA if sec == 0 else 0)
        _merge((a_out(sec), rows // (2 * RA) * KH * 7), (p_terms(sec + 1), RO * KH / (2 * RP)),
               (mac if sec == n_sec - 2 else _take(mac, MAC_COST * rows / mac_rows), MAC_COST * rows / mac_rows))
    fence()
    out = a_out(n_sec - 1)
    half_cost = RO // (2 * RA) * KH * 7 // 2
    _merge((b_post(NG - 1), NC), (_take(out, half_cost), half_cost))
    ob_copy(NG - 1).start()
    _merge((out, 1))
    for g in range(NG):
        ob_copy(g).wait()
    for i in range(S // (2 * RA)):
        oa_copy(i).wait()


@jax.jit
def pallas_concat_heads__linear_attn_block__ssm_conv_h3__prompt_kernel(
    A_x: jax.Array,
    A_wqkv: jax.Array,
    A_wo: jax.Array,
    B_q: jax.Array,
    B_k: jax.Array,
    B_v: jax.Array,
    B_shift_k: jax.Array,
    B_ssm_k: jax.Array,
    B_ssm_D: jax.Array,
):
    hbm = pl.BlockSpec(memory_space=pl.ANY)
    vmem = pl.BlockSpec(memory_space=pltpu.VMEM)
    out = pl.pallas_call(
        _kernel,
        out_shape=jax.ShapeDtypeStruct((S, 2 * D), BF16),
        in_specs=[hbm] * 7 + [vmem] * 4,
        out_specs=hbm,
        scratch_shapes=[
            pltpu.VMEM((S, D), BF16),
            pltpu.VMEM((2, 7, KH, HS // 2, CG), BF16),
            pltpu.VMEM((NG, 3, NG, CG, CG), BF16),
            pltpu.VMEM((2, 3, 7, KH, CG, CG), BF16),
            pltpu.VMEM((NG, CG, D), BF16),
            pltpu.VMEM((NG, S, CG), BF16),
            pltpu.VMEM((NG, S, CG), BF16),
            pltpu.VMEM((NG, S, CG), BF16),
            pltpu.VMEM((NG, CG, S), BF16),
            pltpu.VMEM((NG, KS + 1, 8, CG), F32),
            pltpu.VMEM((S + 8, CG), F32),
            pltpu.VMEM((2, S, CG), BF16),
            pltpu.VMEM((NC, 2 * T, CG), F32),
            pltpu.VMEM((NC, 2 * T, CG), F32),
            pltpu.VMEM((NC, 2 * T, CG), BF16),
            pltpu.VMEM((2, HS, CG), BF16),
            pltpu.VMEM((2, HS, CG), BF16),
            pltpu.VMEM((NG, 2, 8, CG), F32),
            pltpu.VMEM((NG, 2, CG, CG), F32),
            pltpu.VMEM((2, 8 * CG // DH, CG), BF16),
            pltpu.VMEM((2, CG, CG), BF16),
            pltpu.VMEM((NG, 2, HS, CG), BF16),
            pltpu.VMEM((2, 7, KH, RO // 2, CG), BF16),
            pltpu.VMEM((NG, NG, CG, CG), BF16),
            pltpu.VMEM((KH, 7, KH, CG, CG), BF16),
            pltpu.VMEM((NG, S, CG), BF16),
            pltpu.VMEM((S, D), BF16),
            pltpu.SemaphoreType.DMA((len(XB) - 1,)),
            pltpu.SemaphoreType.DMA((NG, 8)),
            pltpu.SemaphoreType.DMA((NG,)),
            pltpu.SemaphoreType.DMA((S // (2 * RA),)),
            pltpu.SemaphoreType.REGULAR,
        ],
        compiler_params=pltpu.CompilerParams(vmem_limit_bytes=100 * 1024 * 1024, flags=FLAGS),
    )(A_x.reshape(S, D), A_wqkv.reshape(NG, CG, 3 * D), A_wo, B_q.reshape(S, D), B_k.reshape(S, D),
      B_v.reshape(S, D), B_ssm_k, B_shift_k.T, B_ssm_D.reshape(NG, CG), _FWD, _INV)
    return out.reshape(1, S, 2 * D)
```

```python
import jax
import jax.numpy as jnp
import numpy as np
import jax.experimental.pallas as pl
import jax.experimental.pallas.tpu as pltpu

S, D, H = 2048, 1024, 32
DH = D // H
CG = 128
NG = D // CG
T = 128
NC = S // T
KS = 4
NP = NG // 2
HS = S // 2
KH = NG // 2
RA = 64
NB = 2
RP = 32
RO = 512
XB = (0, 256, 512, 768, 1024, 1536, 2048)
LAG_KV = 2048
MAC_RATE = 1.0
FLAGS = None
F32, BF16, U32 = jnp.float32, jnp.bfloat16, jnp.uint32


def _dft_matrices():
    k = np.concatenate([np.arange(0, T, 2), np.arange(1, T, 2)])
    ang = np.pi * (2 * k[:, None] + 1) / (2 * T) * np.arange(T)[None, :]
    re = np.cos(ang).reshape(T // 8, 1, 8, T)
    im = -np.sin(ang).reshape(T // 8, 1, 8, T)
    fwd = np.concatenate([re, im], axis=1).reshape(2 * T, T)
    inv = fwd.T / T
    inv = np.stack([inv[:, :T], inv[:, T:]])
    return fwd.astype(BF16), inv.astype(BF16)


_FWD, _INV = _dft_matrices()


def _dot(a, b):
    return jnp.dot(a, b, preferred_element_type=F32)


def _dot_nt(a, b):
    return jax.lax.dot_general(a, b, (((1,), (1,)), ((), ())), preferred_element_type=F32)


def _dot_tn(a, b):
    return jax.lax.dot_general(a, b, (((0,), (0,)), ((), ())), preferred_element_type=F32)


def _phi(t):
    return jnp.where(t > 0, t + 1.0, jnp.exp(t)) + 1e-6


def _ld(ref, lead, r0, n):
    return pltpu.bitcast(ref.bitcast(U32)[lead + (pl.ds(r0 // 2, n // 2), slice(None))], BF16)


def _merge(*streams):
    done = [0.0] * len(streams)
    live = list(range(len(streams)))
    while live:
        i = min(live, key=lambda s: done[s] / streams[s][1])
        cost = next(streams[i][0], None)
        if cost is None:
            live.remove(i)
        else:
            done[i] += cost


def _take(stream, cost):
    while cost > 0:
        c = next(stream, None)
        if c is None:
            return
        cost -= c
        yield c


def _lhs_terms(a11, a12, a21, a22):
    return a11 + a22, a21 + a22, a11, a22, a11 + a12, a21 - a11, a12 - a22


def _rhs_terms(b11, b12, b21, b22):
    return b11 + b22, b11, b12 - b22, b21 - b11, b22, b11 + b12, b21 + b22


def _strassen(lhs, rhs, emit):
    def prod(i, acc=None):
        for kb in range(KH):
            part = _dot(lhs(i, kb), rhs(i, kb))
            acc = part if acc is None else acc + part
        return acc

    m1 = prod(0)
    yield 1
    m2 = prod(1)
    c22 = m1 - m2
    yield 1
    m4 = prod(3)
    emit(1, 0, m2 + m4)
    c11 = m1 + m4
    yield 1
    m3 = prod(2)
    c22 = c22 + m3
    yield 1
    emit(1, 1, prod(5, c22))
    yield 1
    m5 = prod(4)
    emit(0, 1, m3 + m5)
    c11 = c11 - m5
    yield 1
    emit(0, 0, prod(6, c11))
    yield 1


def _kernel(x_hbm, wqkv_hbm, wo_hbm, q_hbm, k_hbm, v_hbm, h_hbm, shk_ref, dd_ref, fwd_ref, inv_ref,
            out_hbm,
            x_buf, xs_buf, w_buf, ws_buf, wo_buf, q_buf, k_buf, v_buf, h_buf, tap_buf, kf_buf, kv_buf,
            xf_buf, hf_buf, yf_buf, pk_buf, pv_buf, z_buf, kvs_buf, zs_buf, kvbd_buf, pq_buf, ps_buf,
            m_buf, ms_buf, ob_buf, oa_buf, x_sem, in_sem, ob_sem, oa_sem, fence_sem):

    def rows_of(i, n):
        return i * n if isinstance(i, int) else pl.multiple_of(i * n, n)

    H_IN, K_IN, V_IN, Q_IN, WO_IN, WQ_IN, WK_IN, WV_IN = range(8)
    W_IN = (WQ_IN, WK_IN, WV_IN)

    def in_copy(g, which):
        if which in W_IN:
            t = which - WQ_IN
            src, dst = wqkv_hbm.at[:, :, pl.ds(rows_of(t * NG + g, CG), CG)], w_buf.at[g, t]
        elif which in (H_IN, WO_IN):
            hbm, buf = (h_hbm, h_buf) if which == H_IN else (wo_hbm, wo_buf)
            src, dst = hbm.at[pl.ds(rows_of(g, CG), CG)], buf.at[g]
        else:
            hbm, buf = {K_IN: (k_hbm, k_buf), V_IN: (v_hbm, v_buf), Q_IN: (q_hbm, q_buf)}[which]
            src, dst = hbm.at[:, pl.ds(rows_of(g, CG), CG)], buf.at[g]
        return pltpu.make_async_copy(src, dst, in_sem.at[g, which])

    def in_start(g, *whiches):
        for which in whiches:
            in_copy(g, which).start()

    def in_wait(g, *whiches):
        for which in whiches:
            in_copy(g, which).wait()

    def x_copy(c):
        rows = pl.ds(XB[c], XB[c + 1] - XB[c])
        return pltpu.make_async_copy(x_hbm.at[rows], x_buf.at[rows], x_sem.at[c])

    def ob_copy(g):
        return pltpu.make_async_copy(ob_buf.at[g], out_hbm.at[:, pl.ds(rows_of(NG + g, CG), CG)], ob_sem.at[g])

    def oa_copy(i):
        rows = pl.ds(i * 2 * RA, 2 * RA)
        return pltpu.make_async_copy(oa_buf.at[rows], out_hbm.at[rows, pl.ds(0, D)], oa_sem.at[i])

    def fence():
        pl.semaphore_signal(fence_sem, 1)
        pl.semaphore_wait(fence_sem, 1)

    def x_terms(r_lo, r_hi):
        for r0 in range(r_lo, r_hi, 2 * RA):
            for kb in range(KH):
                for r in range(0, RA, RP):
                    blocks = [x_buf[pl.ds(r0 + a * RA + r, RP), pl.ds((b * KH + kb) * CG, CG)].astype(F32)
                              for a in range(2) for b in range(2)]
                    for i, term in enumerate(_lhs_terms(*blocks)):
                        xs_buf[r0 // HS, i, kb, pl.ds(r0 % HS // 2 + r, RP), :] = term.astype(BF16)
                    yield 1

    def w_terms(p, tiles, kbs):
        for t in tiles:
            for kb in kbs:
                for r in range(0, CG, RP):
                    blocks = [_ld(w_buf, (2 * p + b, t, a * KH + kb), r, RP).astype(F32)
                              for a in range(2) for b in range(2)]
                    for i, term in enumerate(_rhs_terms(*blocks)):
                        if i not in (1, 4):
                            ws_buf[p % 2, t, i, kb, pl.ds(r, RP), :] = term.astype(BF16)
                    yield 1

    def kv_block(s, j, b):
        kv = _dot_tn(_ld(pk_buf, (j,), b * CG, CG), _ld(pv_buf, (j,), b * CG, CG))
        kvs_buf[s, j] = kv if b == 0 else kvs_buf[s, j] + kv

    def a_main(s, tiles=(0, 1, 2), r_lo=0, r_hi=HS, state=None):
        p, half = s // 2, s % 2
        state = state or {"todo": [], "n": 0, "zs": [None, None]}
        todo, zs = state["todo"], state["zs"]
        for r0 in range(r_lo, r_hi, 2 * RA):
            for t in tiles:
                def lhs(i, kb):
                    return _ld(xs_buf, (half, i, kb), r0 // 2, RA)

                def rhs(i, kb):
                    if i == 1:
                        return _ld(w_buf, (2 * p, t, kb), 0, CG)
                    if i == 4:
                        return _ld(w_buf, (2 * p + 1, t, KH + kb), 0, CG)
                    return _ld(ws_buf, (p % 2, t, i, kb), 0, CG)

                def emit(a, j, val):
                    rows = pl.ds(r0 + a * RA, RA)
                    if t == 0:
                        pq_buf[2 * p + j, half, rows, :] = _phi(val).astype(BF16)
                    elif t == 1:
                        pk = _phi(val)
                        z = jnp.sum(pk.reshape(RA // 8, 8, CG), axis=0)
                        zs[j] = z if zs[j] is None else zs[j] + z
                        pk_buf[j, rows, :] = pk.astype(BF16)
                    else:
                        pv_buf[j, rows, :] = val.astype(BF16)

                for _ in _strassen(lhs, rhs, emit):
                    state["n"] += KH * RA
                    yield KH * RA
                    if todo and todo[0][0] <= state["n"]:
                        kv_block(s, *todo.pop(0)[1:])
                        yield CG
            if 2 in tiles and (r0 + 2 * RA) % CG == 0 and r0 + 2 * RA < HS:
                todo += [(state["n"] + LAG_KV, j, (r0 + 2 * RA) // CG - 1) for j in range(2)]
        if r_hi == HS:
            for _, j, b in todo:
                kv_block(s, j, b)
            for j in range(2):
                z_buf[s, j] = zs[j]

    def a_last(s):
        for j in range(2):
            kv_block(s, j, HS // CG - 1)

    def a_heads(g):
        s0, j, slot = g // 2 * 2, g % 2, g % 2
        col_head = jax.lax.broadcasted_iota(jnp.int32, (CG, CG), 1) // DH
        row_head = jax.lax.broadcasted_iota(jnp.int32, (CG, CG), 0) // DH
        kvbd_buf[slot] = jnp.where(row_head == col_head, kvs_buf[s0, j] + kvs_buf[s0 + 1, j], 0.0).astype(BF16)
        z = jnp.sum(z_buf[s0, j] + z_buf[s0 + 1, j], axis=0, keepdims=True)
        sel = (jax.lax.broadcasted_iota(jnp.int32, (8 * CG // DH, CG), 0) // 8
               == jax.lax.broadcasted_iota(jnp.int32, (8 * CG // DH, CG), 1) // DH)
        zs_buf[slot] = jnp.where(sel, z, 0.0).astype(BF16)

    def a_norm(g):
        for half in range(2):
            for r0 in range(0, HS, CG):
                pq = _ld(pq_buf, (g, half), r0, CG)
                den = _dot_nt(_ld(zs_buf, (g % 2,), 0, 8 * CG // DH), pq) + 1e-6
                rcp = pl.reciprocal(den, approx=True)
                rcp = rcp * (2.0 - den * rcp)
                rcp = jnp.concatenate([rcp[8 * (c // DH):8 * (c // DH) + 8] for c in range(0, CG, 8)], axis=0)
                pq_buf[g, half, pl.ds(r0, CG), :] = (pq.astype(F32) * rcp.T).astype(BF16)
                yield 1

    def a_mix(g):
        for n in range(NG):
            m_buf[n, g] = _dot(_ld(kvbd_buf, (g % 2,), 0, CG), wo_buf[g, :, pl.ds(n * CG, CG)]).astype(BF16)
            yield 1

    def m_terms():
        for t in range(KH):
            for kb in range(KH):
                for r in range(0, CG, RP):
                    blocks = [_ld(m_buf, (b * KH + t, a * KH + kb), r, RP).astype(F32)
                              for a in range(2) for b in range(2)]
                    for i, term in enumerate(_rhs_terms(*blocks)):
                        if i not in (1, 4):
                            ms_buf[t, i, kb, pl.ds(r, RP), :] = term.astype(BF16)
                    yield 1

    def p_terms(sec):
        for r0 in range(max(sec * RO, 2 * RA), (sec + 1) * RO, 2 * RA):
            for kb in range(KH):
                for r in range(0, RA, RP):
                    blocks = [_ld(pq_buf, (b * KH + kb, r0 // HS), r0 % HS + a * RA + r, RP).astype(F32)
                              for a in range(2) for b in range(2)]
                    for i, term in enumerate(_lhs_terms(*blocks)):
                        if i not in (2, 3):
                            ps_buf[sec % 2, i, kb, pl.ds(r0 % RO // 2 + r, RP), :] = term.astype(BF16)
                    yield 1

    def a_out_plain():
        for n in range(NG):
            acc = None
            for g in range(NG):
                part = _dot(_ld(pq_buf, (g, 0), 0, 2 * RA), _ld(m_buf, (n, g), 0, CG))
                acc = part if acc is None else acc + part
                yield 1
            oa_buf[pl.ds(0, 2 * RA), pl.ds(n * CG, CG)] = acc.astype(BF16)
        oa_copy(0).start()

    def a_out(sec):
        for r0 in range(max(sec * RO, 2 * RA), (sec + 1) * RO, 2 * RA):
            for t in range(KH):
                def lhs(i, kb):
                    if i == 2:
                        return _ld(pq_buf, (kb, r0 // HS), r0 % HS, RA)
                    if i == 3:
                        return _ld(pq_buf, (KH + kb, r0 // HS), r0 % HS + RA, RA)
                    return _ld(ps_buf, (sec % 2, i, kb), r0 % RO // 2, RA)

                def rhs(i, kb):
                    if i == 1:
                        return _ld(m_buf, (t, kb), 0, CG)
                    if i == 4:
                        return _ld(m_buf, (KH + t, KH + kb), 0, CG)
                    return _ld(ms_buf, (t, i, kb), 0, CG)

                def emit(a, b, val):
                    oa_buf[pl.ds(r0 + a * RA, RA), pl.ds((b * KH + t) * CG, CG)] = val.astype(BF16)

                yield from _strassen(lhs, rhs, emit)
            oa_copy(r0 // (2 * RA)).start()

    def b_pre(g):
        taps = [jnp.concatenate([tap_buf[g, t]] * (RP // 8), axis=0) for t in range(KS)]
        for r0 in range(0, S, RP):
            kf = _ld(k_buf, (g,), r0, RP).astype(F32)
            kf_buf[pl.ds(8 + r0, RP), :] = kf
            acc = kf * taps[0]
            for t in range(1, KS):
                acc = acc + kf_buf[pl.ds(8 + r0 - t, RP), :] * taps[t]
            kv_buf[g % 2, pl.ds(r0, RP), :] = (acc * _ld(v_buf, (g,), r0, RP).astype(F32)).astype(BF16)
            yield 1

    def spectrum(buf, j, res, factors):
        parts = []
        for r in range(0, 2 * T, 16):
            parts += factors(res[r:r + 8], res[r + 8:r + 16])
        buf[j] = jnp.concatenate(parts, axis=0)

    def b_filter(g):
        for j in range(NC):
            spectrum(hf_buf, j, _dot_nt(_ld(fwd_ref, (), 0, 2 * T), h_buf[g, :, pl.ds(j * T, T)]),
                     lambda re, im: [re, im - re, re + im])
            yield 1

    def b_signal(g):
        for j in range(NC):
            spectrum(xf_buf, j, _dot(_ld(fwd_ref, (), 0, 2 * T), _ld(kv_buf, (g % 2,), j * T, T)),
                     lambda re, im: [re + im, re, im])
            yield 1

    def b_mac():
        for r in range(T // 8):
            rows = [pl.ds(24 * r + 8 * u, 8) for u in range(3)]
            even = r < T // 16
            prev = None
            for i0 in range(0, NC, NB):
                acc = [None] * NB
                hs = {}
                for j in range(i0 + NB):
                    xs = [xf_buf[j, u, :] for u in rows]
                    n = 0
                    for a in range(NB):
                        m = i0 + a - j
                        if m < 0:
                            continue
                        if m not in hs:
                            hs[m] = [hf_buf[m, u, :] for u in rows]
                        ks = [h * x for h, x in zip(hs[m], xs)]
                        acc[a] = ks if acc[a] is None else [c + k for c, k in zip(acc[a], ks)]
                        n += 1
                    yield n
                for a in range(NB):
                    cur = yr, yi = acc[a][0] - acc[a][2], acc[a][0] + acc[a][1]
                    if prev is not None:
                        yr, yi = (yr - prev[1], yi + prev[0]) if even else (yr + prev[1], yi - prev[0])
                    prev = cur
                    yf_buf[i0 + a, pl.ds(16 * r, 16), :] = jnp.concatenate([yr, yi], axis=0).astype(BF16)

    def b_post(g):
        dvec = jnp.concatenate([tap_buf[g, KS]] * (T // 8), axis=0)
        for i in range(NC):
            inv = jnp.concatenate([_ld(inv_ref, (0,), 0, T), _ld(inv_ref, (1,), 0, T)], axis=1)
            y = _dot(inv, _ld(yf_buf, (i,), 0, 2 * T)) + _ld(kv_buf, (g % 2,), i * T, T).astype(F32) * dvec
            ob_buf[g, pl.ds(i * T, T), :] = (_ld(q_buf, (g,), i * T, T).astype(F32) * y).astype(BF16)
            yield 1

    TILE_COST = 7 * KH * HS // 2
    MAIN_COST = 3 * TILE_COST + 2 * HS
    MAC_COST = (T // 8) * NC * (NC + 1) // 2
    PRE_COST = S // RP
    NORM_COST = S // CG
    KB_COST = CG // RP
    all_kb = range(KH)

    def rows_cost(c, n_tiles):
        return n_tiles * 7 * KH * (XB[c + 1] - XB[c]) // 2

    def x_cost(c):
        return (XB[c + 1] - XB[c]) * KH / (2 * RP)

    state = {"todo": [], "n": 0, "zs": [None, None]}
    x_copy(0).start()
    in_start(0, WQ_IN)
    in_start(1, WQ_IN)
    x_copy(0).wait()
    in_start(0, WK_IN)
    in_start(1, WK_IN)
    _merge((x_terms(XB[0], XB[1]), 1))
    in_wait(0, WQ_IN)
    in_wait(1, WQ_IN)
    in_start(0, WV_IN)
    in_start(1, WV_IN)
    _merge((w_terms(0, (0,), all_kb), 1))
    fence()
    _merge((a_main(0, (0,), XB[0], XB[1], state), 1))
    in_wait(0, WK_IN)
    in_wait(1, WK_IN)
    x_copy(1).start()
    _merge((w_terms(0, (1,), all_kb), 1))
    in_wait(0, WV_IN)
    in_wait(1, WV_IN)
    x_copy(2).start()
    fence()
    _merge((a_main(0, (1,), XB[0], XB[1], state), rows_cost(0, 1)), (w_terms(0, (2,), all_kb), KH * KB_COST))
    x_copy(1).wait()
    x_copy(3).start()
    fence()
    _merge((a_main(0, (2,), XB[0], XB[1], state), rows_cost(0, 1)), (x_terms(XB[1], XB[2]), x_cost(1)))
    x_copy(2).wait()
    x_copy(4).start()
    fence()
    _merge((a_main(0, (0, 1, 2), XB[1], XB[2], state), rows_cost(1, 3)), (x_terms(XB[2], XB[3]), x_cost(2)))
    x_copy(3).wait()
    x_copy(5).start()
    fence()
    _merge((a_main(0, (0, 1, 2), XB[2], XB[3], state), rows_cost(2, 3)), (x_terms(XB[3], XB[4]), x_cost(3)))
    x_copy(4).wait()
    in_start(0, K_IN, V_IN)
    fence()
    _merge((a_main(0, (0, 1, 2), XB[3], XB[4], state), rows_cost(3, 3)), (x_terms(XB[4], XB[5]), x_cost(4)))
    x_copy(5).wait()
    in_start(0, H_IN)
    in_start(2, *W_IN)
    fence()
    state = {"todo": [], "n": 0, "zs": [None, None]}
    a_last(0)
    _merge((a_main(1, (0, 1, 2), 0, XB[5] - HS, state), rows_cost(4, 3)), (x_terms(XB[5], XB[6]), x_cost(5)))
    in_start(3, *W_IN)
    in_start(1, K_IN, V_IN)
    kf_buf[0:8, :] = jnp.zeros((8, CG), F32)
    shk = shk_ref[...].astype(F32)
    dd = dd_ref[...].astype(F32)
    for g in range(NG):
        for t in range(KS):
            tap_buf[g, t] = jnp.broadcast_to(shk[t:t + 1, g * CG:(g + 1) * CG], (8, CG))
        tap_buf[g, KS] = jnp.broadcast_to(dd[g:g + 1, :], (8, CG))
    in_wait(0, K_IN, V_IN)
    fence()
    _merge((a_main(1, (0, 1, 2), XB[5] - HS, HS, state), rows_cost(5, 3)), (b_pre(0), PRE_COST))
    in_wait(0, H_IN)
    in_wait(2, *W_IN)
    in_wait(3, *W_IN)
    in_start(4, *W_IN)
    in_start(5, *W_IN)
    in_start(0, WO_IN)
    in_start(1, WO_IN)
    fence()
    a_last(1)
    a_heads(0)
    _merge((b_filter(0), NC), (b_signal(0), NC), (w_terms(1, range(3), all_kb), 3 * KH * KB_COST))

    def step(s, carry):
        in_start(s - 1, H_IN)
        in_start(s - 2, Q_IN)
        in_start(s, K_IN, V_IN, WO_IN)
        in_wait(s - 1, K_IN, V_IN)
        fence()
        _merge((a_main(s), MAIN_COST), (b_mac(), MAC_RATE * MAC_COST), (b_pre(s - 1), PRE_COST))
        in_wait(s - 1, H_IN)
        in_wait(s - 2, Q_IN, WO_IN)

        @pl.when(jnp.logical_and(s % 2 == 0, s + 2 < NG))
        def _():
            in_wait(s + 2, *W_IN)
            in_wait(s + 3, *W_IN)

        @pl.when(jnp.logical_and(s % 2 == 1, s + 3 < NG))
        def _():
            in_start(s + 3, *W_IN)
            in_start(s + 4, *W_IN)

        fence()
        a_last(s)
        a_heads(s - 1)
        kbs = [s % 2 * (KH // 2) + i for i in range(KH // 2)]
        _merge((b_filter(s - 1), NC), (b_signal(s - 1), NC), (b_post(s - 2), NC),
               (w_terms((s // 2 + 1) % NP, range(3), kbs), 3 * KH // 2 * KB_COST),
               (a_norm(s - 2), NORM_COST), (a_mix(s - 2), NG))
        ob_copy(s - 2).start()
        return carry

    jax.lax.fori_loop(2, NG, step, 0)

    g6, g7 = NG - 2, NG - 1
    in_start(g6, Q_IN)
    in_start(g7, H_IN, Q_IN)
    in_wait(g6, WO_IN)
    in_wait(g7, WO_IN, K_IN, V_IN)
    a_heads(g7)
    fence()
    SEC_COST = RO // (2 * RA) * KH * 7
    TERMS_COST = RO * KH / (2 * RP)
    mac = b_mac()
    _merge((a_norm(g6), NORM_COST), (a_norm(g7), NORM_COST), (a_mix(g6), NG), (a_mix(g7), NG),
           (_take(mac, MAC_COST / 4), MAC_COST / 4))
    fence()
    _merge((a_out_plain(), NG * NG), (m_terms(), KH * KH * KB_COST), (p_terms(0), (RO - 2 * RA) * KH / (2 * RP)))
    fence()
    _merge((a_out(0), SEC_COST - KH * 7), (mac, MAC_COST * 3 / 4), (b_pre(g7), PRE_COST))
    in_wait(g6, Q_IN)
    in_wait(g7, H_IN)
    fence()
    _merge((b_filter(g7), NC), (b_signal(g7), NC), (b_post(g6), NC), (p_terms(1), TERMS_COST))
    ob_copy(g6).start()
    mac = b_mac()
    for sec in (1, 2):
        fence()
        _merge((a_out(sec), SEC_COST), (p_terms(sec + 1), TERMS_COST),
               (mac if sec == 2 else _take(mac, MAC_COST / 2), MAC_COST / 2))
    in_wait(g7, Q_IN)
    fence()
    out = a_out(3)
    _merge((b_post(g7), NC), (_take(out, SEC_COST // 2), SEC_COST // 2))
    ob_copy(g7).start()
    _merge((out, 1))
    for g in range(NG):
        ob_copy(g).wait()
    for i in range(S // (2 * RA)):
        oa_copy(i).wait()


@jax.jit
def pallas_concat_heads__linear_attn_block__ssm_conv_h3__prompt_kernel(
    A_x: jax.Array,
    A_wqkv: jax.Array,
    A_wo: jax.Array,
    B_q: jax.Array,
    B_k: jax.Array,
    B_v: jax.Array,
    B_shift_k: jax.Array,
    B_ssm_k: jax.Array,
    B_ssm_D: jax.Array,
):
    hbm = pl.BlockSpec(memory_space=pl.ANY)
    vmem = pl.BlockSpec(memory_space=pltpu.VMEM)
    out = pl.pallas_call(
        _kernel,
        out_shape=jax.ShapeDtypeStruct((S, 2 * D), BF16),
        in_specs=[hbm] * 7 + [vmem] * 4,
        out_specs=hbm,
        scratch_shapes=[
            pltpu.VMEM((S, D), BF16),
            pltpu.VMEM((2, 7, KH, HS // 2, CG), BF16),
            pltpu.VMEM((NG, 3, NG, CG, CG), BF16),
            pltpu.VMEM((2, 3, 7, KH, CG, CG), BF16),
            pltpu.VMEM((NG, CG, D), BF16),
            pltpu.VMEM((NG, S, CG), BF16),
            pltpu.VMEM((NG, S, CG), BF16),
            pltpu.VMEM((NG, S, CG), BF16),
            pltpu.VMEM((NG, CG, S), BF16),
            pltpu.VMEM((NG, KS + 1, 8, CG), F32),
            pltpu.VMEM((S + 8, CG), F32),
            pltpu.VMEM((2, S, CG), BF16),
            pltpu.VMEM((NC, 3 * T, CG), F32),
            pltpu.VMEM((NC, 3 * T, CG), F32),
            pltpu.VMEM((NC, 2 * T, CG), BF16),
            pltpu.VMEM((2, HS, CG), BF16),
            pltpu.VMEM((2, HS, CG), BF16),
            pltpu.VMEM((NG, 2, 8, CG), F32),
            pltpu.VMEM((NG, 2, CG, CG), F32),
            pltpu.VMEM((2, 8 * CG // DH, CG), BF16),
            pltpu.VMEM((2, CG, CG), BF16),
            pltpu.VMEM((NG, 2, HS, CG), BF16),
            pltpu.VMEM((2, 7, KH, RO // 2, CG), BF16),
            pltpu.VMEM((NG, NG, CG, CG), BF16),
            pltpu.VMEM((KH, 7, KH, CG, CG), BF16),
            pltpu.VMEM((NG, S, CG), BF16),
            pltpu.VMEM((S, D), BF16),
            pltpu.SemaphoreType.DMA((len(XB) - 1,)),
            pltpu.SemaphoreType.DMA((NG, 8)),
            pltpu.SemaphoreType.DMA((NG,)),
            pltpu.SemaphoreType.DMA((S // (2 * RA),)),
            pltpu.SemaphoreType.REGULAR,
        ],
        compiler_params=pltpu.CompilerParams(vmem_limit_bytes=100 * 1024 * 1024, flags=FLAGS),
    )(A_x.reshape(S, D), A_wqkv.reshape(NG, CG, 3 * D), A_wo, B_q.reshape(S, D), B_k.reshape(S, D),
      B_v.reshape(S, D), B_ssm_k, B_shift_k.T, B_ssm_D.reshape(NG, CG), _FWD, _INV)
    return out.reshape(1, S, 2 * D)
```

```python
import jax
import jax.numpy as jnp
import numpy as np
import jax.experimental.pallas as pl
import jax.experimental.pallas.tpu as pltpu

S, D, H = 2048, 1024, 32
DH = D // H
CG = 128
NG = D // CG
T = 128
NC = S // T
KS = 4
NP = NG // 2
HS = S // 2
KH = NG // 2
RA = 64
NB = 2
RP = 32
RO = 512
XB = (0, 256, 512, 768, 1024, 1536, 2048)
LAG_KV = 2048
MAC_RATE = 1.0
PRE_LAG = 64
FLAGS = None
F32, BF16, U32 = jnp.float32, jnp.bfloat16, jnp.uint32


def _dft_matrices():
    k = np.concatenate([np.arange(0, T, 2), np.arange(1, T, 2)])
    ang = np.pi * (2 * k[:, None] + 1) / (2 * T) * np.arange(T)[None, :]
    re = np.cos(ang).reshape(T // 8, 1, 8, T)
    im = -np.sin(ang).reshape(T // 8, 1, 8, T)
    fwd = np.concatenate([re, im], axis=1).reshape(2 * T, T)
    inv = fwd.T / T
    inv = np.stack([inv[:, :T], inv[:, T:]])
    return fwd.astype(BF16), inv.astype(BF16)


_FWD, _INV = _dft_matrices()


def _dot(a, b):
    return jnp.dot(a, b, preferred_element_type=F32)


def _dot_nt(a, b):
    return jax.lax.dot_general(a, b, (((1,), (1,)), ((), ())), preferred_element_type=F32)


def _dot_tn(a, b):
    return jax.lax.dot_general(a, b, (((0,), (0,)), ((), ())), preferred_element_type=F32)


def _phi(t):
    return jnp.where(t > 0, t + 1.0, jnp.exp(t)) + 1e-6


def _ld(ref, lead, r0, n):
    return pltpu.bitcast(ref.bitcast(U32)[lead + (pl.ds(r0 // 2, n // 2), slice(None))], BF16)


def _merge(*streams):
    done = [0.0] * len(streams)
    live = list(range(len(streams)))
    while live:
        i = min(live, key=lambda s: done[s] / streams[s][1])
        cost = next(streams[i][0], None)
        if cost is None:
            live.remove(i)
        else:
            done[i] += cost


def _take(stream, cost):
    while cost > 0:
        c = next(stream, None)
        if c is None:
            return
        cost -= c
        yield c


def _lhs_terms(a11, a12, a21, a22):
    return a11 + a22, a21 + a22, a11, a22, a11 + a12, a21 - a11, a12 - a22


def _rhs_terms(b11, b12, b21, b22):
    return b11 + b22, b11, b12 - b22, b21 - b11, b22, b11 + b12, b21 + b22


def _strassen(lhs, rhs, emit):
    def prod(i, acc=None):
        for kb in range(KH):
            part = _dot(lhs(i, kb), rhs(i, kb))
            acc = part if acc is None else acc + part
        return acc

    m1 = prod(0)
    yield 1
    m2 = prod(1)
    c22 = m1 - m2
    yield 1
    m4 = prod(3)
    emit(1, 0, m2 + m4)
    c11 = m1 + m4
    yield 1
    m3 = prod(2)
    c22 = c22 + m3
    yield 1
    emit(1, 1, prod(5, c22))
    yield 1
    m5 = prod(4)
    emit(0, 1, m3 + m5)
    c11 = c11 - m5
    yield 1
    emit(0, 0, prod(6, c11))
    yield 1


def _kernel(x_hbm, wqkv_hbm, wo_hbm, q_hbm, k_hbm, v_hbm, h_hbm, shk_hbm, dd_hbm, fwd_hbm, inv_hbm,
            out_hbm,
            x_buf, xs_buf, w_buf, ws_buf, wo_buf, q_buf, k_buf, v_buf, h_buf, tap_buf, kf_buf, kv_buf,
            xf_buf, hf_buf, yf_buf, pk_buf, pv_buf, z_buf, kvs_buf, zs_buf, kvbd_buf, pq_buf, ps_buf,
            m_buf, ms_buf, ob_buf, oa_buf, fwd_ref, inv_ref, shk_ref, dd_ref,
            x_sem, in_sem, small_sem, ob_sem, oa_sem, fence_sem):

    def rows_of(i, n):
        return i * n if isinstance(i, int) else pl.multiple_of(i * n, n)

    H_IN, K_IN, V_IN, Q_IN, WO_IN, WQ_IN, WK_IN, WV_IN = range(8)
    W_IN = (WQ_IN, WK_IN, WV_IN)

    def in_copy(g, which):
        if which in W_IN:
            t = which - WQ_IN
            src, dst = wqkv_hbm.at[:, :, pl.ds(rows_of(t * NG + g, CG), CG)], w_buf.at[g, t]
        elif which in (H_IN, WO_IN):
            hbm, buf = (h_hbm, h_buf) if which == H_IN else (wo_hbm, wo_buf)
            src, dst = hbm.at[pl.ds(rows_of(g, CG), CG)], buf.at[g]
        else:
            hbm, buf = {K_IN: (k_hbm, k_buf), V_IN: (v_hbm, v_buf), Q_IN: (q_hbm, q_buf)}[which]
            src, dst = hbm.at[:, pl.ds(rows_of(g, CG), CG)], buf.at[g]
        return pltpu.make_async_copy(src, dst, in_sem.at[g, which])

    def in_start(g, *whiches):
        for which in whiches:
            in_copy(g, which).start()

    def in_wait(g, *whiches):
        for which in whiches:
            in_copy(g, which).wait()

    def x_copy(c):
        rows = pl.ds(XB[c], XB[c + 1] - XB[c])
        return pltpu.make_async_copy(x_hbm.at[rows], x_buf.at[rows], x_sem.at[c])

    def ob_copy(g):
        return pltpu.make_async_copy(ob_buf.at[g], out_hbm.at[:, pl.ds(rows_of(NG + g, CG), CG)], ob_sem.at[g])

    def oa_copy(i):
        rows = pl.ds(i * 2 * RA, 2 * RA)
        return pltpu.make_async_copy(oa_buf.at[rows], out_hbm.at[rows, pl.ds(0, D)], oa_sem.at[i])

    def last_copy(n):
        rows, cols = pl.ds(S - 2 * RA, 2 * RA), pl.ds(n * CG, CG)
        return pltpu.make_async_copy(oa_buf.at[rows, cols], out_hbm.at[rows, cols], oa_sem.at[S // (2 * RA) - 1])

    def fence():
        pl.semaphore_signal(fence_sem, 1)
        pl.semaphore_wait(fence_sem, 1)

    def x_terms(r_lo, r_hi):
        for r0 in range(r_lo, r_hi, 2 * RA):
            for kb in range(KH):
                for r in range(0, RA, RP):
                    blocks = [x_buf[pl.ds(r0 + a * RA + r, RP), pl.ds((b * KH + kb) * CG, CG)].astype(F32)
                              for a in range(2) for b in range(2)]
                    for i, term in enumerate(_lhs_terms(*blocks)):
                        xs_buf[r0 // HS, i, kb, pl.ds(r0 % HS // 2 + r, RP), :] = term.astype(BF16)
                    yield 1

    def w_terms(p, tiles, kbs):
        for t in tiles:
            for kb in kbs:
                for r in range(0, CG, RP):
                    blocks = [_ld(w_buf, (2 * p + b, t, a * KH + kb), r, RP).astype(F32)
                              for a in range(2) for b in range(2)]
                    for i, term in enumerate(_rhs_terms(*blocks)):
                        if i not in (1, 4):
                            ws_buf[p & 1, t, i, kb, pl.ds(r, RP), :] = term.astype(BF16)
                    yield 1

    def kv_block(s, j, b):
        kv = _dot_tn(_ld(pk_buf, (j,), b * CG, CG), _ld(pv_buf, (j,), b * CG, CG))
        kvs_buf[s, j] = kv if b == 0 else kvs_buf[s, j] + kv

    def a_main(s, tiles=(0, 1, 2), r_lo=0, r_hi=HS, state=None):
        p, half = s >> 1, s & 1
        state = state or {"todo": [], "n": 0, "zs": [None, None]}
        todo, zs = state["todo"], state["zs"]
        for r0 in range(r_lo, r_hi, 2 * RA):
            for t in tiles:
                def lhs(i, kb):
                    return _ld(xs_buf, (half, i, kb), r0 // 2, RA)

                def rhs(i, kb):
                    if i == 1:
                        return _ld(w_buf, (2 * p, t, kb), 0, CG)
                    if i == 4:
                        return _ld(w_buf, (2 * p + 1, t, KH + kb), 0, CG)
                    return _ld(ws_buf, (p & 1, t, i, kb), 0, CG)

                def emit(a, j, val):
                    rows = pl.ds(r0 + a * RA, RA)
                    if t == 0:
                        pq_buf[2 * p + j, half, rows, :] = _phi(val).astype(BF16)
                    elif t == 1:
                        pk = _phi(val)
                        z = jnp.sum(pk.reshape(RA // 8, 8, CG), axis=0)
                        zs[j] = z if zs[j] is None else zs[j] + z
                        pk_buf[j, rows, :] = pk.astype(BF16)
                    else:
                        pv_buf[j, rows, :] = val.astype(BF16)

                for _ in _strassen(lhs, rhs, emit):
                    state["n"] += KH * RA
                    yield KH * RA
                    if todo and todo[0][0] <= state["n"]:
                        kv_block(s, *todo.pop(0)[1:])
                        yield CG
            if 2 in tiles and (r0 + 2 * RA) % CG == 0 and r0 + 2 * RA < HS:
                todo += [(state["n"] + LAG_KV, j, (r0 + 2 * RA) // CG - 1) for j in range(2)]
        if r_hi == HS:
            for _, j, b in todo:
                kv_block(s, j, b)
            for j in range(2):
                z_buf[s, j] = zs[j]

    def a_last(s):
        for j in range(2):
            kv_block(s, j, HS // CG - 1)

    def a_heads(g):
        s0, j, slot = g >> 1 << 1, g & 1, g & 1
        col_head = jax.lax.broadcasted_iota(jnp.int32, (CG, CG), 1) // DH
        row_head = jax.lax.broadcasted_iota(jnp.int32, (CG, CG), 0) // DH
        kvbd_buf[slot] = jnp.where(row_head == col_head, kvs_buf[s0, j] + kvs_buf[s0 + 1, j], 0.0).astype(BF16)
        z = jnp.sum(z_buf[s0, j] + z_buf[s0 + 1, j], axis=0, keepdims=True)
        sel = (jax.lax.broadcasted_iota(jnp.int32, (8 * CG // DH, CG), 0) // 8
               == jax.lax.broadcasted_iota(jnp.int32, (8 * CG // DH, CG), 1) // DH)
        zs_buf[slot] = jnp.where(sel, z, 0.0).astype(BF16)

    def a_norm(g):
        for half in range(2):
            for r0 in range(0, HS, CG):
                pq = _ld(pq_buf, (g, half), r0, CG)
                den = _dot_nt(_ld(zs_buf, (g & 1,), 0, 8 * CG // DH), pq) + 1e-6
                rcp = pl.reciprocal(den, approx=True)
                rcp = rcp * (2.0 - den * rcp)
                rcp = jnp.concatenate([rcp[8 * (c // DH):8 * (c // DH) + 8] for c in range(0, CG, 8)], axis=0)
                pq_buf[g, half, pl.ds(r0, CG), :] = (pq.astype(F32) * rcp.T).astype(BF16)
                yield 1

    def a_mix(g):
        for n in range(NG):
            m_buf[n, g] = _dot(_ld(kvbd_buf, (g & 1,), 0, CG), wo_buf[g, :, pl.ds(n * CG, CG)]).astype(BF16)
            yield 1

    def m_terms():
        for t in range(KH):
            for kb in range(KH):
                for r in range(0, CG, RP):
                    blocks = [_ld(m_buf, (b * KH + t, a * KH + kb), r, RP).astype(F32)
                              for a in range(2) for b in range(2)]
                    for i, term in enumerate(_rhs_terms(*blocks)):
                        if i not in (1, 4):
                            ms_buf[t, i, kb, pl.ds(r, RP), :] = term.astype(BF16)
                    yield 1

    def p_terms(sec):
        for r0 in range(max(sec * RO, 2 * RA), (sec + 1) * RO, 2 * RA):
            for kb in range(KH):
                for r in range(0, RA, RP):
                    blocks = [_ld(pq_buf, (b * KH + kb, r0 // HS), r0 % HS + a * RA + r, RP).astype(F32)
                              for a in range(2) for b in range(2)]
                    for i, term in enumerate(_lhs_terms(*blocks)):
                        if i not in (2, 3):
                            ps_buf[sec % 2, i, kb, pl.ds(r0 % RO // 2 + r, RP), :] = term.astype(BF16)
                    yield 1

    def a_out_plain():
        for n in range(NG):
            acc = None
            for g in range(NG):
                part = _dot(_ld(pq_buf, (g, 0), 0, 2 * RA), _ld(m_buf, (n, g), 0, CG))
                acc = part if acc is None else acc + part
                yield 1
            oa_buf[pl.ds(0, 2 * RA), pl.ds(n * CG, CG)] = acc.astype(BF16)
        oa_copy(0).start()

    def a_out(sec):
        for r0 in range(max(sec * RO, 2 * RA), (sec + 1) * RO, 2 * RA):
            for t in range(KH):
                def lhs(i, kb):
                    if i == 2:
                        return _ld(pq_buf, (kb, r0 // HS), r0 % HS, RA)
                    if i == 3:
                        return _ld(pq_buf, (KH + kb, r0 // HS), r0 % HS + RA, RA)
                    return _ld(ps_buf, (sec % 2, i, kb), r0 % RO // 2, RA)

                def rhs(i, kb):
                    if i == 1:
                        return _ld(m_buf, (t, kb), 0, CG)
                    if i == 4:
                        return _ld(m_buf, (KH + t, KH + kb), 0, CG)
                    return _ld(ms_buf, (t, i, kb), 0, CG)

                def emit(a, b, val):
                    oa_buf[pl.ds(r0 + a * RA, RA), pl.ds((b * KH + t) * CG, CG)] = val.astype(BF16)

                yield from _strassen(lhs, rhs, emit)
                if r0 + 2 * RA == S:
                    for b in range(2):
                        last_copy(b * KH + t).start()
            if r0 + 2 * RA < S:
                oa_copy(r0 // (2 * RA)).start()

    def b_pre(g):
        taps = [jnp.concatenate([tap_buf[g, t]] * (RP // 8), axis=0) for t in range(KS)]
        for r0 in range(-PRE_LAG, S, RP):
            if r0 + PRE_LAG < S:
                kf_buf[pl.ds(8 + r0 + PRE_LAG, RP), :] = _ld(k_buf, (g,), r0 + PRE_LAG, RP).astype(F32)
            if r0 < 0:
                continue
            acc = kf_buf[pl.ds(8 + r0, RP), :] * taps[0]
            for t in range(1, KS):
                acc = acc + kf_buf[pl.ds(8 + r0 - t, RP), :] * taps[t]
            kv_buf[g & 3, pl.ds(r0, RP), :] = (acc * _ld(v_buf, (g,), r0, RP).astype(F32)).astype(BF16)
            yield 1

    def spectrum(buf, j, res, factors):
        parts = []
        for r in range(0, 2 * T, 16):
            parts += factors(res[r:r + 8], res[r + 8:r + 16])
        buf[j] = jnp.concatenate(parts, axis=0)

    def b_filter(g, u=0):
        for j in range(NC):
            spectrum(hf_buf.at[u], j, _dot_nt(_ld(fwd_ref, (), 0, 2 * T), h_buf[g, :, pl.ds(j * T, T)]),
                     lambda re, im: [re, im - re, re + im])
            yield 1

    def b_signal(g, u=0):
        for j in range(NC):
            spectrum(xf_buf.at[u], j, _dot(_ld(fwd_ref, (), 0, 2 * T), _ld(kv_buf, (g & 3,), j * T, T)),
                     lambda re, im: [re + im, re, im])
            yield 1

    def b_mac(u=0):
        for r in range(T // 8):
            rows = [pl.ds(24 * r + o, 8) for o in (0, 8, 16)]
            even = r < T // 16
            prev = None
            for i0 in range(0, NC, NB):
                acc = [None] * NB
                hs = {}
                for j in range(i0 + NB):
                    xs = [xf_buf[u, j, rr, :] for rr in rows]
                    n = 0
                    for a in range(NB):
                        m = i0 + a - j
                        if m < 0:
                            continue
                        if m not in hs:
                            hs[m] = [hf_buf[u, m, rr, :] for rr in rows]
                        ks = [h * x for h, x in zip(hs[m], xs)]
                        acc[a] = ks if acc[a] is None else [c + k for c, k in zip(acc[a], ks)]
                        n += 1
                    yield n
                for a in range(NB):
                    cur = yr, yi = acc[a][0] - acc[a][2], acc[a][0] + acc[a][1]
                    if prev is not None:
                        yr, yi = (yr - prev[1], yi + prev[0]) if even else (yr + prev[1], yi - prev[0])
                    prev = cur
                    yf_buf[u, i0 + a, pl.ds(16 * r, 16), :] = jnp.concatenate([yr, yi], axis=0).astype(BF16)

    def b_post(g, u=0):
        dvec = jnp.concatenate([tap_buf[g, KS]] * (T // 8), axis=0)
        for i in range(NC):
            inv = jnp.concatenate([_ld(inv_ref, (0,), 0, T), _ld(inv_ref, (1,), 0, T)], axis=1)
            y = _dot(inv, _ld(yf_buf, (u, i), 0, 2 * T)) + _ld(kv_buf, (g & 3,), i * T, T).astype(F32) * dvec
            ob_buf[g, pl.ds(i * T, T), :] = (_ld(q_buf, (g,), i * T, T).astype(F32) * y).astype(BF16)
            yield 1

    TILE_COST = 7 * KH * HS // 2
    MAIN_COST = 3 * TILE_COST + 2 * HS
    MAC_COST = (T // 8) * NC * (NC + 1) // 2
    PRE_COST = S // RP
    NORM_COST = S // CG
    KB_COST = CG // RP
    all_kb = range(KH)

    def rows_cost(c, n_tiles):
        return n_tiles * 7 * KH * (XB[c + 1] - XB[c]) // 2

    def x_cost(c):
        return (XB[c + 1] - XB[c]) * KH / (2 * RP)

    state = {"todo": [], "n": 0, "zs": [None, None]}
    small = [pltpu.make_async_copy(src, dst, small_sem.at[i]) for i, (src, dst) in enumerate(
        ((shk_hbm, shk_ref), (dd_hbm, dd_ref), (fwd_hbm, fwd_ref), (inv_hbm, inv_ref)))]

    def pair_start(which):
        in_start(0, which)
        in_start(1, which)

    def pair_wait(which):
        in_wait(0, which)
        in_wait(1, which)

    x_copy(0).start()
    pair_start(WQ_IN)
    x_copy(0).wait()
    x_copy(1).start()
    _merge((x_terms(XB[0], XB[1]), 1))
    pair_wait(WQ_IN)
    pair_start(WK_IN)
    _merge((w_terms(0, (0,), all_kb), 1))
    fence()
    _merge((a_main(0, (0,), XB[0], XB[1], state), 1))
    x_copy(1).wait()
    pair_start(WV_IN)
    _merge((x_terms(XB[1], XB[2]), 1))
    fence()
    _merge((a_main(0, (0,), XB[1], XB[2], state), 1))
    pair_wait(WK_IN)
    x_copy(2).start()
    _merge((w_terms(0, (1,), all_kb), 1))
    pair_wait(WV_IN)
    x_copy(3).start()
    fence()
    _merge((a_main(0, (1,), XB[0], XB[2], state), 2 * rows_cost(0, 1)), (w_terms(0, (2,), all_kb), KH * KB_COST))
    x_copy(2).wait()
    x_copy(4).start()
    fence()
    _merge((a_main(0, (2,), XB[0], XB[2], state), 2 * rows_cost(0, 1)), (x_terms(XB[2], XB[3]), x_cost(2)))
    x_copy(3).wait()
    x_copy(5).start()
    for c in small:
        c.start()
    fence()
    _merge((a_main(0, (0, 1, 2), XB[2], XB[3], state), rows_cost(2, 3)), (x_terms(XB[3], XB[4]), x_cost(3)))
    x_copy(4).wait()
    in_start(0, K_IN, V_IN)
    fence()
    _merge((a_main(0, (0, 1, 2), XB[3], XB[4], state), rows_cost(3, 3)), (x_terms(XB[4], XB[5]), x_cost(4)))
    x_copy(5).wait()
    in_start(0, H_IN)
    in_start(2, *W_IN)
    fence()
    state = {"todo": [], "n": 0, "zs": [None, None]}
    a_last(0)
    _merge((a_main(1, (0, 1, 2), 0, XB[5] - HS, state), rows_cost(4, 3)), (x_terms(XB[5], XB[6]), x_cost(5)))
    in_start(3, *W_IN)
    in_start(1, K_IN, V_IN)
    for c in small:
        c.wait()
    kf_buf[0:8, :] = jnp.zeros((8, CG), F32)
    shk = shk_ref[...].astype(F32)
    dd = dd_ref[...].astype(F32)
    for g in range(NG):
        for t in range(KS):
            tap_buf[g, t] = jnp.broadcast_to(shk[t:t + 1, g * CG:(g + 1) * CG], (8, CG))
        tap_buf[g, KS] = jnp.broadcast_to(dd[g:g + 1, :], (8, CG))
    in_wait(0, K_IN, V_IN)
    fence()
    _merge((a_main(1, (0, 1, 2), XB[5] - HS, HS, state), rows_cost(5, 3)), (b_pre(0), PRE_COST))
    in_wait(0, H_IN)
    in_wait(1, K_IN, V_IN)
    in_start(2, K_IN, V_IN)
    in_wait(2, *W_IN)
    in_wait(3, *W_IN)
    in_start(4, *W_IN)
    in_start(5, *W_IN)
    in_start(0, WO_IN)
    in_start(1, WO_IN)
    fence()
    a_last(1)
    a_heads(0)
    _merge((b_filter(0), NC), (b_signal(0), NC), (w_terms(1, range(3), all_kb), 3 * KH * KB_COST),
           (b_pre(1), PRE_COST))

    def step(s, carry):
        in_start(s - 1, H_IN)
        in_start(s - 2, Q_IN)
        in_start(s, WO_IN)

        @pl.when(s + 1 < NG)
        def _():
            in_start(s + 1, K_IN, V_IN)

        @pl.when(s + 1 == NG)
        def _():
            in_start(s, H_IN)

        in_wait(s, K_IN, V_IN)
        fence()
        _merge((a_main(s), MAIN_COST), (b_mac(), MAC_RATE * MAC_COST), (b_pre(s), PRE_COST))
        in_wait(s - 1, H_IN)
        in_wait(s - 2, Q_IN, WO_IN)

        @pl.when(jnp.logical_and((s & 1) == 0, s + 2 < NG))
        def _():
            in_wait(s + 2, *W_IN)
            in_wait(s + 3, *W_IN)

        @pl.when(jnp.logical_and((s & 1) == 1, s + 3 < NG))
        def _():
            in_start(s + 3, *W_IN)
            in_start(s + 4, *W_IN)

        fence()
        a_last(s)
        a_heads(s - 1)
        kbs = [(s & 1) * (KH // 2) + i for i in range(KH // 2)]
        _merge((b_filter(s - 1), NC), (b_signal(s - 1), NC), (b_post(s - 2), NC),
               (w_terms(((s >> 1) + 1) & (NP - 1), range(3), kbs), 3 * KH // 2 * KB_COST),
               (a_norm(s - 2), NORM_COST), (a_mix(s - 2), NG))
        ob_copy(s - 2).start()
        return carry

    jax.lax.fori_loop(2, NG, step, 0)

    g6, g7 = NG - 2, NG - 1
    in_start(g6, Q_IN)
    in_start(g7, Q_IN)
    in_wait(g6, WO_IN)
    in_wait(g7, WO_IN, H_IN)
    a_heads(g7)
    fence()
    SEC_COST = RO // (2 * RA) * KH * 7
    TERMS_COST = RO * KH / (2 * RP)
    mac = b_mac()
    _merge((b_filter(g7, 1), NC), (b_signal(g7, 1), NC), (a_norm(g6), NORM_COST), (a_norm(g7), NORM_COST),
           (a_mix(g6), NG), (a_mix(g7), NG), (_take(mac, MAC_COST / 4), MAC_COST / 4))
    fence()
    _merge((a_out_plain(), NG * NG), (m_terms(), KH * KH * KB_COST), (p_terms(0), (RO - 2 * RA) * KH / (2 * RP)))
    fence()
    _merge((a_out(0), SEC_COST - KH * 7), (mac, MAC_COST * 3 / 4), (p_terms(1), TERMS_COST))
    in_wait(g6, Q_IN)
    in_wait(g7, Q_IN)
    mac = b_mac(1)
    fence()
    _merge((a_out(1), SEC_COST), (p_terms(2), TERMS_COST), (_take(mac, MAC_COST / 2), MAC_COST / 2),
           (b_post(g6), NC))
    ob_copy(g6).start()
    fence()
    _merge((a_out(2), SEC_COST), (p_terms(3), TERMS_COST), (mac, MAC_COST / 2))
    fence()
    out = a_out(3)
    _merge((b_post(g7, 1), NC), (_take(out, SEC_COST // 2), SEC_COST // 2))
    ob_copy(g7).start()
    _merge((out, 1))
    for g in range(NG):
        ob_copy(g).wait()
    for i in range(S // (2 * RA) - 1):
        oa_copy(i).wait()
    for n in range(NG):
        last_copy(n).wait()


@jax.jit
def pallas_concat_heads__linear_attn_block__ssm_conv_h3__prompt_kernel(
    A_x: jax.Array,
    A_wqkv: jax.Array,
    A_wo: jax.Array,
    B_q: jax.Array,
    B_k: jax.Array,
    B_v: jax.Array,
    B_shift_k: jax.Array,
    B_ssm_k: jax.Array,
    B_ssm_D: jax.Array,
):
    hbm = pl.BlockSpec(memory_space=pl.ANY)
    out = pl.pallas_call(
        _kernel,
        out_shape=jax.ShapeDtypeStruct((S, 2 * D), BF16),
        in_specs=[hbm] * 11,
        out_specs=hbm,
        scratch_shapes=[
            pltpu.VMEM((S, D), BF16),
            pltpu.VMEM((2, 7, KH, HS // 2, CG), BF16),
            pltpu.VMEM((NG, 3, NG, CG, CG), BF16),
            pltpu.VMEM((2, 3, 7, KH, CG, CG), BF16),
            pltpu.VMEM((NG, CG, D), BF16),
            pltpu.VMEM((NG, S, CG), BF16),
            pltpu.VMEM((NG, S, CG), BF16),
            pltpu.VMEM((NG, S, CG), BF16),
            pltpu.VMEM((NG, CG, S), BF16),
            pltpu.VMEM((NG, KS + 1, 8, CG), F32),
            pltpu.VMEM((S + 8, CG), F32),
            pltpu.VMEM((4, S, CG), BF16),
            pltpu.VMEM((2, NC, 3 * T, CG), F32),
            pltpu.VMEM((2, NC, 3 * T, CG), F32),
            pltpu.VMEM((2, NC, 2 * T, CG), BF16),
            pltpu.VMEM((2, HS, CG), BF16),
            pltpu.VMEM((2, HS, CG), BF16),
            pltpu.VMEM((NG, 2, 8, CG), F32),
            pltpu.VMEM((NG, 2, CG, CG), F32),
            pltpu.VMEM((2, 8 * CG // DH, CG), BF16),
            pltpu.VMEM((2, CG, CG), BF16),
            pltpu.VMEM((NG, 2, HS, CG), BF16),
            pltpu.VMEM((2, 7, KH, RO // 2, CG), BF16),
            pltpu.VMEM((NG, NG, CG, CG), BF16),
            pltpu.VMEM((KH, 7, KH, CG, CG), BF16),
            pltpu.VMEM((NG, S, CG), BF16),
            pltpu.VMEM((S, D), BF16),
            pltpu.VMEM(_FWD.shape, BF16),
            pltpu.VMEM(_INV.shape, BF16),
            pltpu.VMEM((KS, D), BF16),
            pltpu.VMEM((NG, CG), BF16),
            pltpu.SemaphoreType.DMA((len(XB) - 1,)),
            pltpu.SemaphoreType.DMA((NG, 8)),
            pltpu.SemaphoreType.DMA((4,)),
            pltpu.SemaphoreType.DMA((NG,)),
            pltpu.SemaphoreType.DMA((S // (2 * RA),)),
            pltpu.SemaphoreType.REGULAR,
        ],
        compiler_params=pltpu.CompilerParams(vmem_limit_bytes=100 * 1024 * 1024, flags=FLAGS),
    )(A_x.reshape(S, D), A_wqkv.reshape(NG, CG, 3 * D), A_wo, B_q.reshape(S, D), B_k.reshape(S, D),
      B_v.reshape(S, D), B_ssm_k, B_shift_k.T, B_ssm_D.reshape(NG, CG), _FWD, _INV)
    return out.reshape(1, S, 2 * D)
```

```python
import jax
import jax.numpy as jnp
import numpy as np
import jax.experimental.pallas as pl
import jax.experimental.pallas.tpu as pltpu

S, D, H = 2048, 1024, 32
DH = D // H
CG = 128
NG = D // CG
T = 128
NC = S // T
KS = 4
NP = NG // 2
HS = S // 2
KH = NG // 2
RA = 64
NB = 2
RP = 32
RO = 512
XB = (0, 256, 512, 768, 1024, 1536, 2048)
LAG_KV = 2048
MAC_RATE = 1.0
PRE_LAG = 64
FLAGS = None
F32, BF16, U32 = jnp.float32, jnp.bfloat16, jnp.uint32


def _dft_matrices():
    k = np.concatenate([np.arange(0, T, 2), np.arange(1, T, 2)])
    ang = np.pi * (2 * k[:, None] + 1) / (2 * T) * np.arange(T)[None, :]
    re = np.cos(ang).reshape(T // 8, 1, 8, T)
    im = -np.sin(ang).reshape(T // 8, 1, 8, T)
    fwd = np.concatenate([re, im], axis=1).reshape(2 * T, T)
    inv = fwd.T / T
    inv = np.stack([inv[:, :T], inv[:, T:]])
    return fwd.astype(BF16), inv.astype(BF16)


_FWD, _INV = _dft_matrices()


def _dot(a, b):
    return jnp.dot(a, b, preferred_element_type=F32)


def _dot_nt(a, b):
    return jax.lax.dot_general(a, b, (((1,), (1,)), ((), ())), preferred_element_type=F32)


def _dot_tn(a, b):
    return jax.lax.dot_general(a, b, (((0,), (0,)), ((), ())), preferred_element_type=F32)


def _phi(t):
    return jnp.where(t > 0, t + 1.0, jnp.exp(t)) + 1e-6


def _ld(ref, lead, r0, n):
    return pltpu.bitcast(ref.bitcast(U32)[lead + (pl.ds(r0 // 2, n // 2), slice(None))], BF16)


def _merge(*streams):
    done = [0.0] * len(streams)
    live = list(range(len(streams)))
    while live:
        i = min(live, key=lambda s: done[s] / streams[s][1])
        cost = next(streams[i][0], None)
        if cost is None:
            live.remove(i)
        else:
            done[i] += cost


def _take(stream, cost):
    while cost > 0:
        c = next(stream, None)
        if c is None:
            return
        cost -= c
        yield c


def _lhs_terms(a11, a12, a21, a22):
    return a11 + a22, a21 + a22, a11, a22, a11 + a12, a21 - a11, a12 - a22


def _rhs_terms(b11, b12, b21, b22):
    return b11 + b22, b11, b12 - b22, b21 - b11, b22, b11 + b12, b21 + b22


def _strassen(lhs, rhs, emit):
    def prod(i, acc=None):
        for kb in range(KH):
            part = _dot(lhs(i, kb), rhs(i, kb))
            acc = part if acc is None else acc + part
        return acc

    m1 = prod(0)
    yield 1
    m2 = prod(1)
    c22 = m1 - m2
    yield 1
    m4 = prod(3)
    emit(1, 0, m2 + m4)
    c11 = m1 + m4
    yield 1
    m3 = prod(2)
    c22 = c22 + m3
    yield 1
    emit(1, 1, prod(5, c22))
    yield 1
    m5 = prod(4)
    emit(0, 1, m3 + m5)
    c11 = c11 - m5
    yield 1
    emit(0, 0, prod(6, c11))
    yield 1


def _kernel(x_hbm, wqkv_hbm, wo_hbm, q_hbm, k_hbm, v_hbm, h_hbm, shk_hbm, dd_hbm, fwd_hbm, inv_hbm,
            out_hbm,
            x_buf, xs_buf, w_buf, ws_buf, wo_buf, q_buf, k_buf, v_buf, h_buf, tap_buf, kf_buf, kv_buf,
            xf_buf, hf_buf, yf_buf, pk_buf, pv_buf, z_buf, kvs_buf, zs_buf, kvbd_buf, pq_buf, ps_buf,
            m_buf, ms_buf, ob_buf, oa_buf, fwd_ref, inv_ref, shk_ref, dd_ref,
            x_sem, in_sem, small_sem, ob_sem, oa_sem, fence_sem):

    def rows_of(i, n):
        return i * n if isinstance(i, int) else pl.multiple_of(i * n, n)

    H_IN, K_IN, V_IN, Q_IN, WO_IN, WQ_IN, WK_IN, WV_IN = range(8)
    W_IN = (WQ_IN, WK_IN, WV_IN)

    def in_copy(g, which):
        if which in W_IN:
            t = which - WQ_IN
            src, dst = wqkv_hbm.at[:, :, pl.ds(rows_of(t * NG + g, CG), CG)], w_buf.at[g, t]
        elif which in (H_IN, WO_IN):
            hbm, buf = (h_hbm, h_buf) if which == H_IN else (wo_hbm, wo_buf)
            src, dst = hbm.at[pl.ds(rows_of(g, CG), CG)], buf.at[g]
        else:
            hbm, buf = {K_IN: (k_hbm, k_buf), V_IN: (v_hbm, v_buf), Q_IN: (q_hbm, q_buf)}[which]
            src, dst = hbm.at[:, pl.ds(rows_of(g, CG), CG)], buf.at[g]
        return pltpu.make_async_copy(src, dst, in_sem.at[g, which])

    def in_start(g, *whiches):
        for which in whiches:
            in_copy(g, which).start()

    def in_wait(g, *whiches):
        for which in whiches:
            in_copy(g, which).wait()

    def x_copy(c):
        rows = pl.ds(XB[c], XB[c + 1] - XB[c])
        return pltpu.make_async_copy(x_hbm.at[rows], x_buf.at[rows], x_sem.at[c])

    def ob_copy(g):
        return pltpu.make_async_copy(ob_buf.at[g], out_hbm.at[:, pl.ds(rows_of(NG + g, CG), CG)], ob_sem.at[g])

    def oa_copy(i):
        rows = pl.ds(i * 2 * RA, 2 * RA)
        return pltpu.make_async_copy(oa_buf.at[rows], out_hbm.at[rows, pl.ds(0, D)], oa_sem.at[i])

    def last_copy(n):
        rows, cols = pl.ds(S - 2 * RA, 2 * RA), pl.ds(n * CG, CG)
        return pltpu.make_async_copy(oa_buf.at[rows, cols], out_hbm.at[rows, cols], oa_sem.at[S // (2 * RA) - 1])

    def fence():
        pl.semaphore_signal(fence_sem, 1)
        pl.semaphore_wait(fence_sem, 1)

    def x_terms(r_lo, r_hi):
        for r0 in range(r_lo, r_hi, 2 * RA):
            for kb in range(KH):
                for r in range(0, RA, RP):
                    blocks = [x_buf[pl.ds(r0 + a * RA + r, RP), pl.ds((b * KH + kb) * CG, CG)].astype(F32)
                              for a in range(2) for b in range(2)]
                    for i, term in enumerate(_lhs_terms(*blocks)):
                        xs_buf[r0 // HS, i, kb, pl.ds(r0 % HS // 2 + r, RP), :] = term.astype(BF16)
                    yield 1

    def w_terms(p, tiles, kbs):
        for t in tiles:
            for kb in kbs:
                for r in range(0, CG, RP):
                    blocks = [_ld(w_buf, (2 * p + b, t, a * KH + kb), r, RP).astype(F32)
                              for a in range(2) for b in range(2)]
                    for i, term in enumerate(_rhs_terms(*blocks)):
                        if i not in (1, 4):
                            ws_buf[p & 1, t, i, kb, pl.ds(r, RP), :] = term.astype(BF16)
                    yield 1

    def kv_block(s, j, b):
        kv = _dot_tn(_ld(pk_buf, (j,), b * CG, CG), _ld(pv_buf, (j,), b * CG, CG))
        kvs_buf[s, j] = kv if b == 0 else kvs_buf[s, j] + kv

    def a_main(s, tiles=(0, 1, 2), r_lo=0, r_hi=HS, state=None):
        p, half = s >> 1, s & 1
        state = state or {"todo": [], "n": 0, "zs": [None, None]}
        todo, zs = state["todo"], state["zs"]
        for r0 in range(r_lo, r_hi, 2 * RA):
            for t in tiles:
                def lhs(i, kb):
                    return _ld(xs_buf, (half, i, kb), r0 // 2, RA)

                def rhs(i, kb):
                    if i == 1:
                        return _ld(w_buf, (2 * p, t, kb), 0, CG)
                    if i == 4:
                        return _ld(w_buf, (2 * p + 1, t, KH + kb), 0, CG)
                    return _ld(ws_buf, (p & 1, t, i, kb), 0, CG)

                def emit(a, j, val):
                    rows = pl.ds(r0 + a * RA, RA)
                    if t == 0:
                        pq_buf[2 * p + j, half, rows, :] = _phi(val).astype(BF16)
                    elif t == 1:
                        pk = _phi(val)
                        z = jnp.sum(pk.reshape(RA // 8, 8, CG), axis=0)
                        zs[j] = z if zs[j] is None else zs[j] + z
                        pk_buf[j, rows, :] = pk.astype(BF16)
                    else:
                        pv_buf[j, rows, :] = val.astype(BF16)

                for _ in _strassen(lhs, rhs, emit):
                    state["n"] += KH * RA
                    yield KH * RA
                    if todo and todo[0][0] <= state["n"]:
                        kv_block(s, *todo.pop(0)[1:])
                        yield CG
            if 2 in tiles and (r0 + 2 * RA) % CG == 0 and r0 + 2 * RA < HS:
                todo += [(state["n"] + LAG_KV, j, (r0 + 2 * RA) // CG - 1) for j in range(2)]
        if r_hi == HS:
            for _, j, b in todo:
                kv_block(s, j, b)
            for j in range(2):
                z_buf[s, j] = zs[j]

    def a_last(s):
        for j in range(2):
            kv_block(s, j, HS // CG - 1)

    def a_heads(g):
        s0, j, slot = g >> 1 << 1, g & 1, g & 1
        col_head = jax.lax.broadcasted_iota(jnp.int32, (CG, CG), 1) // DH
        row_head = jax.lax.broadcasted_iota(jnp.int32, (CG, CG), 0) // DH
        kvbd_buf[slot] = jnp.where(row_head == col_head, kvs_buf[s0, j] + kvs_buf[s0 + 1, j], 0.0).astype(BF16)
        z = jnp.sum(z_buf[s0, j] + z_buf[s0 + 1, j], axis=0, keepdims=True)
        sel = (jax.lax.broadcasted_iota(jnp.int32, (8 * CG // DH, CG), 0) // 8
               == jax.lax.broadcasted_iota(jnp.int32, (8 * CG // DH, CG), 1) // DH)
        zs_buf[slot] = jnp.where(sel, z, 0.0).astype(BF16)

    def a_norm(g):
        for half in range(2):
            for r0 in range(0, HS, CG):
                pq = _ld(pq_buf, (g, half), r0, CG)
                den = _dot_nt(_ld(zs_buf, (g & 1,), 0, 8 * CG // DH), pq) + 1e-6
                rcp = pl.reciprocal(den, approx=True)
                rcp = rcp * (2.0 - den * rcp)
                rcp = jnp.concatenate([rcp[8 * (c // DH):8 * (c // DH) + 8] for c in range(0, CG, 8)], axis=0)
                pq_buf[g, half, pl.ds(r0, CG), :] = (pq.astype(F32) * rcp.T).astype(BF16)
                yield 1

    def a_mix(g):
        for n in range(NG):
            m_buf[n, g] = _dot(_ld(kvbd_buf, (g & 1,), 0, CG), wo_buf[g, :, pl.ds(n * CG, CG)]).astype(BF16)
            yield 1

    def m_terms():
        for t in range(KH):
            for kb in range(KH):
                for r in range(0, CG, RP):
                    blocks = [_ld(m_buf, (b * KH + t, a * KH + kb), r, RP).astype(F32)
                              for a in range(2) for b in range(2)]
                    for i, term in enumerate(_rhs_terms(*blocks)):
                        if i not in (1, 4):
                            ms_buf[t, i, kb, pl.ds(r, RP), :] = term.astype(BF16)
                    yield 1

    def p_terms(sec):
        for r0 in range(max(sec * RO, 2 * RA), (sec + 1) * RO, 2 * RA):
            for kb in range(KH):
                for r in range(0, RA, RP):
                    blocks = [_ld(pq_buf, (b * KH + kb, r0 // HS), r0 % HS + a * RA + r, RP).astype(F32)
                              for a in range(2) for b in range(2)]
                    for i, term in enumerate(_lhs_terms(*blocks)):
                        if i not in (2, 3):
                            ps_buf[sec % 2, i, kb, pl.ds(r0 % RO // 2 + r, RP), :] = term.astype(BF16)
                    yield 1

    def a_out_plain():
        for n in range(NG):
            acc = None
            for g in range(NG):
                part = _dot(_ld(pq_buf, (g, 0), 0, 2 * RA), _ld(m_buf, (n, g), 0, CG))
                acc = part if acc is None else acc + part
                yield 1
            oa_buf[pl.ds(0, 2 * RA), pl.ds(n * CG, CG)] = acc.astype(BF16)
        oa_copy(0).start()

    def a_out(sec):
        for r0 in range(max(sec * RO, 2 * RA), (sec + 1) * RO, 2 * RA):
            for t in range(KH):
                def lhs(i, kb):
                    if i == 2:
                        return _ld(pq_buf, (kb, r0 // HS), r0 % HS, RA)
                    if i == 3:
                        return _ld(pq_buf, (KH + kb, r0 // HS), r0 % HS + RA, RA)
                    return _ld(ps_buf, (sec % 2, i, kb), r0 % RO // 2, RA)

                def rhs(i, kb):
                    if i == 1:
                        return _ld(m_buf, (t, kb), 0, CG)
                    if i == 4:
                        return _ld(m_buf, (KH + t, KH + kb), 0, CG)
                    return _ld(ms_buf, (t, i, kb), 0, CG)

                def emit(a, b, val):
                    oa_buf[pl.ds(r0 + a * RA, RA), pl.ds((b * KH + t) * CG, CG)] = val.astype(BF16)

                yield from _strassen(lhs, rhs, emit)
                if r0 + 2 * RA == S:
                    for b in range(2):
                        last_copy(b * KH + t).start()
            if r0 + 2 * RA < S:
                oa_copy(r0 // (2 * RA)).start()

    def b_pre(g):
        taps = [jnp.concatenate([tap_buf[g, t]] * (RP // 8), axis=0) for t in range(KS)]
        for r0 in range(-PRE_LAG, S, RP):
            if r0 + PRE_LAG < S:
                kf_buf[pl.ds(8 + r0 + PRE_LAG, RP), :] = _ld(k_buf, (g,), r0 + PRE_LAG, RP).astype(F32)
            if r0 < 0:
                continue
            acc = kf_buf[pl.ds(8 + r0, RP), :] * taps[0]
            for t in range(1, KS):
                acc = acc + kf_buf[pl.ds(8 + r0 - t, RP), :] * taps[t]
            kv_buf[g & 3, pl.ds(r0, RP), :] = (acc * _ld(v_buf, (g,), r0, RP).astype(F32)).astype(BF16)
            yield 1

    def spectrum(buf, j, res, factors):
        parts = []
        for r in range(0, 2 * T, 16):
            parts += factors(res[r:r + 8], res[r + 8:r + 16])
        buf[j] = jnp.concatenate(parts, axis=0)

    def b_filter(g, u=0):
        for j in range(NC):
            spectrum(hf_buf.at[u], j, _dot_nt(_ld(fwd_ref, (), 0, 2 * T), h_buf[g, :, pl.ds(j * T, T)]),
                     lambda re, im: [re, im - re, re + im])
            yield 1

    def b_signal(g, u=0):
        for j in range(NC):
            spectrum(xf_buf.at[u], j, _dot(_ld(fwd_ref, (), 0, 2 * T), _ld(kv_buf, (g & 3,), j * T, T)),
                     lambda re, im: [re + im, re, im])
            yield 1

    def b_mac(u=0):
        for r in range(T // 8):
            rows = [pl.ds(24 * r + o, 8) for o in (0, 8, 16)]
            even = r < T // 16
            prev = None
            for i0 in range(0, NC, NB):
                acc = [None] * NB
                hs = {}
                for j in range(i0 + NB):
                    xs = [xf_buf[u, j, rr, :] for rr in rows]
                    n = 0
                    for a in range(NB):
                        m = i0 + a - j
                        if m < 0:
                            continue
                        if m not in hs:
                            hs[m] = [hf_buf[u, m, rr, :] for rr in rows]
                        ks = [h * x for h, x in zip(hs[m], xs)]
                        acc[a] = ks if acc[a] is None else [c + k for c, k in zip(acc[a], ks)]
                        n += 1
                    yield n
                for a in range(NB):
                    cur = yr, yi = acc[a][0] - acc[a][2], acc[a][0] + acc[a][1]
                    if prev is not None:
                        yr, yi = (yr - prev[1], yi + prev[0]) if even else (yr + prev[1], yi - prev[0])
                    prev = cur
                    yf_buf[u, i0 + a, pl.ds(16 * r, 16), :] = jnp.concatenate([yr, yi], axis=0).astype(BF16)

    def b_post(g, u=0):
        dvec = jnp.concatenate([tap_buf[g, KS]] * (T // 8), axis=0)
        for i in range(NC):
            inv = jnp.concatenate([_ld(inv_ref, (0,), 0, T), _ld(inv_ref, (1,), 0, T)], axis=1)
            y = _dot(inv, _ld(yf_buf, (u, i), 0, 2 * T)) + _ld(kv_buf, (g & 3,), i * T, T).astype(F32) * dvec
            ob_buf[g, pl.ds(i * T, T), :] = (_ld(q_buf, (g,), i * T, T).astype(F32) * y).astype(BF16)
            yield 1

    TILE_COST = 7 * KH * HS // 2
    MAIN_COST = 3 * TILE_COST + 2 * HS
    MAC_COST = (T // 8) * NC * (NC + 1) // 2
    PRE_COST = S // RP
    NORM_COST = S // CG
    KB_COST = CG // RP
    all_kb = range(KH)

    def rows_cost(c, n_tiles):
        return n_tiles * 7 * KH * (XB[c + 1] - XB[c]) // 2

    def x_cost(c):
        return (XB[c + 1] - XB[c]) * KH / (2 * RP)

    state = {"todo": [], "n": 0, "zs": [None, None]}
    small = [pltpu.make_async_copy(src, dst, small_sem.at[i]) for i, (src, dst) in enumerate(
        ((shk_hbm, shk_ref), (dd_hbm, dd_ref.at[pl.ds(0, NG)]), (fwd_hbm, fwd_ref), (inv_hbm, inv_ref)))]

    def pair_start(which):
        in_start(0, which)
        in_start(1, which)

    def pair_wait(which):
        in_wait(0, which)
        in_wait(1, which)

    x_copy(0).start()
    pair_start(WQ_IN)
    x_copy(0).wait()
    x_copy(1).start()
    _merge((x_terms(XB[0], XB[1]), 1))
    pair_wait(WQ_IN)
    pair_start(WK_IN)
    _merge((w_terms(0, (0,), all_kb), 1))
    fence()
    _merge((a_main(0, (0,), XB[0], XB[1], state), 1))
    x_copy(1).wait()
    pair_start(WV_IN)
    _merge((x_terms(XB[1], XB[2]), 1))
    fence()
    _merge((a_main(0, (0,), XB[1], XB[2], state), 1))
    pair_wait(WK_IN)
    x_copy(2).start()
    _merge((w_terms(0, (1,), all_kb), 1))
    pair_wait(WV_IN)
    x_copy(3).start()
    fence()
    _merge((a_main(0, (1,), XB[0], XB[2], state), 2 * rows_cost(0, 1)), (w_terms(0, (2,), all_kb), KH * KB_COST))
    x_copy(2).wait()
    x_copy(4).start()
    fence()
    _merge((a_main(0, (2,), XB[0], XB[2], state), 2 * rows_cost(0, 1)), (x_terms(XB[2], XB[3]), x_cost(2)))
    x_copy(3).wait()
    x_copy(5).start()
    for c in small:
        c.start()
    fence()
    _merge((a_main(0, (0, 1, 2), XB[2], XB[3], state), rows_cost(2, 3)), (x_terms(XB[3], XB[4]), x_cost(3)))
    x_copy(4).wait()
    in_start(0, K_IN, V_IN)
    fence()
    _merge((a_main(0, (0, 1, 2), XB[3], XB[4], state), rows_cost(3, 3)), (x_terms(XB[4], XB[5]), x_cost(4)))
    x_copy(5).wait()
    in_start(2, *W_IN)
    in_start(3, *W_IN)
    fence()
    state = {"todo": [], "n": 0, "zs": [None, None]}
    a_last(0)
    _merge((a_main(1, (0, 1, 2), 0, XB[5] - HS, state), rows_cost(4, 3)), (x_terms(XB[5], XB[6]), x_cost(5)))
    for c in small:
        c.wait()
    kf_buf[0:8, :] = jnp.zeros((8, CG), F32)
    shk = shk_ref[...].astype(F32)
    dd = dd_ref[0:NG, :].astype(F32)
    for g in range(NG):
        for t in range(KS):
            tap_buf[g, t] = jnp.broadcast_to(shk[t:t + 1, g * CG:(g + 1) * CG], (8, CG))
        tap_buf[g, KS] = jnp.broadcast_to(dd[g:g + 1, :], (8, CG))
    in_wait(0, K_IN, V_IN)
    in_wait(2, *W_IN)
    in_wait(3, *W_IN)
    in_start(0, H_IN)
    in_start(1, K_IN, V_IN)
    in_start(2, K_IN, V_IN)
    fence()
    _merge((a_main(1, (0, 1, 2), XB[5] - HS, HS, state), rows_cost(5, 3)), (b_pre(0), PRE_COST),
           (w_terms(1, range(3), all_kb), 3 * KH * KB_COST))
    in_wait(0, H_IN)
    in_wait(1, K_IN, V_IN)
    in_start(0, Q_IN, WO_IN)
    in_start(1, H_IN)
    in_start(3, K_IN, V_IN)
    fence()
    a_last(1)
    a_heads(0)
    _merge((b_filter(0), NC), (b_signal(0), NC), (b_pre(1), PRE_COST))
    in_wait(2, K_IN, V_IN)
    in_start(4, *W_IN)
    in_start(5, *W_IN)

    def step(s, carry):
        _merge((a_main(s), MAIN_COST), (b_mac(), MAC_RATE * MAC_COST), (b_pre(s), PRE_COST))
        in_wait(s - 1, H_IN)
        in_wait(s - 2, Q_IN, WO_IN)
        in_start(s, H_IN)
        in_start(s - 1, Q_IN, WO_IN)

        @pl.when(s + 1 < NG)
        def _():
            in_wait(s + 1, K_IN, V_IN)

        @pl.when(s + 2 < NG)
        def _():
            in_start(s + 2, K_IN, V_IN)

            @pl.when((s & 1) == 0)
            def _():
                in_wait(s + 2, *W_IN)
                in_wait(s + 3, *W_IN)

            @pl.when(s == 3)
            def _():
                in_start(6, *W_IN)
                in_start(7, *W_IN)
                in_start(7, WO_IN)

        fence()
        a_last(s)
        a_heads(s - 1)
        kbs = [(s & 1) * (KH // 2) + i for i in range(KH // 2)]
        _merge((b_filter(s - 1), NC), (b_signal(s - 1), NC), (b_post(s - 2), NC),
               (w_terms(((s >> 1) + 1) & (NP - 1), range(3), kbs), 3 * KH // 2 * KB_COST),
               (a_norm(s - 2), NORM_COST), (a_mix(s - 2), NG))
        ob_copy(s - 2).start()
        return carry

    jax.lax.fori_loop(2, NG, step, 0)

    g6, g7 = NG - 2, NG - 1
    in_start(g7, Q_IN)
    in_wait(g6, WO_IN)
    in_wait(g7, WO_IN, H_IN)
    a_heads(g7)
    fence()
    SEC_COST = RO // (2 * RA) * KH * 7
    TERMS_COST = RO * KH / (2 * RP)
    mac = b_mac()
    _merge((b_filter(g7, 1), NC), (b_signal(g7, 1), NC), (a_norm(g6), NORM_COST), (a_norm(g7), NORM_COST),
           (a_mix(g6), NG), (a_mix(g7), NG), (_take(mac, MAC_COST / 4), MAC_COST / 4))
    fence()
    _merge((a_out_plain(), NG * NG), (m_terms(), KH * KH * KB_COST), (p_terms(0), (RO - 2 * RA) * KH / (2 * RP)))
    fence()
    _merge((a_out(0), SEC_COST - KH * 7), (mac, MAC_COST * 3 / 4), (p_terms(1), TERMS_COST))
    in_wait(g6, Q_IN)
    in_wait(g7, Q_IN)
    mac = b_mac(1)
    fence()
    _merge((a_out(1), SEC_COST), (p_terms(2), TERMS_COST), (_take(mac, MAC_COST / 2), MAC_COST / 2),
           (b_post(g6), NC))
    ob_copy(g6).start()
    fence()
    _merge((a_out(2), SEC_COST), (p_terms(3), TERMS_COST), (mac, MAC_COST / 2))
    fence()
    out = a_out(3)
    _merge((b_post(g7, 1), NC), (_take(out, SEC_COST // 2), SEC_COST // 2))
    ob_copy(g7).start()
    _merge((out, 1))
    for g in range(NG):
        ob_copy(g).wait()
    for i in range(S // (2 * RA) - 1):
        oa_copy(i).wait()
    for n in range(NG):
        last_copy(n).wait()


@jax.jit
def pallas_concat_heads__linear_attn_block__ssm_conv_h3__prompt_kernel(
    A_x: jax.Array,
    A_wqkv: jax.Array,
    A_wo: jax.Array,
    B_q: jax.Array,
    B_k: jax.Array,
    B_v: jax.Array,
    B_shift_k: jax.Array,
    B_ssm_k: jax.Array,
    B_ssm_D: jax.Array,
):
    hbm = pl.BlockSpec(memory_space=pl.ANY)
    out = pl.pallas_call(
        _kernel,
        out_shape=jax.ShapeDtypeStruct((S, 2 * D), BF16),
        in_specs=[hbm] * 11,
        out_specs=hbm,
        scratch_shapes=[
            pltpu.VMEM((S, D), BF16),
            pltpu.VMEM((2, 7, KH, HS // 2, CG), BF16),
            pltpu.VMEM((NG, 3, NG, CG, CG), BF16),
            pltpu.VMEM((2, 3, 7, KH, CG, CG), BF16),
            pltpu.VMEM((NG, CG, D), BF16),
            pltpu.VMEM((NG, S, CG), BF16),
            pltpu.VMEM((NG, S, CG), BF16),
            pltpu.VMEM((NG, S, CG), BF16),
            pltpu.VMEM((NG, CG, S), BF16),
            pltpu.VMEM((NG, KS + 1, 8, CG), F32),
            pltpu.VMEM((S + 8, CG), F32),
            pltpu.VMEM((4, S, CG), BF16),
            pltpu.VMEM((2, NC, 3 * T, CG), F32),
            pltpu.VMEM((2, NC, 3 * T, CG), F32),
            pltpu.VMEM((2, NC, 2 * T, CG), BF16),
            pltpu.VMEM((2, HS, CG), BF16),
            pltpu.VMEM((2, HS, CG), BF16),
            pltpu.VMEM((NG, 2, 8, CG), F32),
            pltpu.VMEM((NG, 2, CG, CG), F32),
            pltpu.VMEM((2, 8 * CG // DH, CG), BF16),
            pltpu.VMEM((2, CG, CG), BF16),
            pltpu.VMEM((NG, 2, HS, CG), BF16),
            pltpu.VMEM((2, 7, KH, RO // 2, CG), BF16),
            pltpu.VMEM((NG, NG, CG, CG), BF16),
            pltpu.VMEM((KH, 7, KH, CG, CG), BF16),
            pltpu.VMEM((NG, S, CG), BF16),
            pltpu.VMEM((S, D), BF16),
            pltpu.VMEM(_FWD.shape, BF16),
            pltpu.VMEM(_INV.shape, BF16),
            pltpu.VMEM((KS, D), BF16),
            pltpu.VMEM((2 * NG, CG), BF16),
            pltpu.SemaphoreType.DMA((len(XB) - 1,)),
            pltpu.SemaphoreType.DMA((NG, 8)),
            pltpu.SemaphoreType.DMA((4,)),
            pltpu.SemaphoreType.DMA((NG,)),
            pltpu.SemaphoreType.DMA((S // (2 * RA),)),
            pltpu.SemaphoreType.REGULAR,
        ],
        compiler_params=pltpu.CompilerParams(vmem_limit_bytes=100 * 1024 * 1024, flags=FLAGS),
    )(A_x.reshape(S, D), A_wqkv.reshape(NG, CG, 3 * D), A_wo, B_q.reshape(S, D), B_k.reshape(S, D),
      B_v.reshape(S, D), B_ssm_k, B_shift_k.T, B_ssm_D.reshape(NG, CG), _FWD, _INV)
    return out.reshape(1, S, 2 * D)
```

```python
import jax
import jax.numpy as jnp
import numpy as np
import jax.experimental.pallas as pl
import jax.experimental.pallas.tpu as pltpu

S, D, H = 2048, 1024, 32
DH = D // H
CG = 128
NG = D // CG
T = 128
NC = S // T
KS = 4
NP = NG // 2
HS = S // 2
KH = NG // 2
RA = 64
NB = 2
RP = 32
RO = 512
XB = (0, 256, 512, 768, 1024, 1536, 2048)
LAG_KV = 2048
MAC_RATE = 1.0
PRE_LAG = 64
FLAGS = None
F32, BF16, U32 = jnp.float32, jnp.bfloat16, jnp.uint32


def _dft_matrices():
    k = np.concatenate([np.arange(0, T, 2), np.arange(1, T, 2)])
    ang = np.pi * (2 * k[:, None] + 1) / (2 * T) * np.arange(T)[None, :]
    re = np.cos(ang).reshape(T // 8, 1, 8, T)
    im = -np.sin(ang).reshape(T // 8, 1, 8, T)
    fwd = np.concatenate([re, im], axis=1).reshape(2 * T, T)
    inv = fwd.T / T
    inv = np.stack([inv[:, :T], inv[:, T:]])
    return fwd.astype(BF16), inv.astype(BF16)


_FWD, _INV = _dft_matrices()


def _dot(a, b):
    return jnp.dot(a, b, preferred_element_type=F32)


def _dot_nt(a, b):
    return jax.lax.dot_general(a, b, (((1,), (1,)), ((), ())), preferred_element_type=F32)


def _dot_tn(a, b):
    return jax.lax.dot_general(a, b, (((0,), (0,)), ((), ())), preferred_element_type=F32)


def _phi(t):
    return jnp.where(t > 0, t + 1.0, jnp.exp(t)) + 1e-6


def _ld(ref, lead, r0, n):
    return pltpu.bitcast(ref.bitcast(U32)[lead + (pl.ds(r0 // 2, n // 2), slice(None))], BF16)


def _merge(*streams):
    done = [0.0] * len(streams)
    live = list(range(len(streams)))
    while live:
        i = min(live, key=lambda s: done[s] / streams[s][1])
        cost = next(streams[i][0], None)
        if cost is None:
            live.remove(i)
        else:
            done[i] += cost


def _take(stream, cost):
    while cost > 0:
        c = next(stream, None)
        if c is None:
            return
        cost -= c
        yield c


def _lhs_terms(a11, a12, a21, a22):
    return a11 + a22, a21 + a22, a11, a22, a11 + a12, a21 - a11, a12 - a22


def _rhs_terms(b11, b12, b21, b22):
    return b11 + b22, b11, b12 - b22, b21 - b11, b22, b11 + b12, b21 + b22


def _strassen(lhs, rhs, emit):
    def prod(i, acc=None):
        for kb in range(KH):
            part = _dot(lhs(i, kb), rhs(i, kb))
            acc = part if acc is None else acc + part
        return acc

    m1 = prod(0)
    yield 1
    m2 = prod(1)
    c22 = m1 - m2
    yield 1
    m4 = prod(3)
    emit(1, 0, m2 + m4)
    c11 = m1 + m4
    yield 1
    m3 = prod(2)
    c22 = c22 + m3
    yield 1
    emit(1, 1, prod(5, c22))
    yield 1
    m5 = prod(4)
    emit(0, 1, m3 + m5)
    c11 = c11 - m5
    yield 1
    emit(0, 0, prod(6, c11))
    yield 1


def _kernel(x_hbm, wqkv_hbm, wo_hbm, q_hbm, k_hbm, v_hbm, h_hbm, shk_hbm, dd_hbm, fwd_hbm, inv_hbm,
            out_hbm,
            x_buf, xs_buf, w_buf, ws_buf, wo_buf, q_buf, k_buf, v_buf, h_buf, tap_buf, kf_buf, kv_buf,
            xf_buf, hf_buf, yf_buf, pk_buf, pv_buf, z_buf, kvs_buf, zs_buf, kvbd_buf, pq_buf, ps_buf,
            m_buf, ms_buf, ob_buf, oa_buf, fwd_ref, inv_ref, shk_ref, dd_ref,
            x_sem, in_sem, small_sem, ob_sem, oa_sem, fence_sem):

    def rows_of(i, n):
        return i * n if isinstance(i, int) else pl.multiple_of(i * n, n)

    H_IN, K_IN, V_IN, Q_IN, WO_IN, WQ_IN, WK_IN, WV_IN = range(8)
    W_IN = (WQ_IN, WK_IN, WV_IN)

    def in_copy(g, which):
        if which in W_IN:
            t = which - WQ_IN
            src, dst = wqkv_hbm.at[:, :, pl.ds(rows_of(t * NG + g, CG), CG)], w_buf.at[g, t]
        elif which in (H_IN, WO_IN):
            hbm, buf = (h_hbm, h_buf) if which == H_IN else (wo_hbm, wo_buf)
            src, dst = hbm.at[pl.ds(rows_of(g, CG), CG)], buf.at[g]
        else:
            hbm, buf = {K_IN: (k_hbm, k_buf), V_IN: (v_hbm, v_buf), Q_IN: (q_hbm, q_buf)}[which]
            src, dst = hbm.at[:, pl.ds(rows_of(g, CG), CG)], buf.at[g]
        return pltpu.make_async_copy(src, dst, in_sem.at[g, which])

    def in_start(g, *whiches):
        for which in whiches:
            in_copy(g, which).start()

    def in_wait(g, *whiches):
        for which in whiches:
            in_copy(g, which).wait()

    def x_copy(c):
        rows = pl.ds(XB[c], XB[c + 1] - XB[c])
        return pltpu.make_async_copy(x_hbm.at[rows], x_buf.at[rows], x_sem.at[c])

    def ob_copy(g):
        return pltpu.make_async_copy(ob_buf.at[g], out_hbm.at[:, pl.ds(rows_of(NG + g, CG), CG)], ob_sem.at[g])

    def oa_copy(i):
        rows = pl.ds(i * 2 * RA, 2 * RA)
        return pltpu.make_async_copy(oa_buf.at[rows], out_hbm.at[rows, pl.ds(0, D)], oa_sem.at[i])

    def last_copy(n):
        rows, cols = pl.ds(S - 2 * RA, 2 * RA), pl.ds(n * CG, CG)
        return pltpu.make_async_copy(oa_buf.at[rows, cols], out_hbm.at[rows, cols], oa_sem.at[S // (2 * RA) - 1])

    def fence():
        pl.semaphore_signal(fence_sem, 1)
        pl.semaphore_wait(fence_sem, 1)

    def x_terms(r_lo, r_hi):
        for r0 in range(r_lo, r_hi, 2 * RA):
            for kb in range(KH):
                for r in range(0, RA, RP):
                    blocks = [x_buf[pl.ds(r0 + a * RA + r, RP), pl.ds((b * KH + kb) * CG, CG)].astype(F32)
                              for a in range(2) for b in range(2)]
                    for i, term in enumerate(_lhs_terms(*blocks)):
                        xs_buf[r0 // HS, i, kb, pl.ds(r0 % HS // 2 + r, RP), :] = term.astype(BF16)
                    yield 1

    def w_terms(p, tiles, kbs):
        for t in tiles:
            for kb in kbs:
                for r in range(0, CG, RP):
                    blocks = [_ld(w_buf, (2 * p + b, t, a * KH + kb), r, RP).astype(F32)
                              for a in range(2) for b in range(2)]
                    for i, term in enumerate(_rhs_terms(*blocks)):
                        if i not in (1, 4):
                            ws_buf[p & 1, t, i, kb, pl.ds(r, RP), :] = term.astype(BF16)
                    yield 1

    def kv_block(s, j, b):
        kv = _dot_tn(_ld(pk_buf, (j,), b * CG, CG), _ld(pv_buf, (j,), b * CG, CG))
        kvs_buf[s, j] = kv if b == 0 else kvs_buf[s, j] + kv

    def a_main(s, tiles=(0, 1, 2), r_lo=0, r_hi=HS, state=None):
        p, half = s >> 1, s & 1
        state = state or {"todo": [], "n": 0, "zs": [None, None]}
        todo, zs = state["todo"], state["zs"]
        for r0 in range(r_lo, r_hi, 2 * RA):
            for t in tiles:
                def lhs(i, kb):
                    return _ld(xs_buf, (half, i, kb), r0 // 2, RA)

                def rhs(i, kb):
                    if i == 1:
                        return _ld(w_buf, (2 * p, t, kb), 0, CG)
                    if i == 4:
                        return _ld(w_buf, (2 * p + 1, t, KH + kb), 0, CG)
                    return _ld(ws_buf, (p & 1, t, i, kb), 0, CG)

                def emit(a, j, val):
                    rows = pl.ds(r0 + a * RA, RA)
                    if t == 0:
                        pq_buf[2 * p + j, half, rows, :] = _phi(val).astype(BF16)
                    elif t == 1:
                        pk = _phi(val)
                        z = jnp.sum(pk.reshape(RA // 8, 8, CG), axis=0)
                        zs[j] = z if zs[j] is None else zs[j] + z
                        pk_buf[j, rows, :] = pk.astype(BF16)
                    else:
                        pv_buf[j, rows, :] = val.astype(BF16)

                for _ in _strassen(lhs, rhs, emit):
                    state["n"] += KH * RA
                    yield KH * RA
                    if todo and todo[0][0] <= state["n"]:
                        kv_block(s, *todo.pop(0)[1:])
                        yield CG
            if 2 in tiles and (r0 + 2 * RA) % CG == 0 and r0 + 2 * RA < HS:
                todo += [(state["n"] + LAG_KV, j, (r0 + 2 * RA) // CG - 1) for j in range(2)]
        if r_hi == HS:
            for _, j, b in todo:
                kv_block(s, j, b)
            for j in range(2):
                z_buf[s, j] = zs[j]

    def a_last(s):
        for j in range(2):
            kv_block(s, j, HS // CG - 1)

    def a_heads(g):
        s0, j, slot = g >> 1 << 1, g & 1, g & 1
        col_head = jax.lax.broadcasted_iota(jnp.int32, (CG, CG), 1) // DH
        row_head = jax.lax.broadcasted_iota(jnp.int32, (CG, CG), 0) // DH
        kvbd_buf[slot] = jnp.where(row_head == col_head, kvs_buf[s0, j] + kvs_buf[s0 + 1, j], 0.0).astype(BF16)
        z = jnp.sum(z_buf[s0, j] + z_buf[s0 + 1, j], axis=0, keepdims=True)
        sel = (jax.lax.broadcasted_iota(jnp.int32, (8 * CG // DH, CG), 0) // 8
               == jax.lax.broadcasted_iota(jnp.int32, (8 * CG // DH, CG), 1) // DH)
        zs_buf[slot] = jnp.where(sel, z, 0.0).astype(BF16)

    def a_norm(g):
        for half in range(2):
            for r0 in range(0, HS, CG):
                pq = _ld(pq_buf, (g, half), r0, CG)
                den = _dot_nt(_ld(zs_buf, (g & 1,), 0, 8 * CG // DH), pq) + 1e-6
                rcp = pl.reciprocal(den, approx=True)
                rcp = rcp * (2.0 - den * rcp)
                rcp = jnp.concatenate([rcp[8 * (c // DH):8 * (c // DH) + 8] for c in range(0, CG, 8)], axis=0)
                pq_buf[g, half, pl.ds(r0, CG), :] = (pq.astype(F32) * rcp.T).astype(BF16)
                yield 1

    def a_mix(g):
        for n in range(NG):
            m_buf[n, g] = _dot(_ld(kvbd_buf, (g & 1,), 0, CG), wo_buf[g, :, pl.ds(n * CG, CG)]).astype(BF16)
            yield 1

    def m_terms():
        for t in range(KH):
            for kb in range(KH):
                for r in range(0, CG, RP):
                    blocks = [_ld(m_buf, (b * KH + t, a * KH + kb), r, RP).astype(F32)
                              for a in range(2) for b in range(2)]
                    for i, term in enumerate(_rhs_terms(*blocks)):
                        if i not in (1, 4):
                            ms_buf[t, i, kb, pl.ds(r, RP), :] = term.astype(BF16)
                    yield 1

    def p_terms(sec):
        for r0 in range(max(sec * RO, 2 * RA), (sec + 1) * RO, 2 * RA):
            for kb in range(KH):
                for r in range(0, RA, RP):
                    blocks = [_ld(pq_buf, (b * KH + kb, r0 // HS), r0 % HS + a * RA + r, RP).astype(F32)
                              for a in range(2) for b in range(2)]
                    for i, term in enumerate(_lhs_terms(*blocks)):
                        if i not in (2, 3):
                            ps_buf[sec % 2, i, kb, pl.ds(r0 % RO // 2 + r, RP), :] = term.astype(BF16)
                    yield 1

    def a_out_plain():
        for n in range(NG):
            acc = None
            for g in range(NG):
                part = _dot(_ld(pq_buf, (g, 0), 0, 2 * RA), _ld(m_buf, (n, g), 0, CG))
                acc = part if acc is None else acc + part
                yield 1
            oa_buf[pl.ds(0, 2 * RA), pl.ds(n * CG, CG)] = acc.astype(BF16)
        oa_copy(0).start()

    def a_out(sec):
        for r0 in range(max(sec * RO, 2 * RA), (sec + 1) * RO, 2 * RA):
            for t in range(KH):
                def lhs(i, kb):
                    if i == 2:
                        return _ld(pq_buf, (kb, r0 // HS), r0 % HS, RA)
                    if i == 3:
                        return _ld(pq_buf, (KH + kb, r0 // HS), r0 % HS + RA, RA)
                    return _ld(ps_buf, (sec % 2, i, kb), r0 % RO // 2, RA)

                def rhs(i, kb):
                    if i == 1:
                        return _ld(m_buf, (t, kb), 0, CG)
                    if i == 4:
                        return _ld(m_buf, (KH + t, KH + kb), 0, CG)
                    return _ld(ms_buf, (t, i, kb), 0, CG)

                def emit(a, b, val):
                    oa_buf[pl.ds(r0 + a * RA, RA), pl.ds((b * KH + t) * CG, CG)] = val.astype(BF16)

                yield from _strassen(lhs, rhs, emit)
                if r0 + 2 * RA == S:
                    for b in range(2):
                        last_copy(b * KH + t).start()
            if r0 + 2 * RA < S:
                oa_copy(r0 // (2 * RA)).start()

    def b_pre(g):
        taps = [jnp.concatenate([tap_buf[g, t]] * (RP // 8), axis=0) for t in range(KS)]
        for r0 in range(-PRE_LAG, S, RP):
            if r0 + PRE_LAG < S:
                kf_buf[pl.ds(8 + r0 + PRE_LAG, RP), :] = _ld(k_buf, (g,), r0 + PRE_LAG, RP).astype(F32)
            if r0 < 0:
                continue
            acc = kf_buf[pl.ds(8 + r0, RP), :] * taps[0]
            for t in range(1, KS):
                acc = acc + kf_buf[pl.ds(8 + r0 - t, RP), :] * taps[t]
            kv_buf[g & 3, pl.ds(r0, RP), :] = (acc * _ld(v_buf, (g,), r0, RP).astype(F32)).astype(BF16)
            yield 1

    def spectrum(buf, j, res, factors):
        parts = []
        for r in range(0, 2 * T, 16):
            parts += factors(res[r:r + 8], res[r + 8:r + 16])
        buf[j] = jnp.concatenate(parts, axis=0)

    def b_filter(g):
        for j in range(NC):
            spectrum(hf_buf.at[g & 1], j, _dot_nt(_ld(fwd_ref, (), 0, 2 * T), h_buf[g, :, pl.ds(j * T, T)]),
                     lambda re, im: [re, im - re, re + im])
            yield 1

    def b_signal(g):
        for j in range(NC):
            spectrum(xf_buf.at[g & 1], j, _dot(_ld(fwd_ref, (), 0, 2 * T), _ld(kv_buf, (g & 3,), j * T, T)),
                     lambda re, im: [re + im, re, im])
            yield 1

    def b_mac(g):
        u = g & 1
        for r in range(T // 8):
            rows = [pl.ds(24 * r + o, 8) for o in (0, 8, 16)]
            even = r < T // 16
            prev = None
            for i0 in range(0, NC, NB):
                acc = [None] * NB
                hs = {}
                for j in range(i0 + NB):
                    xs = [xf_buf[u, j, rr, :] for rr in rows]
                    n = 0
                    for a in range(NB):
                        m = i0 + a - j
                        if m < 0:
                            continue
                        if m not in hs:
                            hs[m] = [hf_buf[u, m, rr, :] for rr in rows]
                        ks = [h * x for h, x in zip(hs[m], xs)]
                        acc[a] = ks if acc[a] is None else [c + k for c, k in zip(acc[a], ks)]
                        n += 1
                    yield n
                for a in range(NB):
                    cur = yr, yi = acc[a][0] - acc[a][2], acc[a][0] + acc[a][1]
                    if prev is not None:
                        yr, yi = (yr - prev[1], yi + prev[0]) if even else (yr + prev[1], yi - prev[0])
                    prev = cur
                    yf_buf[u, i0 + a, pl.ds(16 * r, 16), :] = jnp.concatenate([yr, yi], axis=0).astype(BF16)

    def b_post(g):
        dvec = jnp.concatenate([tap_buf[g, KS]] * (T // 8), axis=0)
        for i in range(NC):
            inv = jnp.concatenate([_ld(inv_ref, (0,), 0, T), _ld(inv_ref, (1,), 0, T)], axis=1)
            y = _dot(inv, _ld(yf_buf, (g & 1, i), 0, 2 * T)) + _ld(kv_buf, (g & 3,), i * T, T).astype(F32) * dvec
            ob_buf[g, pl.ds(i * T, T), :] = (_ld(q_buf, (g,), i * T, T).astype(F32) * y).astype(BF16)
            yield 1

    TILE_COST = 7 * KH * HS // 2
    MAIN_COST = 3 * TILE_COST + 2 * HS
    MAC_COST = (T // 8) * NC * (NC + 1) // 2
    PRE_COST = S // RP
    NORM_COST = S // CG
    KB_COST = CG // RP
    all_kb = range(KH)

    def rows_cost(c, n_tiles):
        return n_tiles * 7 * KH * (XB[c + 1] - XB[c]) // 2

    def x_cost(c):
        return (XB[c + 1] - XB[c]) * KH / (2 * RP)

    state = {"todo": [], "n": 0, "zs": [None, None]}
    small = [pltpu.make_async_copy(src, dst, small_sem.at[i]) for i, (src, dst) in enumerate(
        ((shk_hbm, shk_ref), (dd_hbm, dd_ref.at[pl.ds(0, NG)]), (fwd_hbm, fwd_ref), (inv_hbm, inv_ref)))]

    def pair_start(which):
        in_start(0, which)
        in_start(1, which)

    def pair_wait(which):
        in_wait(0, which)
        in_wait(1, which)

    x_copy(0).start()
    pair_start(WQ_IN)
    x_copy(0).wait()
    x_copy(1).start()
    _merge((x_terms(XB[0], XB[1]), 1))
    pair_wait(WQ_IN)
    pair_start(WK_IN)
    _merge((w_terms(0, (0,), all_kb), 1))
    fence()
    _merge((a_main(0, (0,), XB[0], XB[1], state), 1))
    x_copy(1).wait()
    pair_start(WV_IN)
    _merge((x_terms(XB[1], XB[2]), 1))
    fence()
    _merge((a_main(0, (0,), XB[1], XB[2], state), 1))
    pair_wait(WK_IN)
    x_copy(2).start()
    _merge((w_terms(0, (1,), all_kb), 1))
    fence()
    _merge((a_main(0, (1,), XB[0], XB[1], state), 1))
    pair_wait(WV_IN)
    x_copy(3).start()
    fence()
    _merge((a_main(0, (1,), XB[1], XB[2], state), rows_cost(1, 1)), (w_terms(0, (2,), all_kb), KH * KB_COST))
    x_copy(2).wait()
    x_copy(4).start()
    fence()
    _merge((a_main(0, (2,), XB[0], XB[2], state), 2 * rows_cost(0, 1)), (x_terms(XB[2], XB[3]), x_cost(2)))
    x_copy(3).wait()
    x_copy(5).start()
    for c in small:
        c.start()
    fence()
    _merge((a_main(0, (0, 1, 2), XB[2], XB[3], state), rows_cost(2, 3)), (x_terms(XB[3], XB[4]), x_cost(3)))
    x_copy(4).wait()
    in_start(0, K_IN, V_IN)
    fence()
    _merge((a_main(0, (0, 1, 2), XB[3], XB[4], state), rows_cost(3, 3)), (x_terms(XB[4], XB[5]), x_cost(4)))
    x_copy(5).wait()
    in_start(2, *W_IN)
    in_start(3, *W_IN)
    fence()
    state = {"todo": [], "n": 0, "zs": [None, None]}
    a_last(0)
    _merge((a_main(1, (0, 1, 2), 0, XB[5] - HS, state), rows_cost(4, 3)), (x_terms(XB[5], XB[6]), x_cost(5)))
    for c in small:
        c.wait()
    kf_buf[0:8, :] = jnp.zeros((8, CG), F32)
    shk = shk_ref[...].astype(F32)
    dd = dd_ref[0:NG, :].astype(F32)
    for g in range(NG):
        for t in range(KS):
            tap_buf[g, t] = jnp.broadcast_to(shk[t:t + 1, g * CG:(g + 1) * CG], (8, CG))
        tap_buf[g, KS] = jnp.broadcast_to(dd[g:g + 1, :], (8, CG))
    in_wait(0, K_IN, V_IN)
    in_wait(2, *W_IN)
    in_wait(3, *W_IN)
    in_start(0, H_IN)
    in_start(1, K_IN, V_IN)
    in_start(2, K_IN, V_IN)
    fence()
    _merge((a_main(1, (0, 1, 2), XB[5] - HS, HS, state), rows_cost(5, 3)), (b_pre(0), PRE_COST),
           (w_terms(1, range(3), all_kb), 3 * KH * KB_COST))
    in_wait(0, H_IN)
    in_wait(1, K_IN, V_IN)
    in_start(0, WO_IN)
    in_start(1, H_IN)
    fence()
    a_last(1)
    a_heads(0)
    a_heads(1)
    _merge((b_filter(0), NC), (b_signal(0), NC), (b_pre(1), PRE_COST))

    def after_first(stream, *fns):
        yield next(stream)
        for fn in fns:
            fn()
        yield from stream

    def late(stream, cost):
        yield cost
        yield from stream

    for s in range(2, NG):
        in_wait(s - 1, H_IN)
        in_wait(s, K_IN, V_IN)
        in_wait(s - 2, WO_IN)
        if s >= 3:
            in_wait(s - 3, Q_IN)
        if s % 2 == 1 and s + 1 < NG:
            in_wait(s + 1, *W_IN)
            in_wait(s + 2, *W_IN)
        in_start(s, H_IN)
        in_start(s - 1, WO_IN)
        in_start(s - 2, Q_IN)
        if s + 1 < NG:
            in_start(s + 1, K_IN, V_IN)
        else:
            in_start(s, WO_IN)
        if s % 2 == 0 and s + 2 < NG:
            in_start(s + 2, *W_IN)
            in_start(s + 3, *W_IN)
        fence()
        fns = [] if s == 2 else [lambda s=s: a_last(s - 1)]
        if s % 2 == 0 and s > 2:
            fns += [lambda s=s: a_heads(s - 2), lambda s=s: a_heads(s - 1)]
        streams = [(a_main(s), MAIN_COST), (b_mac(s - 2), MAC_RATE * MAC_COST), (b_pre(s), PRE_COST),
                   (after_first(b_filter(s - 1), *fns), NC), (b_signal(s - 1), NC),
                   (late(a_norm(s - 2), NORM_COST / 2), 3 * NORM_COST / 2), (late(a_mix(s - 2), NG / 2), 3 * NG / 2)]
        if s >= 3:
            streams.append((b_post(s - 3), NC))
        if s % 2 == 1 and s + 1 < NG:
            streams.append((w_terms(s // 2 + 1, range(3), all_kb), 3 * KH * KB_COST))
        _merge(*streams)
        if s >= 3:
            ob_copy(s - 3).start()

    g5, g6, g7 = NG - 3, NG - 2, NG - 1
    in_start(g6, Q_IN)
    in_start(g7, Q_IN)
    in_wait(g5, Q_IN)
    in_wait(g6, WO_IN)
    in_wait(g7, WO_IN, H_IN)
    fence()
    SEC_COST = RO // (2 * RA) * KH * 7
    TERMS_COST = RO * KH / (2 * RP)
    mac = b_mac(g6)
    _merge((after_first(b_filter(g7), lambda: a_last(g7), lambda: a_heads(g6), lambda: a_heads(g7)), NC),
           (b_signal(g7), NC), (b_post(g5), NC),
           (late(a_norm(g6), NORM_COST / 3), 4 * NORM_COST / 3), (late(a_norm(g7), NORM_COST / 3), 4 * NORM_COST / 3),
           (late(a_mix(g6), NG / 3), 4 * NG / 3), (late(a_mix(g7), NG / 3), 4 * NG / 3),
           (_take(mac, MAC_COST / 4), MAC_COST / 4))
    ob_copy(g5).start()
    fence()
    _merge((a_out_plain(), NG * NG), (m_terms(), KH * KH * KB_COST), (p_terms(0), (RO - 2 * RA) * KH / (2 * RP)))
    fence()
    _merge((a_out(0), SEC_COST - KH * 7), (mac, MAC_COST * 3 / 4), (p_terms(1), TERMS_COST))
    in_wait(g6, Q_IN)
    in_wait(g7, Q_IN)
    mac = b_mac(g7)
    fence()
    _merge((a_out(1), SEC_COST), (p_terms(2), TERMS_COST), (_take(mac, MAC_COST / 2), MAC_COST / 2),
           (b_post(g6), NC))
    ob_copy(g6).start()
    fence()
    _merge((a_out(2), SEC_COST), (p_terms(3), TERMS_COST), (mac, MAC_COST / 2))
    fence()
    out = a_out(3)
    _merge((b_post(g7), NC), (_take(out, SEC_COST // 2), SEC_COST // 2))
    ob_copy(g7).start()
    _merge((out, 1))
    for g in range(NG):
        ob_copy(g).wait()
    for i in range(S // (2 * RA) - 1):
        oa_copy(i).wait()
    for n in range(NG):
        last_copy(n).wait()


@jax.jit
def pallas_concat_heads__linear_attn_block__ssm_conv_h3__prompt_kernel(
    A_x: jax.Array,
    A_wqkv: jax.Array,
    A_wo: jax.Array,
    B_q: jax.Array,
    B_k: jax.Array,
    B_v: jax.Array,
    B_shift_k: jax.Array,
    B_ssm_k: jax.Array,
    B_ssm_D: jax.Array,
):
    hbm = pl.BlockSpec(memory_space=pl.ANY)
    out = pl.pallas_call(
        _kernel,
        out_shape=jax.ShapeDtypeStruct((S, 2 * D), BF16),
        in_specs=[hbm] * 11,
        out_specs=hbm,
        scratch_shapes=[
            pltpu.VMEM((S, D), BF16),
            pltpu.VMEM((2, 7, KH, HS // 2, CG), BF16),
            pltpu.VMEM((NG, 3, NG, CG, CG), BF16),
            pltpu.VMEM((2, 3, 7, KH, CG, CG), BF16),
            pltpu.VMEM((NG, CG, D), BF16),
            pltpu.VMEM((NG, S, CG), BF16),
            pltpu.VMEM((NG, S, CG), BF16),
            pltpu.VMEM((NG, S, CG), BF16),
            pltpu.VMEM((NG, CG, S), BF16),
            pltpu.VMEM((NG, KS + 1, 8, CG), F32),
            pltpu.VMEM((S + 8, CG), F32),
            pltpu.VMEM((4, S, CG), BF16),
            pltpu.VMEM((2, NC, 3 * T, CG), F32),
            pltpu.VMEM((2, NC, 3 * T, CG), F32),
            pltpu.VMEM((2, NC, 2 * T, CG), BF16),
            pltpu.VMEM((2, HS, CG), BF16),
            pltpu.VMEM((2, HS, CG), BF16),
            pltpu.VMEM((NG, 2, 8, CG), F32),
            pltpu.VMEM((NG, 2, CG, CG), F32),
            pltpu.VMEM((2, 8 * CG // DH, CG), BF16),
            pltpu.VMEM((2, CG, CG), BF16),
            pltpu.VMEM((NG, 2, HS, CG), BF16),
            pltpu.VMEM((2, 7, KH, RO // 2, CG), BF16),
            pltpu.VMEM((NG, NG, CG, CG), BF16),
            pltpu.VMEM((KH, 7, KH, CG, CG), BF16),
            pltpu.VMEM((NG, S, CG), BF16),
            pltpu.VMEM((S, D), BF16),
            pltpu.VMEM(_FWD.shape, BF16),
            pltpu.VMEM(_INV.shape, BF16),
            pltpu.VMEM((KS, D), BF16),
            pltpu.VMEM((2 * NG, CG), BF16),
            pltpu.SemaphoreType.DMA((len(XB) - 1,)),
            pltpu.SemaphoreType.DMA((NG, 8)),
            pltpu.SemaphoreType.DMA((4,)),
            pltpu.SemaphoreType.DMA((NG,)),
            pltpu.SemaphoreType.DMA((S // (2 * RA),)),
            pltpu.SemaphoreType.REGULAR,
        ],
        compiler_params=pltpu.CompilerParams(vmem_limit_bytes=100 * 1024 * 1024, flags=FLAGS),
    )(A_x.reshape(S, D), A_wqkv.reshape(NG, CG, 3 * D), A_wo, B_q.reshape(S, D), B_k.reshape(S, D),
      B_v.reshape(S, D), B_ssm_k, B_shift_k.T, B_ssm_D.reshape(NG, CG), _FWD, _INV)
    return out.reshape(1, S, 2 * D)
```

```python
import jax
import jax.numpy as jnp
import numpy as np
import jax.experimental.pallas as pl
import jax.experimental.pallas.tpu as pltpu

S, D, H = 2048, 1024, 32
DH = D // H
CG = 128
NG = D // CG
T = 128
NC = S // T
KS = 4
NP = NG // 2
HS = S // 2
KH = NG // 2
RA = 64
NB = 2
RP = 32
RO = 512
XB = (0, 256, 512, 768, 1024, 1536, 2048)
LAG_KV = 3072
RF = 256
RI = 128
SHARE = 0.0
MAC_RATE = 1.08
PRE_LAG = 64
FLAGS = None
F32, BF16, U32 = jnp.float32, jnp.bfloat16, jnp.uint32


def _dft_matrices():
    k = np.concatenate([np.arange(0, T, 2), np.arange(1, T, 2)])
    ang = np.pi * (2 * k[:, None] + 1) / (2 * T) * np.arange(T)[None, :]
    re = np.cos(ang).reshape(T // 8, 1, 8, T)
    im = -np.sin(ang).reshape(T // 8, 1, 8, T)
    fwd = np.concatenate([re, im], axis=1).reshape(2 * T, T)
    inv = fwd.T / T
    inv = np.stack([inv[:, :T], inv[:, T:]])
    return fwd.astype(BF16), inv.astype(BF16)


_FWD, _INV = _dft_matrices()


def _dot(a, b):
    return jnp.dot(a, b, preferred_element_type=F32)


def _dot_nt(a, b):
    return jax.lax.dot_general(a, b, (((1,), (1,)), ((), ())), preferred_element_type=F32)


def _dot_tn(a, b):
    return jax.lax.dot_general(a, b, (((0,), (0,)), ((), ())), preferred_element_type=F32)


def _phi(t):
    return jnp.where(t > 0, t + 1.0, jnp.exp(t)) + 1e-6


def _ld(ref, lead, r0, n):
    return pltpu.bitcast(ref.bitcast(U32)[lead + (pl.ds(r0 // 2, n // 2), slice(None))], BF16)


def _merge(*streams):
    done = [0.0] * len(streams)
    live = list(range(len(streams)))
    while live:
        i = min(live, key=lambda s: done[s] / streams[s][1])
        cost = next(streams[i][0], None)
        if cost is None:
            live.remove(i)
        else:
            done[i] += cost


def _take(stream, cost):
    while cost > 0:
        c = next(stream, None)
        if c is None:
            return
        cost -= c
        yield c


def _lhs_terms(a11, a12, a21, a22):
    return a11 + a22, a21 + a22, a11, a22, a11 + a12, a21 - a11, a12 - a22


def _rhs_terms(b11, b12, b21, b22):
    return b11 + b22, b11, b12 - b22, b21 - b11, b22, b11 + b12, b21 + b22


def _strassen(lhs, rhs, emit):
    def prod(i, acc=None):
        for kb in range(KH):
            part = _dot(lhs(i, kb), rhs(i, kb))
            acc = part if acc is None else acc + part
        return acc

    m1 = prod(0)
    yield 1
    m2 = prod(1)
    c22 = m1 - m2
    yield 1
    m4 = prod(3)
    emit(1, 0, m2 + m4)
    c11 = m1 + m4
    yield 1
    m3 = prod(2)
    c22 = c22 + m3
    yield 1
    emit(1, 1, prod(5, c22))
    yield 1
    m5 = prod(4)
    emit(0, 1, m3 + m5)
    c11 = c11 - m5
    yield 1
    emit(0, 0, prod(6, c11))
    yield 1


def _kernel(x_hbm, wqkv_hbm, wo_hbm, q_hbm, k_hbm, v_hbm, h_hbm, shk_hbm, dd_hbm, fwd_hbm, inv_hbm,
            out_hbm,
            x_buf, xs_buf, w_buf, ws_buf, wo_buf, q_buf, k_buf, v_buf, h_buf, tap_buf, kf_buf, kv_buf,
            xf_buf, hf_buf, yf_buf, pk_buf, pv_buf, z_buf, kvs_buf, zrow_buf, zs_buf, kvbd_buf, pq_buf, ps_buf,
            m_buf, ms_buf, ob_buf, oa_buf, fwd_ref, inv_ref, shk_ref, dd_ref,
            x_sem, in_sem, small_sem, ob_sem, oa_sem, fence_sem):

    def rows_of(i, n):
        return i * n if isinstance(i, int) else pl.multiple_of(i * n, n)

    H_IN, K_IN, V_IN, Q_IN, WO_IN, WQ_IN, WK_IN, WV_IN = range(8)
    W_IN = (WQ_IN, WK_IN, WV_IN)

    def in_copy(g, which):
        if which in W_IN:
            t = which - WQ_IN
            src, dst = wqkv_hbm.at[:, :, pl.ds(rows_of(t * NG + g, CG), CG)], w_buf.at[g, t]
        elif which in (H_IN, WO_IN):
            hbm, buf = (h_hbm, h_buf) if which == H_IN else (wo_hbm, wo_buf)
            src, dst = hbm.at[pl.ds(rows_of(g, CG), CG)], buf.at[g]
        else:
            hbm, buf = {K_IN: (k_hbm, k_buf), V_IN: (v_hbm, v_buf), Q_IN: (q_hbm, q_buf)}[which]
            src, dst = hbm.at[:, pl.ds(rows_of(g, CG), CG)], buf.at[g]
        return pltpu.make_async_copy(src, dst, in_sem.at[g, which])

    def in_start(g, *whiches):
        for which in whiches:
            in_copy(g, which).start()

    def in_wait(g, *whiches):
        for which in whiches:
            in_copy(g, which).wait()

    def x_copy(c):
        rows = pl.ds(XB[c], XB[c + 1] - XB[c])
        return pltpu.make_async_copy(x_hbm.at[rows], x_buf.at[rows], x_sem.at[c])

    def ob_copy(g):
        return pltpu.make_async_copy(ob_buf.at[g], out_hbm.at[:, pl.ds(rows_of(NG + g, CG), CG)], ob_sem.at[g])

    def oa_copy(i):
        rows = pl.ds(i * 2 * RA, 2 * RA)
        return pltpu.make_async_copy(oa_buf.at[rows], out_hbm.at[rows, pl.ds(0, D)], oa_sem.at[i])

    def last_copy(n):
        rows, cols = pl.ds(S - 2 * RA, 2 * RA), pl.ds(n * CG, CG)
        return pltpu.make_async_copy(oa_buf.at[rows, cols], out_hbm.at[rows, cols], oa_sem.at[S // (2 * RA) - 1])

    def fence():
        pl.semaphore_signal(fence_sem, 1)
        pl.semaphore_wait(fence_sem, 1)

    def x_terms(r_lo, r_hi):
        for r0 in range(r_lo, r_hi, 2 * RA):
            for kb in range(KH):
                for r in range(0, RA, RP):
                    blocks = [x_buf[pl.ds(r0 + a * RA + r, RP), pl.ds((b * KH + kb) * CG, CG)].astype(F32)
                              for a in range(2) for b in range(2)]
                    for i, term in enumerate(_lhs_terms(*blocks)):
                        xs_buf[r0 // HS, i, kb, pl.ds(r0 % HS // 2 + r, RP), :] = term.astype(BF16)
                    yield 1

    def w_terms(p, tiles, kbs):
        for t in tiles:
            for kb in kbs:
                for r in range(0, CG, RP):
                    blocks = [_ld(w_buf, (2 * p + b, t, a * KH + kb), r, RP).astype(F32)
                              for a in range(2) for b in range(2)]
                    for i, term in enumerate(_rhs_terms(*blocks)):
                        if i not in (1, 4):
                            ws_buf[p & 1, t, i, kb, pl.ds(r, RP), :] = term.astype(BF16)
                    yield 1

    def kv_block(s, j, b):
        kv = _dot_tn(_ld(pk_buf, (j,), b * CG, CG), _ld(pv_buf, (j,), b * CG, CG))
        kvs_buf[s, j] = kv if b == 0 else kvs_buf[s, j] + kv

    def a_main(s, tiles=(0, 1, 2), r_lo=0, r_hi=HS, state=None):
        p, half = s >> 1, s & 1
        state = state or {"todo": [], "n": 0, "zs": [None, None]}
        todo, zs = state["todo"], state["zs"]
        for r0 in range(r_lo, r_hi, 2 * RA):
            for t in tiles:
                def lhs(i, kb):
                    return _ld(xs_buf, (half, i, kb), r0 // 2, RA)

                def rhs(i, kb):
                    if i == 1:
                        return _ld(w_buf, (2 * p, t, kb), 0, CG)
                    if i == 4:
                        return _ld(w_buf, (2 * p + 1, t, KH + kb), 0, CG)
                    return _ld(ws_buf, (p & 1, t, i, kb), 0, CG)

                def emit(a, j, val):
                    rows = pl.ds(r0 + a * RA, RA)
                    if t == 0:
                        pq_buf[2 * p + j, half, rows, :] = _phi(val).astype(BF16)
                    elif t == 1:
                        pk = _phi(val)
                        z = jnp.sum(pk.reshape(RA // 8, 8, CG), axis=0)
                        zs[j] = z if zs[j] is None else zs[j] + z
                        pk_buf[j, rows, :] = pk.astype(BF16)
                    else:
                        pv_buf[j, rows, :] = val.astype(BF16)

                for _ in _strassen(lhs, rhs, emit):
                    state["n"] += KH * RA
                    yield KH * RA
                    if todo and todo[0][0] <= state["n"]:
                        kv_block(s, *todo.pop(0)[1:])
                        yield CG
            if 2 in tiles and (r0 + 2 * RA) % CG == 0 and r0 + 2 * RA < HS:
                todo += [(state["n"] + LAG_KV, j, (r0 + 2 * RA) // CG - 1) for j in range(2)]
        if r_hi == HS:
            for _, j, b in todo:
                kv_block(s, j, b)
            for j in range(2):
                z_buf[s, j] = zs[j]

    def a_last(s):
        for j in range(2):
            kv_block(s, j, HS // CG - 1)

    def a_heads(g):
        s0, j, slot = g >> 1 << 1, g & 1, g & 1
        col_head = jax.lax.broadcasted_iota(jnp.int32, (CG, CG), 1) // DH
        row_head = jax.lax.broadcasted_iota(jnp.int32, (CG, CG), 0) // DH
        kvbd_buf[slot] = jnp.where(row_head == col_head, kvs_buf[s0, j] + kvs_buf[s0 + 1, j], 0.0).astype(BF16)
        z = jnp.sum(z_buf[s0, j] + z_buf[s0 + 1, j], axis=0, keepdims=True)
        zrow_buf[slot] = jnp.broadcast_to(z, (8, CG))
        sel = (jax.lax.broadcasted_iota(jnp.int32, (8 * CG // DH, CG), 0) // 8
               == jax.lax.broadcasted_iota(jnp.int32, (8 * CG // DH, CG), 1) // DH)
        zs_buf[slot] = jnp.where(sel, z, 0.0).astype(BF16)

    def a_norm(g, on_mxu=False):
        z = jnp.concatenate([zrow_buf[g & 1]] * (CG // 8), axis=0)
        for half in range(2):
            for r0 in range(0, HS, CG):
                pq = _ld(pq_buf, (g, half), r0, CG)
                if on_mxu:
                    den = _dot_nt(_ld(zs_buf, (g & 1,), 0, 8 * CG // DH), pq)
                    dens = [den[h:h + 8] for h in range(0, 8 * CG // DH, 8)]
                else:
                    terms = (pq.astype(F32) * z).T
                    dens = []
                    for h in range(0, CG, DH):
                        den = sum(terms[c:c + 8] for c in range(h + 8, h + DH, 8)) + terms[h:h + 8]
                        dens.append(jnp.broadcast_to(jnp.sum(den, axis=0, keepdims=True), (8, CG)))
                rcp = []
                for den in dens:
                    den = den + 1e-6
                    r = pl.reciprocal(den, approx=True)
                    rcp += [r * (2.0 - den * r)] * (DH // 8)
                rcp = jnp.concatenate(rcp, axis=0).T
                pq_buf[g, half, pl.ds(r0, CG), :] = (pq.astype(F32) * rcp).astype(BF16)
                yield 1

    def a_mix(g):
        for n in range(NG):
            m_buf[n, g] = _dot(_ld(kvbd_buf, (g & 1,), 0, CG), wo_buf[g, :, pl.ds(n * CG, CG)]).astype(BF16)
            yield 1

    def m_terms():
        for t in range(KH):
            for kb in range(KH):
                for r in range(0, CG, RP):
                    blocks = [_ld(m_buf, (b * KH + t, a * KH + kb), r, RP).astype(F32)
                              for a in range(2) for b in range(2)]
                    for i, term in enumerate(_rhs_terms(*blocks)):
                        if i not in (1, 4):
                            ms_buf[t, i, kb, pl.ds(r, RP), :] = term.astype(BF16)
                    yield 1

    def p_terms(sec):
        for r0 in range(max(sec * RO, 2 * RA), (sec + 1) * RO, 2 * RA):
            for kb in range(KH):
                for r in range(0, RA, RP):
                    blocks = [_ld(pq_buf, (b * KH + kb, r0 // HS), r0 % HS + a * RA + r, RP).astype(F32)
                              for a in range(2) for b in range(2)]
                    for i, term in enumerate(_lhs_terms(*blocks)):
                        if i not in (2, 3):
                            ps_buf[sec % 2, i, kb, pl.ds(r0 % RO // 2 + r, RP), :] = term.astype(BF16)
                    yield 1

    def a_out_plain():
        for n in range(NG):
            acc = None
            for g in range(NG):
                part = _dot(_ld(pq_buf, (g, 0), 0, 2 * RA), _ld(m_buf, (n, g), 0, CG))
                acc = part if acc is None else acc + part
                yield 1
            oa_buf[pl.ds(0, 2 * RA), pl.ds(n * CG, CG)] = acc.astype(BF16)
        oa_copy(0).start()

    def a_out(sec):
        for r0 in range(max(sec * RO, 2 * RA), (sec + 1) * RO, 2 * RA):
            for t in range(KH):
                def lhs(i, kb):
                    if i == 2:
                        return _ld(pq_buf, (kb, r0 // HS), r0 % HS, RA)
                    if i == 3:
                        return _ld(pq_buf, (KH + kb, r0 // HS), r0 % HS + RA, RA)
                    return _ld(ps_buf, (sec % 2, i, kb), r0 % RO // 2, RA)

                def rhs(i, kb):
                    if i == 1:
                        return _ld(m_buf, (t, kb), 0, CG)
                    if i == 4:
                        return _ld(m_buf, (KH + t, KH + kb), 0, CG)
                    return _ld(ms_buf, (t, i, kb), 0, CG)

                def emit(a, b, val):
                    oa_buf[pl.ds(r0 + a * RA, RA), pl.ds((b * KH + t) * CG, CG)] = val.astype(BF16)

                yield from _strassen(lhs, rhs, emit)
                if r0 + 2 * RA == S:
                    for b in range(2):
                        last_copy(b * KH + t).start()
            if r0 + 2 * RA < S:
                oa_copy(r0 // (2 * RA)).start()

    def b_pre(g):
        taps = [jnp.concatenate([tap_buf[g, t]] * (RP // 8), axis=0) for t in range(KS)]
        for r0 in range(-PRE_LAG, S, RP):
            if r0 + PRE_LAG < S:
                kf_buf[pl.ds(8 + r0 + PRE_LAG, RP), :] = _ld(k_buf, (g,), r0 + PRE_LAG, RP).astype(F32)
            if r0 < 0:
                continue
            acc = kf_buf[pl.ds(8 + r0, RP), :] * taps[0]
            for t in range(1, KS):
                acc = acc + kf_buf[pl.ds(8 + r0 - t, RP), :] * taps[t]
            kv_buf[g & 3, pl.ds(r0, RP), :] = (acc * _ld(v_buf, (g,), r0, RP).astype(F32)).astype(BF16)
            yield 1

    def spectrum(buf, j, f0, res, factors):
        parts = []
        for r in range(0, RF, 16):
            parts += factors(res[r:r + 8], res[r + 8:r + 16])
        buf[j, pl.ds(f0 * 3 // 2, RF * 3 // 2), :] = jnp.concatenate(parts, axis=0)

    def b_filter(g):
        for j in range(NC):
            for f0 in range(0, 2 * T, RF):
                spectrum(hf_buf.at[g & 1], j, f0, _dot_nt(_ld(fwd_ref, (), f0, RF), h_buf[g, :, pl.ds(j * T, T)]),
                         lambda re, im: [re, im - re, re + im])
                yield RF / (2 * T)

    def b_signal(g):
        for j in range(NC):
            for f0 in range(0, 2 * T, RF):
                spectrum(xf_buf.at[g & 1], j, f0, _dot(_ld(fwd_ref, (), f0, RF), _ld(kv_buf, (g & 3,), j * T, T)),
                         lambda re, im: [re + im, re, im])
                yield RF / (2 * T)

    def b_mac(g):
        u = g & 1
        for r in range(T // 8):
            rows = [pl.ds(24 * r + o, 8) for o in (0, 8, 16)]
            even = r < T // 16
            prev = None
            for i0 in range(0, NC, NB):
                acc = [None] * NB
                hs = {}
                for j in range(i0 + NB):
                    xs = [xf_buf[u, j, rr, :] for rr in rows]
                    n = 0
                    for a in range(NB):
                        m = i0 + a - j
                        if m < 0:
                            continue
                        if m not in hs:
                            hs[m] = [hf_buf[u, m, rr, :] for rr in rows]
                        ks = [h * x for h, x in zip(hs[m], xs)]
                        acc[a] = ks if acc[a] is None else [c + k for c, k in zip(acc[a], ks)]
                        n += 1
                    yield n
                for a in range(NB):
                    cur = yr, yi = acc[a][0] - acc[a][2], acc[a][0] + acc[a][1]
                    if prev is not None:
                        yr, yi = (yr - prev[1], yi + prev[0]) if even else (yr + prev[1], yi - prev[0])
                    prev = cur
                    yf_buf[u, i0 + a, pl.ds(16 * r, 16), :] = jnp.concatenate([yr, yi], axis=0).astype(BF16)

    def b_post(g):
        dvec = jnp.concatenate([tap_buf[g, KS]] * (RI // 8), axis=0)
        for i in range(NC):
            for r in range(0, T, RI):
                inv = jnp.concatenate([_ld(inv_ref, (0,), r, RI), _ld(inv_ref, (1,), r, RI)], axis=1)
                y = _dot(inv, _ld(yf_buf, (g & 1, i), 0, 2 * T))
                y = y + _ld(kv_buf, (g & 3,), i * T + r, RI).astype(F32) * dvec
                ob_buf[g, pl.ds(i * T + r, RI), :] = (_ld(q_buf, (g,), i * T + r, RI).astype(F32) * y).astype(BF16)
                yield RI / T

    TILE_COST = 7 * KH * HS // 2
    MAIN_COST = 3 * TILE_COST + 2 * HS
    MAC_COST = (T // 8) * NC * (NC + 1) // 2
    PRE_COST = S // RP
    NORM_COST = S // CG
    KB_COST = CG // RP
    all_kb = range(KH)

    def rows_cost(c, n_tiles):
        return n_tiles * 7 * KH * (XB[c + 1] - XB[c]) // 2

    def x_cost(c):
        return (XB[c + 1] - XB[c]) * KH / (2 * RP)

    state = {"todo": [], "n": 0, "zs": [None, None]}
    small = [pltpu.make_async_copy(src, dst, small_sem.at[i]) for i, (src, dst) in enumerate(
        ((shk_hbm, shk_ref), (dd_hbm, dd_ref.at[pl.ds(0, NG)]), (fwd_hbm, fwd_ref), (inv_hbm, inv_ref)))]

    def pair_start(which):
        in_start(0, which)
        in_start(1, which)

    def pair_wait(which):
        in_wait(0, which)
        in_wait(1, which)

    x_copy(0).start()
    pair_start(WQ_IN)
    x_copy(0).wait()
    x_copy(1).start()
    _merge((x_terms(XB[0], XB[1]), 1))
    pair_wait(WQ_IN)
    pair_start(WK_IN)
    _merge((w_terms(0, (0,), all_kb), 1))
    fence()
    _merge((a_main(0, (0,), XB[0], XB[1], state), 1))
    x_copy(1).wait()
    pair_start(WV_IN)
    _merge((x_terms(XB[1], XB[2]), 1))
    fence()
    _merge((a_main(0, (0,), XB[1], XB[2], state), 1))
    pair_wait(WK_IN)
    x_copy(2).start()
    _merge((w_terms(0, (1,), all_kb), 1))
    fence()
    _merge((a_main(0, (1,), XB[0], XB[1], state), 1))
    pair_wait(WV_IN)
    x_copy(3).start()
    fence()
    _merge((a_main(0, (1,), XB[1], XB[2], state), rows_cost(1, 1)), (w_terms(0, (2,), all_kb), KH * KB_COST))
    x_copy(2).wait()
    x_copy(4).start()
    fence()
    _merge((a_main(0, (2,), XB[0], XB[2], state), 2 * rows_cost(0, 1)), (x_terms(XB[2], XB[3]), x_cost(2)))
    x_copy(3).wait()
    x_copy(5).start()
    for c in small:
        c.start()
    fence()
    _merge((a_main(0, (0, 1, 2), XB[2], XB[3], state), rows_cost(2, 3)), (x_terms(XB[3], XB[4]), x_cost(3)))
    x_copy(4).wait()
    in_start(0, K_IN, V_IN)
    fence()
    _merge((a_main(0, (0, 1, 2), XB[3], XB[4], state), rows_cost(3, 3)), (x_terms(XB[4], XB[5]), x_cost(4)))
    x_copy(5).wait()
    in_start(2, *W_IN)
    in_start(3, *W_IN)
    fence()
    state = {"todo": [], "n": 0, "zs": [None, None]}
    a_last(0)
    _merge((a_main(1, (0, 1, 2), 0, XB[5] - HS, state), rows_cost(4, 3)), (x_terms(XB[5], XB[6]), x_cost(5)))
    for c in small:
        c.wait()
    kf_buf[0:8, :] = jnp.zeros((8, CG), F32)
    shk = shk_ref[...].astype(F32)
    dd = dd_ref[0:NG, :].astype(F32)
    for g in range(NG):
        for t in range(KS):
            tap_buf[g, t] = jnp.broadcast_to(shk[t:t + 1, g * CG:(g + 1) * CG], (8, CG))
        tap_buf[g, KS] = jnp.broadcast_to(dd[g:g + 1, :], (8, CG))
    in_wait(0, K_IN, V_IN)
    in_wait(2, *W_IN)
    in_wait(3, *W_IN)
    in_start(0, H_IN)
    in_start(1, K_IN, V_IN)
    in_start(2, K_IN, V_IN)
    fence()
    _merge((a_main(1, (0, 1, 2), XB[5] - HS, HS, state), rows_cost(5, 3)), (b_pre(0), PRE_COST),
           (w_terms(1, range(3), all_kb), 3 * KH * KB_COST))
    in_wait(0, H_IN)
    in_wait(1, K_IN, V_IN)
    in_start(0, WO_IN)
    in_start(1, H_IN)
    fence()
    a_last(1)
    a_heads(0)
    a_heads(1)
    _merge((b_filter(0), NC), (b_signal(0), NC), (b_pre(1), PRE_COST))

    def after_first(stream, *fns):
        yield next(stream)
        for fn in fns:
            fn()
        yield from stream

    def late(stream, cost):
        yield cost
        yield from stream

    for s in range(2, NG):
        in_wait(s - 1, H_IN)
        in_wait(s, K_IN, V_IN)
        in_wait(s - 2, WO_IN)
        if s >= 3:
            in_wait(s - 3, Q_IN)
        if s % 2 == 1 and s + 1 < NG:
            in_wait(s + 1, *W_IN)
            in_wait(s + 2, *W_IN)
        in_start(s, H_IN)
        in_start(s - 1, WO_IN)
        in_start(s - 2, Q_IN)
        if s + 1 < NG:
            in_start(s + 1, K_IN, V_IN)
        else:
            in_start(s, WO_IN)
        if s % 2 == 0 and s + 2 < NG:
            in_start(s + 2, *W_IN)
            in_start(s + 3, *W_IN)
        fence()
        fns = [] if s == 2 else [lambda s=s: a_last(s - 1)]
        if s % 2 == 0 and s > 2:
            fns += [lambda s=s: a_heads(s - 2), lambda s=s: a_heads(s - 1)]
        streams = [(a_main(s), MAIN_COST), (b_mac(s - 2), MAC_RATE * MAC_COST), (b_pre(s), PRE_COST),
                   (after_first(b_filter(s - 1), *fns), NC), (b_signal(s - 1), NC),
                   (late(a_norm(s - 2), NORM_COST / 2), 3 * NORM_COST / 2), (late(a_mix(s - 2), NG / 2), 3 * NG / 2)]
        if s >= 3:
            streams.append((b_post(s - 3), NC))
        if s % 2 == 1 and s + 1 < NG:
            streams.append((w_terms(s // 2 + 1, range(3), all_kb), 3 * KH * KB_COST))
        _merge(*streams)
        if s >= 3:
            ob_copy(s - 3).start()

    g5, g6, g7 = NG - 3, NG - 2, NG - 1
    in_start(g6, Q_IN)
    in_start(g7, Q_IN)
    in_wait(g5, Q_IN)
    in_wait(g6, WO_IN)
    in_wait(g7, WO_IN, H_IN)
    fence()
    SEC_COST = RO // (2 * RA) * KH * 7
    TERMS_COST = RO * KH / (2 * RP)
    mac = b_mac(g6)
    _merge((after_first(b_filter(g7), lambda: a_last(g7), lambda: a_heads(g6), lambda: a_heads(g7)), NC),
           (b_signal(g7), NC), (b_post(g5), NC),
           (late(a_norm(g6, True), NORM_COST / 3), 4 * NORM_COST / 3), (late(a_norm(g7, True), NORM_COST / 3), 4 * NORM_COST / 3),
           (late(a_mix(g6), NG / 3), 4 * NG / 3), (late(a_mix(g7), NG / 3), 4 * NG / 3),
           (_take(mac, MAC_COST / 4), MAC_COST / 4))
    ob_copy(g5).start()
    fence()
    _merge((a_out_plain(), NG * NG), (m_terms(), KH * KH * KB_COST), (p_terms(0), (RO - 2 * RA) * KH / (2 * RP)))
    fence()
    _merge((a_out(0), SEC_COST - KH * 7), (mac, MAC_COST * 3 / 4), (p_terms(1), TERMS_COST))
    in_wait(g6, Q_IN)
    in_wait(g7, Q_IN)
    mac = b_mac(g7)
    fence()
    _merge((a_out(1), SEC_COST), (p_terms(2), TERMS_COST), (_take(mac, MAC_COST * SHARE), MAC_COST * SHARE + 1e-3),
           (b_post(g6), NC))
    ob_copy(g6).start()
    fence()
    _merge((a_out(2), SEC_COST), (p_terms(3), TERMS_COST), (mac, MAC_COST * (1 - SHARE)))
    fence()
    out = a_out(3)
    _merge((b_post(g7), NC), (_take(out, SEC_COST // 2), SEC_COST // 2))
    ob_copy(g7).start()
    _merge((out, 1))
    for g in range(NG):
        ob_copy(g).wait()
    for i in range(S // (2 * RA) - 1):
        oa_copy(i).wait()
    for n in range(NG):
        last_copy(n).wait()


@jax.jit
def pallas_concat_heads__linear_attn_block__ssm_conv_h3__prompt_kernel(
    A_x: jax.Array,
    A_wqkv: jax.Array,
    A_wo: jax.Array,
    B_q: jax.Array,
    B_k: jax.Array,
    B_v: jax.Array,
    B_shift_k: jax.Array,
    B_ssm_k: jax.Array,
    B_ssm_D: jax.Array,
):
    hbm = pl.BlockSpec(memory_space=pl.ANY)
    out = pl.pallas_call(
        _kernel,
        out_shape=jax.ShapeDtypeStruct((S, 2 * D), BF16),
        in_specs=[hbm] * 11,
        out_specs=hbm,
        scratch_shapes=[
            pltpu.VMEM((S, D), BF16),
            pltpu.VMEM((2, 7, KH, HS // 2, CG), BF16),
            pltpu.VMEM((NG, 3, NG, CG, CG), BF16),
            pltpu.VMEM((2, 3, 7, KH, CG, CG), BF16),
            pltpu.VMEM((NG, CG, D), BF16),
            pltpu.VMEM((NG, S, CG), BF16),
            pltpu.VMEM((NG, S, CG), BF16),
            pltpu.VMEM((NG, S, CG), BF16),
            pltpu.VMEM((NG, CG, S), BF16),
            pltpu.VMEM((NG, KS + 1, 8, CG), F32),
            pltpu.VMEM((S + 8, CG), F32),
            pltpu.VMEM((4, S, CG), BF16),
            pltpu.VMEM((2, NC, 3 * T, CG), F32),
            pltpu.VMEM((2, NC, 3 * T, CG), F32),
            pltpu.VMEM((2, NC, 2 * T, CG), BF16),
            pltpu.VMEM((2, HS, CG), BF16),
            pltpu.VMEM((2, HS, CG), BF16),
            pltpu.VMEM((NG, 2, 8, CG), F32),
            pltpu.VMEM((NG, 2, CG, CG), F32),
            pltpu.VMEM((2, 8, CG), F32),
            pltpu.VMEM((2, 8 * CG // DH, CG), BF16),
            pltpu.VMEM((2, CG, CG), BF16),
            pltpu.VMEM((NG, 2, HS, CG), BF16),
            pltpu.VMEM((2, 7, KH, RO // 2, CG), BF16),
            pltpu.VMEM((NG, NG, CG, CG), BF16),
            pltpu.VMEM((KH, 7, KH, CG, CG), BF16),
            pltpu.VMEM((NG, S, CG), BF16),
            pltpu.VMEM((S, D), BF16),
            pltpu.VMEM(_FWD.shape, BF16),
            pltpu.VMEM(_INV.shape, BF16),
            pltpu.VMEM((KS, D), BF16),
            pltpu.VMEM((2 * NG, CG), BF16),
            pltpu.SemaphoreType.DMA((len(XB) - 1,)),
            pltpu.SemaphoreType.DMA((NG, 8)),
            pltpu.SemaphoreType.DMA((4,)),
            pltpu.SemaphoreType.DMA((NG,)),
            pltpu.SemaphoreType.DMA((S // (2 * RA),)),
            pltpu.SemaphoreType.REGULAR,
        ],
        compiler_params=pltpu.CompilerParams(vmem_limit_bytes=100 * 1024 * 1024, flags=FLAGS),
    )(A_x.reshape(S, D), A_wqkv.reshape(NG, CG, 3 * D), A_wo, B_q.reshape(S, D), B_k.reshape(S, D),
      B_v.reshape(S, D), B_ssm_k, B_shift_k.T, B_ssm_D.reshape(NG, CG), _FWD, _INV)
    return out.reshape(1, S, 2 * D)
```

```python
import jax
import jax.numpy as jnp
import numpy as np
import jax.experimental.pallas as pl
import jax.experimental.pallas.tpu as pltpu

S, D, H = 2048, 1024, 32
DH = D // H
CG = 128
NG = D // CG
T = 128
NC = S // T
KS = 4
NP = NG // 2
HS = S // 2
KH = NG // 2
RA = 64
NB = 2
RP = 32
RO = 512
XB = (0, 256, 512, 768, 1024, 1536, 2048)
LAG_KV = 3072
MAC_RATE = 1.08
PRE_LAG = 64
FLAGS = None
F32, BF16, U32 = jnp.float32, jnp.bfloat16, jnp.uint32


def _dft_matrices():
    k = np.concatenate([np.arange(0, T, 2), np.arange(1, T, 2)])
    ang = np.pi * (2 * k[:, None] + 1) / (2 * T) * np.arange(T)[None, :]
    re = np.cos(ang).reshape(T // 8, 1, 8, T)
    im = -np.sin(ang).reshape(T // 8, 1, 8, T)
    fwd = np.concatenate([re, im], axis=1).reshape(2 * T, T)
    inv = fwd.T / T
    inv = np.stack([inv[:, :T], inv[:, T:]])
    return fwd.astype(BF16), inv.astype(BF16)


_FWD, _INV = _dft_matrices()


def _dot(a, b):
    return jnp.dot(a, b, preferred_element_type=F32)


def _dot_nt(a, b):
    return jax.lax.dot_general(a, b, (((1,), (1,)), ((), ())), preferred_element_type=F32)


def _dot_tn(a, b):
    return jax.lax.dot_general(a, b, (((0,), (0,)), ((), ())), preferred_element_type=F32)


def _phi(t):
    return jnp.where(t > 0, t + 1.0, jnp.exp(t)) + 1e-6


def _ld(ref, lead, r0, n):
    return pltpu.bitcast(ref.bitcast(U32)[lead + (pl.ds(r0 // 2, n // 2), slice(None))], BF16)


def _merge(*streams):
    done = [0.0] * len(streams)
    live = list(range(len(streams)))
    while live:
        i = min(live, key=lambda s: done[s] / streams[s][1])
        cost = next(streams[i][0], None)
        if cost is None:
            live.remove(i)
        else:
            done[i] += cost


def _take(stream, cost):
    while cost > 0:
        c = next(stream, None)
        if c is None:
            return
        cost -= c
        yield c


def _lhs_terms(a11, a12, a21, a22):
    return a11 + a22, a21 + a22, a11, a22, a11 + a12, a21 - a11, a12 - a22


def _rhs_terms(b11, b12, b21, b22):
    return b11 + b22, b11, b12 - b22, b21 - b11, b22, b11 + b12, b21 + b22


def _strassen(lhs, rhs, emit):
    def prod(i, acc=None):
        for kb in range(KH):
            part = _dot(lhs(i, kb), rhs(i, kb))
            acc = part if acc is None else acc + part
        return acc

    m1 = prod(0)
    yield 1
    m2 = prod(1)
    c22 = m1 - m2
    yield 1
    m4 = prod(3)
    emit(1, 0, m2 + m4)
    c11 = m1 + m4
    yield 1
    m3 = prod(2)
    c22 = c22 + m3
    yield 1
    emit(1, 1, prod(5, c22))
    yield 1
    m5 = prod(4)
    emit(0, 1, m3 + m5)
    c11 = c11 - m5
    yield 1
    emit(0, 0, prod(6, c11))
    yield 1


def _kernel(x_hbm, wqkv_hbm, wo_hbm, q_hbm, k_hbm, v_hbm, h_hbm, shk_hbm, dd_hbm, fwd_hbm, inv_hbm,
            out_hbm,
            x_buf, xs_buf, w_buf, ws_buf, wo_buf, q_buf, k_buf, v_buf, h_buf, tap_buf, kf_buf, kv_buf,
            xf_buf, hf_buf, yf_buf, pk_buf, pv_buf, z_buf, kvs_buf, zrow_buf, zs_buf, kvbd_buf, pq_buf, ps_buf,
            m_buf, ms_buf, ob_buf, oa_buf, fwd_ref, inv_ref, shk_ref, dd_ref,
            x_sem, in_sem, small_sem, ob_sem, oa_sem, fence_sem):

    def rows_of(i, n):
        return i * n if isinstance(i, int) else pl.multiple_of(i * n, n)

    H_IN, K_IN, V_IN, Q_IN, WO_IN, WQ_IN, WK_IN, WV_IN = range(8)
    W_IN = (WQ_IN, WK_IN, WV_IN)

    def in_copy(g, which):
        if which in W_IN:
            t = which - WQ_IN
            src, dst = wqkv_hbm.at[:, :, pl.ds(rows_of(t * NG + g, CG), CG)], w_buf.at[g, t]
        elif which in (H_IN, WO_IN):
            hbm, buf = (h_hbm, h_buf) if which == H_IN else (wo_hbm, wo_buf)
            src, dst = hbm.at[pl.ds(rows_of(g, CG), CG)], buf.at[g]
        else:
            hbm, buf = {K_IN: (k_hbm, k_buf), V_IN: (v_hbm, v_buf), Q_IN: (q_hbm, q_buf)}[which]
            src, dst = hbm.at[:, pl.ds(rows_of(g, CG), CG)], buf.at[g]
        return pltpu.make_async_copy(src, dst, in_sem.at[g, which])

    def in_start(g, *whiches):
        for which in whiches:
            in_copy(g, which).start()

    def in_wait(g, *whiches):
        for which in whiches:
            in_copy(g, which).wait()

    def x_copy(c):
        rows = pl.ds(XB[c], XB[c + 1] - XB[c])
        return pltpu.make_async_copy(x_hbm.at[rows], x_buf.at[rows], x_sem.at[c])

    def ob_copy(g):
        return pltpu.make_async_copy(ob_buf.at[g], out_hbm.at[:, pl.ds(rows_of(NG + g, CG), CG)], ob_sem.at[g])

    def oa_copy(i):
        rows = pl.ds(i * 2 * RA, 2 * RA)
        return pltpu.make_async_copy(oa_buf.at[rows], out_hbm.at[rows, pl.ds(0, D)], oa_sem.at[i])

    def last_copy(n):
        rows, cols = pl.ds(S - 2 * RA, 2 * RA), pl.ds(n * CG, CG)
        return pltpu.make_async_copy(oa_buf.at[rows, cols], out_hbm.at[rows, cols], oa_sem.at[S // (2 * RA) - 1])

    def fence():
        pl.semaphore_signal(fence_sem, 1)
        pl.semaphore_wait(fence_sem, 1)

    def x_terms(r_lo, r_hi):
        for r0 in range(r_lo, r_hi, 2 * RA):
            for kb in range(KH):
                for r in range(0, RA, RP):
                    blocks = [x_buf[pl.ds(r0 + a * RA + r, RP), pl.ds((b * KH + kb) * CG, CG)].astype(F32)
                              for a in range(2) for b in range(2)]
                    for i, term in enumerate(_lhs_terms(*blocks)):
                        xs_buf[r0 // HS, i, kb, pl.ds(r0 % HS // 2 + r, RP), :] = term.astype(BF16)
                    yield 1

    def w_terms(p, tiles, kbs):
        for t in tiles:
            for kb in kbs:
                for r in range(0, CG, RP):
                    blocks = [_ld(w_buf, (2 * p + b, t, a * KH + kb), r, RP).astype(F32)
                              for a in range(2) for b in range(2)]
                    for i, term in enumerate(_rhs_terms(*blocks)):
                        if i not in (1, 4):
                            ws_buf[p & 1, t, i, kb, pl.ds(r, RP), :] = term.astype(BF16)
                    yield 1

    def kv_block(s, j, b):
        kv = _dot_tn(_ld(pk_buf, (j,), b * CG, CG), _ld(pv_buf, (j,), b * CG, CG))
        kvs_buf[s, j] = kv if b == 0 else kvs_buf[s, j] + kv

    def a_main(s, tiles=(0, 1, 2), r_lo=0, r_hi=HS, state=None):
        p, half = s >> 1, s & 1
        state = state or {"todo": [], "n": 0, "zs": [None, None]}
        todo, zs = state["todo"], state["zs"]
        for r0 in range(r_lo, r_hi, 2 * RA):
            for t in tiles:
                def lhs(i, kb):
                    return _ld(xs_buf, (half, i, kb), r0 // 2, RA)

                def rhs(i, kb):
                    if i == 1:
                        return _ld(w_buf, (2 * p, t, kb), 0, CG)
                    if i == 4:
                        return _ld(w_buf, (2 * p + 1, t, KH + kb), 0, CG)
                    return _ld(ws_buf, (p & 1, t, i, kb), 0, CG)

                def emit(a, j, val):
                    rows = pl.ds(r0 + a * RA, RA)
                    if t == 0:
                        pq_buf[2 * p + j, half, rows, :] = _phi(val).astype(BF16)
                    elif t == 1:
                        pk = _phi(val)
                        z = jnp.sum(pk.reshape(RA // 8, 8, CG), axis=0)
                        zs[j] = z if zs[j] is None else zs[j] + z
                        pk_buf[j, rows, :] = pk.astype(BF16)
                    else:
                        pv_buf[j, rows, :] = val.astype(BF16)

                for _ in _strassen(lhs, rhs, emit):
                    state["n"] += KH * RA
                    yield KH * RA
                    if todo and todo[0][0] <= state["n"]:
                        kv_block(s, *todo.pop(0)[1:])
                        yield CG
            if 2 in tiles and (r0 + 2 * RA) % CG == 0 and r0 + 2 * RA < HS:
                todo += [(state["n"] + LAG_KV, j, (r0 + 2 * RA) // CG - 1) for j in range(2)]
        if r_hi == HS:
            for _, j, b in todo:
                kv_block(s, j, b)
            for j in range(2):
                z_buf[s, j] = zs[j]

    def a_last(s):
        for j in range(2):
            kv_block(s, j, HS // CG - 1)

    def a_heads(g):
        s0, j, slot = g >> 1 << 1, g & 1, g & 1
        col_head = jax.lax.broadcasted_iota(jnp.int32, (CG, CG), 1) // DH
        row_head = jax.lax.broadcasted_iota(jnp.int32, (CG, CG), 0) // DH
        kvbd_buf[slot] = jnp.where(row_head == col_head, kvs_buf[s0, j] + kvs_buf[s0 + 1, j], 0.0).astype(BF16)
        z = jnp.sum(z_buf[s0, j] + z_buf[s0 + 1, j], axis=0, keepdims=True)
        zrow_buf[slot] = jnp.broadcast_to(z, (8, CG))
        sel = (jax.lax.broadcasted_iota(jnp.int32, (8 * CG // DH, CG), 0) // 8
               == jax.lax.broadcasted_iota(jnp.int32, (8 * CG // DH, CG), 1) // DH)
        zs_buf[slot] = jnp.where(sel, z, 0.0).astype(BF16)

    def a_norm(g, on_mxu=False):
        z = jnp.concatenate([zrow_buf[g & 1]] * (CG // 8), axis=0)
        for half in range(2):
            for r0 in range(0, HS, CG):
                pq = _ld(pq_buf, (g, half), r0, CG)
                if on_mxu:
                    den = _dot_nt(_ld(zs_buf, (g & 1,), 0, 8 * CG // DH), pq)
                    dens = [den[h:h + 8] for h in range(0, 8 * CG // DH, 8)]
                else:
                    terms = (pq.astype(F32) * z).T
                    dens = []
                    for h in range(0, CG, DH):
                        den = sum(terms[c:c + 8] for c in range(h + 8, h + DH, 8)) + terms[h:h + 8]
                        dens.append(jnp.broadcast_to(jnp.sum(den, axis=0, keepdims=True), (8, CG)))
                rcp = []
                for den in dens:
                    den = den + 1e-6
                    r = pl.reciprocal(den, approx=True)
                    rcp += [r * (2.0 - den * r)] * (DH // 8)
                rcp = jnp.concatenate(rcp, axis=0).T
                pq_buf[g, half, pl.ds(r0, CG), :] = (pq.astype(F32) * rcp).astype(BF16)
                yield 1

    def a_mix(g):
        for n in range(NG):
            m_buf[n, g] = _dot(_ld(kvbd_buf, (g & 1,), 0, CG), wo_buf[g, :, pl.ds(n * CG, CG)]).astype(BF16)
            yield 1

    def m_terms():
        for t in range(KH):
            for kb in range(KH):
                for r in range(0, CG, RP):
                    blocks = [_ld(m_buf, (b * KH + t, a * KH + kb), r, RP).astype(F32)
                              for a in range(2) for b in range(2)]
                    for i, term in enumerate(_rhs_terms(*blocks)):
                        if i not in (1, 4):
                            ms_buf[t, i, kb, pl.ds(r, RP), :] = term.astype(BF16)
                    yield 1

    def p_terms(sec):
        for r0 in range(max(sec * RO, 2 * RA), (sec + 1) * RO, 2 * RA):
            for kb in range(KH):
                for r in range(0, RA, RP):
                    blocks = [_ld(pq_buf, (b * KH + kb, r0 // HS), r0 % HS + a * RA + r, RP).astype(F32)
                              for a in range(2) for b in range(2)]
                    for i, term in enumerate(_lhs_terms(*blocks)):
                        if i not in (2, 3):
                            ps_buf[sec % 2, i, kb, pl.ds(r0 % RO // 2 + r, RP), :] = term.astype(BF16)
                    yield 1

    def a_out_plain():
        for n in range(NG):
            acc = None
            for g in range(NG):
                part = _dot(_ld(pq_buf, (g, 0), 0, 2 * RA), _ld(m_buf, (n, g), 0, CG))
                acc = part if acc is None else acc + part
                yield 1
            oa_buf[pl.ds(0, 2 * RA), pl.ds(n * CG, CG)] = acc.astype(BF16)
        oa_copy(0).start()

    def a_out(sec):
        for r0 in range(max(sec * RO, 2 * RA), (sec + 1) * RO, 2 * RA):
            for t in range(KH):
                def lhs(i, kb):
                    if i == 2:
                        return _ld(pq_buf, (kb, r0 // HS), r0 % HS, RA)
                    if i == 3:
                        return _ld(pq_buf, (KH + kb, r0 // HS), r0 % HS + RA, RA)
                    return _ld(ps_buf, (sec % 2, i, kb), r0 % RO // 2, RA)

                def rhs(i, kb):
                    if i == 1:
                        return _ld(m_buf, (t, kb), 0, CG)
                    if i == 4:
                        return _ld(m_buf, (KH + t, KH + kb), 0, CG)
                    return _ld(ms_buf, (t, i, kb), 0, CG)

                def emit(a, b, val):
                    oa_buf[pl.ds(r0 + a * RA, RA), pl.ds((b * KH + t) * CG, CG)] = val.astype(BF16)

                yield from _strassen(lhs, rhs, emit)
                if r0 + 2 * RA == S:
                    for b in range(2):
                        last_copy(b * KH + t).start()
            if r0 + 2 * RA < S:
                oa_copy(r0 // (2 * RA)).start()

    def b_pre(g):
        taps = [jnp.concatenate([tap_buf[g, t]] * (RP // 8), axis=0) for t in range(KS)]
        for r0 in range(-PRE_LAG, S, RP):
            if r0 + PRE_LAG < S:
                kf_buf[pl.ds(8 + r0 + PRE_LAG, RP), :] = _ld(k_buf, (g,), r0 + PRE_LAG, RP).astype(F32)
            if r0 < 0:
                continue
            acc = kf_buf[pl.ds(8 + r0, RP), :] * taps[0]
            for t in range(1, KS):
                acc = acc + kf_buf[pl.ds(8 + r0 - t, RP), :] * taps[t]
            kv_buf[g & 3, pl.ds(r0, RP), :] = (acc * _ld(v_buf, (g,), r0, RP).astype(F32)).astype(BF16)
            yield 1

    def spectrum(buf, j, res, factors):
        parts = []
        for r in range(0, 2 * T, 16):
            parts += factors(res[r:r + 8], res[r + 8:r + 16])
        buf[j] = jnp.concatenate(parts, axis=0)

    def b_filter(g):
        for j in range(NC):
            res = _dot_nt(_ld(fwd_ref, (), 0, 2 * T), h_buf[g, :, pl.ds(j * T, T)])
            spectrum(hf_buf.at[g % 2], j, res, lambda re, im: [re, im - re, re + im])
            yield 1

    def b_signal(g):
        for j in range(NC):
            res = _dot(_ld(fwd_ref, (), 0, 2 * T), _ld(kv_buf, (g % 4,), j * T, T))
            spectrum(xf_buf.at[g % 2], j, res, lambda re, im: [re + im, re, im])
            yield 1

    def b_mac(g):
        u = g & 1
        for r in range(T // 8):
            rows = [pl.ds(24 * r + o, 8) for o in (0, 8, 16)]
            even = r < T // 16
            prev = None
            for i0 in range(0, NC, NB):
                acc = [None] * NB
                hs = {}
                for j in range(i0 + NB):
                    xs = [xf_buf[u, j, rr, :] for rr in rows]
                    n = 0
                    for a in range(NB):
                        m = i0 + a - j
                        if m < 0:
                            continue
                        if m not in hs:
                            hs[m] = [hf_buf[u, m, rr, :] for rr in rows]
                        ks = [h * x for h, x in zip(hs[m], xs)]
                        acc[a] = ks if acc[a] is None else [c + k for c, k in zip(acc[a], ks)]
                        n += 1
                    yield n
                for a in range(NB):
                    cur = yr, yi = acc[a][0] - acc[a][2], acc[a][0] + acc[a][1]
                    if prev is not None:
                        yr, yi = (yr - prev[1], yi + prev[0]) if even else (yr + prev[1], yi - prev[0])
                    prev = cur
                    yf_buf[u, i0 + a, pl.ds(16 * r, 16), :] = jnp.concatenate([yr, yi], axis=0).astype(BF16)

    def b_post(g):
        dvec = jnp.concatenate([tap_buf[g, KS]] * (T // 8), axis=0)
        for i in range(NC):
            inv = jnp.concatenate([_ld(inv_ref, (0,), 0, T), _ld(inv_ref, (1,), 0, T)], axis=1)
            y = _dot(inv, _ld(yf_buf, (g % 2, i), 0, 2 * T)) + _ld(kv_buf, (g % 4,), i * T, T).astype(F32) * dvec
            ob_buf[g, pl.ds(i * T, T), :] = (_ld(q_buf, (g,), i * T, T).astype(F32) * y).astype(BF16)
            yield 1

    TILE_COST = 7 * KH * HS // 2
    MAIN_COST = 3 * TILE_COST + 2 * HS
    MAC_COST = (T // 8) * NC * (NC + 1) // 2
    PRE_COST = S // RP
    NORM_COST = S // CG
    KB_COST = CG // RP
    all_kb = range(KH)

    def rows_cost(c, n_tiles):
        return n_tiles * 7 * KH * (XB[c + 1] - XB[c]) // 2

    def x_cost(c):
        return (XB[c + 1] - XB[c]) * KH / (2 * RP)

    state = {"todo": [], "n": 0, "zs": [None, None]}
    small = [pltpu.make_async_copy(src, dst, small_sem.at[i]) for i, (src, dst) in enumerate(
        ((shk_hbm, shk_ref), (dd_hbm, dd_ref.at[pl.ds(0, NG)]), (fwd_hbm, fwd_ref), (inv_hbm, inv_ref)))]

    def pair_start(which):
        in_start(0, which)
        in_start(1, which)

    def pair_wait(which):
        in_wait(0, which)
        in_wait(1, which)

    x_copy(0).start()
    pair_start(WQ_IN)
    x_copy(0).wait()
    x_copy(1).start()
    _merge((x_terms(XB[0], XB[1]), 1))
    pair_wait(WQ_IN)
    pair_start(WK_IN)
    _merge((w_terms(0, (0,), all_kb), 1))
    fence()
    _merge((a_main(0, (0,), XB[0], XB[1], state), 1))
    x_copy(1).wait()
    pair_start(WV_IN)
    _merge((x_terms(XB[1], XB[2]), 1))
    fence()
    _merge((a_main(0, (0,), XB[1], XB[2], state), 1))
    pair_wait(WK_IN)
    x_copy(2).start()
    _merge((w_terms(0, (1,), all_kb), 1))
    fence()
    _merge((a_main(0, (1,), XB[0], XB[1], state), 1))
    pair_wait(WV_IN)
    x_copy(3).start()
    fence()
    _merge((a_main(0, (1,), XB[1], XB[2], state), rows_cost(1, 1)), (w_terms(0, (2,), all_kb), KH * KB_COST))
    x_copy(2).wait()
    x_copy(4).start()
    fence()
    _merge((a_main(0, (2,), XB[0], XB[2], state), 2 * rows_cost(0, 1)), (x_terms(XB[2], XB[3]), x_cost(2)))
    x_copy(3).wait()
    x_copy(5).start()
    for c in small:
        c.start()
    fence()
    _merge((a_main(0, (0, 1, 2), XB[2], XB[3], state), rows_cost(2, 3)), (x_terms(XB[3], XB[4]), x_cost(3)))
    x_copy(4).wait()
    in_start(0, K_IN, V_IN)
    fence()
    _merge((a_main(0, (0, 1, 2), XB[3], XB[4], state), rows_cost(3, 3)), (x_terms(XB[4], XB[5]), x_cost(4)))
    x_copy(5).wait()
    in_start(2, *W_IN)
    in_start(3, *W_IN)
    fence()
    state = {"todo": [], "n": 0, "zs": [None, None]}
    a_last(0)
    _merge((a_main(1, (0, 1, 2), 0, XB[5] - HS, state), rows_cost(4, 3)), (x_terms(XB[5], XB[6]), x_cost(5)))
    for c in small:
        c.wait()
    kf_buf[0:8, :] = jnp.zeros((8, CG), F32)
    shk = shk_ref[...].astype(F32)
    dd = dd_ref[0:NG, :].astype(F32)
    for g in range(NG):
        for t in range(KS):
            tap_buf[g, t] = jnp.broadcast_to(shk[t:t + 1, g * CG:(g + 1) * CG], (8, CG))
        tap_buf[g, KS] = jnp.broadcast_to(dd[g:g + 1, :], (8, CG))
    in_wait(0, K_IN, V_IN)
    in_wait(2, *W_IN)
    in_wait(3, *W_IN)
    in_start(0, H_IN)
    in_start(1, K_IN, V_IN)
    in_start(2, K_IN, V_IN)
    fence()
    _merge((a_main(1, (0, 1, 2), XB[5] - HS, HS, state), rows_cost(5, 3)), (b_pre(0), PRE_COST),
           (w_terms(1, range(3), all_kb), 3 * KH * KB_COST))
    in_wait(0, H_IN)
    in_wait(1, K_IN, V_IN)
    in_start(0, WO_IN)
    in_start(1, H_IN)
    fence()
    a_last(1)
    a_heads(0)
    a_heads(1)
    _merge((b_filter(0), NC), (b_signal(0), NC), (b_pre(1), PRE_COST))

    def after_first(stream, *fns):
        yield next(stream)
        for fn in fns:
            fn()
        yield from stream

    def late(stream, cost):
        yield cost
        yield from stream

    for s in range(2, NG):
        in_wait(s - 1, H_IN)
        in_wait(s, K_IN, V_IN)
        in_wait(s - 2, WO_IN)
        if s >= 3:
            in_wait(s - 3, Q_IN)
        if s % 2 == 1 and s + 1 < NG:
            in_wait(s + 1, *W_IN)
            in_wait(s + 2, *W_IN)
        in_start(s, H_IN)
        in_start(s - 1, WO_IN)
        in_start(s - 2, Q_IN)
        if s + 1 < NG:
            in_start(s + 1, K_IN, V_IN)
        else:
            in_start(s, WO_IN)
        if s % 2 == 0 and s + 2 < NG:
            in_start(s + 2, *W_IN)
            in_start(s + 3, *W_IN)
        fence()
        fns = [] if s == 2 else [lambda s=s: a_last(s - 1)]
        if s % 2 == 0 and s > 2:
            fns += [lambda s=s: a_heads(s - 2), lambda s=s: a_heads(s - 1)]
        streams = [(a_main(s), MAIN_COST), (b_mac(s - 2), MAC_RATE * MAC_COST), (b_pre(s), PRE_COST),
                   (after_first(b_filter(s - 1), *fns), NC), (b_signal(s - 1), NC),
                   (late(a_norm(s - 2), NORM_COST / 2), 3 * NORM_COST / 2), (late(a_mix(s - 2), NG / 2), 3 * NG / 2)]
        if s >= 3:
            streams.append((b_post(s - 3), NC))
        if s % 2 == 1 and s + 1 < NG:
            streams.append((w_terms(s // 2 + 1, range(3), all_kb), 3 * KH * KB_COST))
        _merge(*streams)
        if s >= 3:
            ob_copy(s - 3).start()

    g5, g6, g7 = NG - 3, NG - 2, NG - 1
    in_start(g6, Q_IN)
    in_start(g7, Q_IN)
    in_wait(g5, Q_IN)
    in_wait(g6, WO_IN)
    in_wait(g7, WO_IN, H_IN)
    fence()
    SEC_COST = RO // (2 * RA) * KH * 7
    TERMS_COST = RO * KH / (2 * RP)
    mac = b_mac(g6)
    _merge((after_first(b_filter(g7), lambda: a_last(g7), lambda: a_heads(g6), lambda: a_heads(g7)), NC),
           (b_signal(g7), NC), (b_post(g5), NC),
           (late(a_norm(g6, True), NORM_COST / 3), 4 * NORM_COST / 3), (late(a_norm(g7, True), NORM_COST / 3), 4 * NORM_COST / 3),
           (late(a_mix(g6), NG / 3), 4 * NG / 3), (late(a_mix(g7), NG / 3), 4 * NG / 3),
           (_take(mac, MAC_COST / 4), MAC_COST / 4))
    ob_copy(g5).start()
    fence()
    _merge((a_out_plain(), NG * NG), (m_terms(), KH * KH * KB_COST), (p_terms(0), (RO - 2 * RA) * KH / (2 * RP)))
    fence()
    _merge((a_out(0), SEC_COST - KH * 7), (mac, MAC_COST * 3 / 4), (p_terms(1), TERMS_COST))
    mac = b_mac(g7)
    fence()
    _merge((a_out(1), SEC_COST), (p_terms(2), TERMS_COST), (_take(mac, MAC_COST / 2), MAC_COST / 2))
    fence()
    _merge((a_out(2), SEC_COST), (p_terms(3), TERMS_COST), (mac, MAC_COST / 2))
    in_wait(g6, Q_IN)
    in_wait(g7, Q_IN)
    fence()
    out = a_out(3)
    for g in (g6, g7):
        _merge((b_post(g), NC), (_take(out, SEC_COST * 3 // 8), SEC_COST * 3 // 8))
        ob_copy(g).start()
    _merge((out, 1))
    for g in range(NG):
        ob_copy(g).wait()
    for i in range(S // (2 * RA) - 1):
        oa_copy(i).wait()
    for n in range(NG):
        last_copy(n).wait()


@jax.jit
def pallas_concat_heads__linear_attn_block__ssm_conv_h3__prompt_kernel(
    A_x: jax.Array,
    A_wqkv: jax.Array,
    A_wo: jax.Array,
    B_q: jax.Array,
    B_k: jax.Array,
    B_v: jax.Array,
    B_shift_k: jax.Array,
    B_ssm_k: jax.Array,
    B_ssm_D: jax.Array,
):
    hbm = pl.BlockSpec(memory_space=pl.ANY)
    out = pl.pallas_call(
        _kernel,
        out_shape=jax.ShapeDtypeStruct((S, 2 * D), BF16),
        in_specs=[hbm] * 11,
        out_specs=hbm,
        scratch_shapes=[
            pltpu.VMEM((S, D), BF16),
            pltpu.VMEM((2, 7, KH, HS // 2, CG), BF16),
            pltpu.VMEM((NG, 3, NG, CG, CG), BF16),
            pltpu.VMEM((2, 3, 7, KH, CG, CG), BF16),
            pltpu.VMEM((NG, CG, D), BF16),
            pltpu.VMEM((NG, S, CG), BF16),
            pltpu.VMEM((NG, S, CG), BF16),
            pltpu.VMEM((NG, S, CG), BF16),
            pltpu.VMEM((NG, CG, S), BF16),
            pltpu.VMEM((NG, KS + 1, 8, CG), F32),
            pltpu.VMEM((S + 8, CG), F32),
            pltpu.VMEM((4, S, CG), BF16),
            pltpu.VMEM((2, NC, 3 * T, CG), F32),
            pltpu.VMEM((2, NC, 3 * T, CG), F32),
            pltpu.VMEM((2, NC, 2 * T, CG), BF16),
            pltpu.VMEM((2, HS, CG), BF16),
            pltpu.VMEM((2, HS, CG), BF16),
            pltpu.VMEM((NG, 2, 8, CG), F32),
            pltpu.VMEM((NG, 2, CG, CG), F32),
            pltpu.VMEM((2, 8, CG), F32),
            pltpu.VMEM((2, 8 * CG // DH, CG), BF16),
            pltpu.VMEM((2, CG, CG), BF16),
            pltpu.VMEM((NG, 2, HS, CG), BF16),
            pltpu.VMEM((2, 7, KH, RO // 2, CG), BF16),
            pltpu.VMEM((NG, NG, CG, CG), BF16),
            pltpu.VMEM((KH, 7, KH, CG, CG), BF16),
            pltpu.VMEM((NG, S, CG), BF16),
            pltpu.VMEM((S, D), BF16),
            pltpu.VMEM(_FWD.shape, BF16),
            pltpu.VMEM(_INV.shape, BF16),
            pltpu.VMEM((KS, D), BF16),
            pltpu.VMEM((2 * NG, CG), BF16),
            pltpu.SemaphoreType.DMA((len(XB) - 1,)),
            pltpu.SemaphoreType.DMA((NG, 8)),
            pltpu.SemaphoreType.DMA((4,)),
            pltpu.SemaphoreType.DMA((NG,)),
            pltpu.SemaphoreType.DMA((S // (2 * RA),)),
            pltpu.SemaphoreType.REGULAR,
        ],
        compiler_params=pltpu.CompilerParams(vmem_limit_bytes=100 * 1024 * 1024, flags=FLAGS),
    )(A_x.reshape(S, D), A_wqkv.reshape(NG, CG, 3 * D), A_wo, B_q.reshape(S, D), B_k.reshape(S, D),
      B_v.reshape(S, D), B_ssm_k, B_shift_k.T, B_ssm_D.reshape(NG, CG), _FWD, _INV)
    return out.reshape(1, S, 2 * D)
```

```python
import jax
import jax.numpy as jnp
import numpy as np
import jax.experimental.pallas as pl
import jax.experimental.pallas.tpu as pltpu

S, D, H = 2048, 1024, 32
DH = D // H
CG = 128
NG = D // CG
T = 128
NC = S // T
KS = 4
HS = S // 2
KH = NG // 2
RA = 64
NB = 2
RP = 32
RO = 512
XB = (0, 256, 512, 768, 1024, 1536, 2048)
LAG_KV = 3072
MAC_RATE = 1.08
PRE_LAG = 64
F32, BF16, U32 = jnp.float32, jnp.bfloat16, jnp.uint32


def _dft_matrices():
    k = np.concatenate([np.arange(0, T, 2), np.arange(1, T, 2)])
    ang = np.pi * (2 * k[:, None] + 1) / (2 * T) * np.arange(T)[None, :]
    re = np.cos(ang).reshape(T // 8, 1, 8, T)
    im = -np.sin(ang).reshape(T // 8, 1, 8, T)
    fwd = np.concatenate([re, im], axis=1).reshape(2 * T, T)
    inv = fwd.T / T
    inv = np.stack([inv[:, :T], inv[:, T:]])
    return fwd.astype(BF16), inv.astype(BF16)


_FWD, _INV = _dft_matrices()


def _dot(a, b):
    return jnp.dot(a, b, preferred_element_type=F32)


def _dot_nt(a, b):
    return jax.lax.dot_general(a, b, (((1,), (1,)), ((), ())), preferred_element_type=F32)


def _dot_tn(a, b):
    return jax.lax.dot_general(a, b, (((0,), (0,)), ((), ())), preferred_element_type=F32)


def _phi(t):
    return jnp.where(t > 0, t + 1.0, jnp.exp(t)) + 1e-6


def _ld(ref, lead, r0, n):
    return pltpu.bitcast(ref.bitcast(U32)[lead + (pl.ds(r0 // 2, n // 2), slice(None))], BF16)


def _merge(*streams):
    done = [0.0] * len(streams)
    live = list(range(len(streams)))
    while live:
        i = min(live, key=lambda s: done[s] / streams[s][1])
        cost = next(streams[i][0], None)
        if cost is None:
            live.remove(i)
        else:
            done[i] += cost


def _take(stream, cost):
    while cost > 0:
        c = next(stream, None)
        if c is None:
            return
        cost -= c
        yield c


def _lhs_terms(a11, a12, a21, a22):
    return a11 + a22, a21 + a22, a11, a22, a11 + a12, a21 - a11, a12 - a22


def _rhs_terms(b11, b12, b21, b22):
    return b11 + b22, b11, b12 - b22, b21 - b11, b22, b11 + b12, b21 + b22


def _strassen(lhs, rhs, emit):
    def prod(i, acc=None):
        for kb in range(KH):
            part = _dot(lhs(i, kb), rhs(i, kb))
            acc = part if acc is None else acc + part
        return acc

    m1 = prod(0)
    yield 1
    m2 = prod(1)
    c22 = m1 - m2
    yield 1
    m4 = prod(3)
    emit(1, 0, m2 + m4)
    c11 = m1 + m4
    yield 1
    m3 = prod(2)
    c22 = c22 + m3
    yield 1
    emit(1, 1, prod(5, c22))
    yield 1
    m5 = prod(4)
    emit(0, 1, m3 + m5)
    c11 = c11 - m5
    yield 1
    emit(0, 0, prod(6, c11))
    yield 1


def _kernel(x_hbm, wqkv_hbm, wo_hbm, q_hbm, k_hbm, v_hbm, h_hbm, shk_hbm, dd_hbm, fwd_hbm, inv_hbm,
            out_hbm,
            x_buf, xs_buf, w_buf, ws_buf, wo_buf, q_buf, k_buf, v_buf, h_buf, tap_buf, kf_buf, kv_buf,
            xf_buf, hf_buf, yf_buf, pk_buf, pv_buf, z_buf, kvs_buf, zrow_buf, zs_buf, kvbd_buf, pq_buf, ps_buf,
            m_buf, ms_buf, ob_buf, oa_buf, fwd_ref, inv_ref, shk_ref, dd_ref,
            x_sem, in_sem, small_sem, ob_sem, oa_sem, fence_sem):

    H_IN, K_IN, V_IN, Q_IN, WO_IN, WQ_IN, WK_IN, WV_IN = range(8)
    W_IN = (WQ_IN, WK_IN, WV_IN)

    def in_copy(g, which):
        if which in W_IN:
            t = which - WQ_IN
            src, dst = wqkv_hbm.at[:, :, pl.ds((t * NG + g) * CG, CG)], w_buf.at[g, t]
        elif which in (H_IN, WO_IN):
            hbm, buf = (h_hbm, h_buf) if which == H_IN else (wo_hbm, wo_buf)
            src, dst = hbm.at[pl.ds(g * CG, CG)], buf.at[g]
        else:
            hbm, buf = {K_IN: (k_hbm, k_buf), V_IN: (v_hbm, v_buf), Q_IN: (q_hbm, q_buf)}[which]
            src, dst = hbm.at[:, pl.ds(g * CG, CG)], buf.at[g]
        return pltpu.make_async_copy(src, dst, in_sem.at[g, which])

    def in_start(g, *whiches):
        for which in whiches:
            in_copy(g, which).start()

    def in_wait(g, *whiches):
        for which in whiches:
            in_copy(g, which).wait()

    def x_copy(c):
        rows = pl.ds(XB[c], XB[c + 1] - XB[c])
        return pltpu.make_async_copy(x_hbm.at[rows], x_buf.at[rows], x_sem.at[c])

    def ob_copy(g):
        return pltpu.make_async_copy(ob_buf.at[g], out_hbm.at[:, pl.ds((NG + g) * CG, CG)], ob_sem.at[g])

    def oa_copy(i):
        rows = pl.ds(i * 2 * RA, 2 * RA)
        return pltpu.make_async_copy(oa_buf.at[rows], out_hbm.at[rows, pl.ds(0, D)], oa_sem.at[i])

    def last_copy(n):
        rows, cols = pl.ds(S - 2 * RA, 2 * RA), pl.ds(n * CG, CG)
        return pltpu.make_async_copy(oa_buf.at[rows, cols], out_hbm.at[rows, cols], oa_sem.at[S // (2 * RA) - 1])

    def fence():
        pl.semaphore_signal(fence_sem, 1)
        pl.semaphore_wait(fence_sem, 1)

    def x_terms(r_lo, r_hi):
        for r0 in range(r_lo, r_hi, 2 * RA):
            for kb in range(KH):
                for r in range(0, RA, RP):
                    blocks = [x_buf[pl.ds(r0 + a * RA + r, RP), pl.ds((b * KH + kb) * CG, CG)].astype(F32)
                              for a in range(2) for b in range(2)]
                    for i, term in enumerate(_lhs_terms(*blocks)):
                        xs_buf[r0 // HS, i, kb, pl.ds(r0 % HS // 2 + r, RP), :] = term.astype(BF16)
                    yield 1

    def w_terms(p, tiles, kbs):
        for t in tiles:
            for kb in kbs:
                for r in range(0, CG, RP):
                    blocks = [_ld(w_buf, (2 * p + b, t, a * KH + kb), r, RP).astype(F32)
                              for a in range(2) for b in range(2)]
                    for i, term in enumerate(_rhs_terms(*blocks)):
                        if i not in (1, 4):
                            ws_buf[p % 2, t, i, kb, pl.ds(r, RP), :] = term.astype(BF16)
                    yield 1

    def kv_block(s, j, b):
        kv = _dot_tn(_ld(pk_buf, (j,), b * CG, CG), _ld(pv_buf, (j,), b * CG, CG))
        kvs_buf[s, j] = kv if b == 0 else kvs_buf[s, j] + kv

    def a_main(s, tiles=(0, 1, 2), r_lo=0, r_hi=HS, state=None):
        p, half = s // 2, s % 2
        state = state or {"todo": [], "n": 0, "zs": [None, None]}
        todo, zs = state["todo"], state["zs"]
        for r0 in range(r_lo, r_hi, 2 * RA):
            for t in tiles:
                def lhs(i, kb):
                    return _ld(xs_buf, (half, i, kb), r0 // 2, RA)

                def rhs(i, kb):
                    if i == 1:
                        return _ld(w_buf, (2 * p, t, kb), 0, CG)
                    if i == 4:
                        return _ld(w_buf, (2 * p + 1, t, KH + kb), 0, CG)
                    return _ld(ws_buf, (p % 2, t, i, kb), 0, CG)

                def emit(a, j, val):
                    rows = pl.ds(r0 + a * RA, RA)
                    if t == 0:
                        pq_buf[2 * p + j, half, rows, :] = _phi(val).astype(BF16)
                    elif t == 1:
                        pk = _phi(val)
                        z = jnp.sum(pk.reshape(RA // 8, 8, CG), axis=0)
                        zs[j] = z if zs[j] is None else zs[j] + z
                        pk_buf[j, rows, :] = pk.astype(BF16)
                    else:
                        pv_buf[j, rows, :] = val.astype(BF16)

                for _ in _strassen(lhs, rhs, emit):
                    state["n"] += KH * RA
                    yield KH * RA
                    if todo and todo[0][0] <= state["n"]:
                        kv_block(s, *todo.pop(0)[1:])
                        yield CG
            if 2 in tiles and (r0 + 2 * RA) % CG == 0 and r0 + 2 * RA < HS:
                todo += [(state["n"] + LAG_KV, j, (r0 + 2 * RA) // CG - 1) for j in range(2)]
        if r_hi == HS:
            for _, j, b in todo:
                kv_block(s, j, b)
            for j in range(2):
                z_buf[s, j] = zs[j]

    def a_last(s):
        for j in range(2):
            kv_block(s, j, HS // CG - 1)

    def a_heads(g):
        s0, j, slot = g // 2 * 2, g % 2, g % 2
        col_head = jax.lax.broadcasted_iota(jnp.int32, (CG, CG), 1) // DH
        row_head = jax.lax.broadcasted_iota(jnp.int32, (CG, CG), 0) // DH
        kvbd_buf[slot] = jnp.where(row_head == col_head, kvs_buf[s0, j] + kvs_buf[s0 + 1, j], 0.0).astype(BF16)
        z = jnp.sum(z_buf[s0, j] + z_buf[s0 + 1, j], axis=0, keepdims=True)
        zrow_buf[slot] = jnp.broadcast_to(z, (8, CG))
        sel = (jax.lax.broadcasted_iota(jnp.int32, (8 * CG // DH, CG), 0) // 8
               == jax.lax.broadcasted_iota(jnp.int32, (8 * CG // DH, CG), 1) // DH)
        zs_buf[slot] = jnp.where(sel, z, 0.0).astype(BF16)

    def a_norm(g, on_mxu=False):
        z = jnp.concatenate([zrow_buf[g % 2]] * (CG // 8), axis=0)
        for half in range(2):
            for r0 in range(0, HS, CG):
                pq = _ld(pq_buf, (g, half), r0, CG)
                if on_mxu:
                    den = _dot_nt(_ld(zs_buf, (g % 2,), 0, 8 * CG // DH), pq)
                    dens = [den[h:h + 8] for h in range(0, 8 * CG // DH, 8)]
                else:
                    terms = (pq.astype(F32) * z).T
                    dens = []
                    for h in range(0, CG, DH):
                        den = sum(terms[c:c + 8] for c in range(h + 8, h + DH, 8)) + terms[h:h + 8]
                        dens.append(jnp.broadcast_to(jnp.sum(den, axis=0, keepdims=True), (8, CG)))
                rcp = []
                for den in dens:
                    den = den + 1e-6
                    r = pl.reciprocal(den, approx=True)
                    rcp += [r * (2.0 - den * r)] * (DH // 8)
                rcp = jnp.concatenate(rcp, axis=0).T
                pq_buf[g, half, pl.ds(r0, CG), :] = (pq.astype(F32) * rcp).astype(BF16)
                yield 1

    def a_mix(g):
        for n in range(NG):
            m_buf[n, g] = _dot(_ld(kvbd_buf, (g % 2,), 0, CG), wo_buf[g, :, pl.ds(n * CG, CG)]).astype(BF16)
            yield 1

    def m_terms():
        for t in range(KH):
            for kb in range(KH):
                for r in range(0, CG, RP):
                    blocks = [_ld(m_buf, (b * KH + t, a * KH + kb), r, RP).astype(F32)
                              for a in range(2) for b in range(2)]
                    for i, term in enumerate(_rhs_terms(*blocks)):
                        if i not in (1, 4):
                            ms_buf[t, i, kb, pl.ds(r, RP), :] = term.astype(BF16)
                    yield 1

    def p_terms(sec):
        for r0 in range(max(sec * RO, 2 * RA), (sec + 1) * RO, 2 * RA):
            for kb in range(KH):
                for r in range(0, RA, RP):
                    blocks = [_ld(pq_buf, (b * KH + kb, r0 // HS), r0 % HS + a * RA + r, RP).astype(F32)
                              for a in range(2) for b in range(2)]
                    for i, term in enumerate(_lhs_terms(*blocks)):
                        if i not in (2, 3):
                            ps_buf[sec % 2, i, kb, pl.ds(r0 % RO // 2 + r, RP), :] = term.astype(BF16)
                    yield 1

    def a_out_plain():
        for n in range(NG):
            acc = None
            for g in range(NG):
                part = _dot(_ld(pq_buf, (g, 0), 0, 2 * RA), _ld(m_buf, (n, g), 0, CG))
                acc = part if acc is None else acc + part
                yield 1
            oa_buf[pl.ds(0, 2 * RA), pl.ds(n * CG, CG)] = acc.astype(BF16)
        oa_copy(0).start()

    def a_out(sec):
        for r0 in range(max(sec * RO, 2 * RA), (sec + 1) * RO, 2 * RA):
            for t in range(KH):
                def lhs(i, kb):
                    if i == 2:
                        return _ld(pq_buf, (kb, r0 // HS), r0 % HS, RA)
                    if i == 3:
                        return _ld(pq_buf, (KH + kb, r0 // HS), r0 % HS + RA, RA)
                    return _ld(ps_buf, (sec % 2, i, kb), r0 % RO // 2, RA)

                def rhs(i, kb):
                    if i == 1:
                        return _ld(m_buf, (t, kb), 0, CG)
                    if i == 4:
                        return _ld(m_buf, (KH + t, KH + kb), 0, CG)
                    return _ld(ms_buf, (t, i, kb), 0, CG)

                def emit(a, b, val):
                    oa_buf[pl.ds(r0 + a * RA, RA), pl.ds((b * KH + t) * CG, CG)] = val.astype(BF16)

                yield from _strassen(lhs, rhs, emit)
                if r0 + 2 * RA == S:
                    for b in range(2):
                        last_copy(b * KH + t).start()
            if r0 + 2 * RA < S:
                oa_copy(r0 // (2 * RA)).start()

    def b_pre(g):
        taps = [jnp.concatenate([tap_buf[g, t]] * (RP // 8), axis=0) for t in range(KS)]
        for r0 in range(-PRE_LAG, S, RP):
            if r0 + PRE_LAG < S:
                kf_buf[pl.ds(8 + r0 + PRE_LAG, RP), :] = _ld(k_buf, (g,), r0 + PRE_LAG, RP).astype(F32)
            if r0 < 0:
                continue
            acc = kf_buf[pl.ds(8 + r0, RP), :] * taps[0]
            for t in range(1, KS):
                acc = acc + kf_buf[pl.ds(8 + r0 - t, RP), :] * taps[t]
            kv_buf[g % 4, pl.ds(r0, RP), :] = (acc * _ld(v_buf, (g,), r0, RP).astype(F32)).astype(BF16)
            yield 1

    def spectrum(buf, j, res, factors):
        parts = []
        for r in range(0, 2 * T, 16):
            parts += factors(res[r:r + 8], res[r + 8:r + 16])
        buf[j] = jnp.concatenate(parts, axis=0)

    def b_filter(g):
        for j in range(NC):
            res = _dot_nt(_ld(fwd_ref, (), 0, 2 * T), h_buf[g, :, pl.ds(j * T, T)])
            spectrum(hf_buf.at[g % 2], j, res, lambda re, im: [re, im - re, re + im])
            yield 1

    def b_signal(g):
        for j in range(NC):
            res = _dot(_ld(fwd_ref, (), 0, 2 * T), _ld(kv_buf, (g % 4,), j * T, T))
            spectrum(xf_buf.at[g % 2], j, res, lambda re, im: [re + im, re, im])
            yield 1

    def b_mac(g):
        u = g % 2
        for r in range(T // 8):
            rows = [pl.ds(24 * r + o, 8) for o in (0, 8, 16)]
            even = r < T // 16
            prev = None
            for i0 in range(0, NC, NB):
                acc = [None] * NB
                hs = {}
                for j in range(i0 + NB):
                    xs = [xf_buf[u, j, rr, :] for rr in rows]
                    n = 0
                    for a in range(NB):
                        m = i0 + a - j
                        if m < 0:
                            continue
                        if m not in hs:
                            hs[m] = [hf_buf[u, m, rr, :] for rr in rows]
                        ks = [h * x for h, x in zip(hs[m], xs)]
                        acc[a] = ks if acc[a] is None else [c + k for c, k in zip(acc[a], ks)]
                        n += 1
                    yield n
                for a in range(NB):
                    cur = yr, yi = acc[a][0] - acc[a][2], acc[a][0] + acc[a][1]
                    if prev is not None:
                        yr, yi = (yr - prev[1], yi + prev[0]) if even else (yr + prev[1], yi - prev[0])
                    prev = cur
                    yf_buf[u, i0 + a, pl.ds(16 * r, 16), :] = jnp.concatenate([yr, yi], axis=0).astype(BF16)

    def b_post(g):
        dvec = jnp.concatenate([tap_buf[g, KS]] * (T // 8), axis=0)
        for i in range(NC):
            inv = jnp.concatenate([_ld(inv_ref, (0,), 0, T), _ld(inv_ref, (1,), 0, T)], axis=1)
            y = _dot(inv, _ld(yf_buf, (g % 2, i), 0, 2 * T)) + _ld(kv_buf, (g % 4,), i * T, T).astype(F32) * dvec
            ob_buf[g, pl.ds(i * T, T), :] = (_ld(q_buf, (g,), i * T, T).astype(F32) * y).astype(BF16)
            yield 1

    TILE_COST = 7 * KH * HS // 2
    MAIN_COST = 3 * TILE_COST + 2 * HS
    MAC_COST = (T // 8) * NC * (NC + 1) // 2
    PRE_COST = S // RP
    NORM_COST = S // CG
    KB_COST = CG // RP
    all_kb = range(KH)

    def rows_cost(c, n_tiles):
        return n_tiles * 7 * KH * (XB[c + 1] - XB[c]) // 2

    def x_cost(c):
        return (XB[c + 1] - XB[c]) * KH / (2 * RP)

    state = {"todo": [], "n": 0, "zs": [None, None]}
    small = [pltpu.make_async_copy(src, dst, small_sem.at[i]) for i, (src, dst) in enumerate(
        ((shk_hbm, shk_ref), (dd_hbm, dd_ref.at[pl.ds(0, NG)]), (fwd_hbm, fwd_ref), (inv_hbm, inv_ref)))]

    def pair_start(which):
        in_start(0, which)
        in_start(1, which)

    def pair_wait(which):
        in_wait(0, which)
        in_wait(1, which)

    x_copy(0).start()
    pair_start(WQ_IN)
    x_copy(0).wait()
    x_copy(1).start()
    _merge((x_terms(XB[0], XB[1]), 1))
    pair_wait(WQ_IN)
    pair_start(WK_IN)
    _merge((w_terms(0, (0,), all_kb), 1))
    fence()
    _merge((a_main(0, (0,), XB[0], XB[1], state), 1))
    x_copy(1).wait()
    pair_start(WV_IN)
    _merge((x_terms(XB[1], XB[2]), 1))
    fence()
    _merge((a_main(0, (0,), XB[1], XB[2], state), 1))
    pair_wait(WK_IN)
    x_copy(2).start()
    _merge((w_terms(0, (1,), all_kb), 1))
    fence()
    _merge((a_main(0, (1,), XB[0], XB[1], state), 1))
    pair_wait(WV_IN)
    x_copy(3).start()
    fence()
    _merge((a_main(0, (1,), XB[1], XB[2], state), rows_cost(1, 1)), (w_terms(0, (2,), all_kb), KH * KB_COST))
    x_copy(2).wait()
    x_copy(4).start()
    fence()
    _merge((a_main(0, (2,), XB[0], XB[2], state), 2 * rows_cost(0, 1)), (x_terms(XB[2], XB[3]), x_cost(2)))
    x_copy(3).wait()
    x_copy(5).start()
    for c in small:
        c.start()
    fence()
    _merge((a_main(0, (0, 1, 2), XB[2], XB[3], state), rows_cost(2, 3)), (x_terms(XB[3], XB[4]), x_cost(3)))
    x_copy(4).wait()
    in_start(0, K_IN, V_IN)
    fence()
    _merge((a_main(0, (0, 1, 2), XB[3], XB[4], state), rows_cost(3, 3)), (x_terms(XB[4], XB[5]), x_cost(4)))
    x_copy(5).wait()
    in_start(2, *W_IN)
    in_start(3, *W_IN)
    fence()
    state = {"todo": [], "n": 0, "zs": [None, None]}
    a_last(0)
    _merge((a_main(1, (0, 1, 2), 0, XB[5] - HS, state), rows_cost(4, 3)), (x_terms(XB[5], XB[6]), x_cost(5)))
    for c in small:
        c.wait()
    kf_buf[0:8, :] = jnp.zeros((8, CG), F32)
    shk = shk_ref[...].astype(F32)
    dd = dd_ref[0:NG, :].astype(F32)
    for g in range(NG):
        for t in range(KS):
            tap_buf[g, t] = jnp.broadcast_to(shk[t:t + 1, g * CG:(g + 1) * CG], (8, CG))
        tap_buf[g, KS] = jnp.broadcast_to(dd[g:g + 1, :], (8, CG))
    in_wait(0, K_IN, V_IN)
    in_wait(2, *W_IN)
    in_wait(3, *W_IN)
    in_start(0, H_IN)
    in_start(1, K_IN, V_IN)
    in_start(2, K_IN, V_IN)
    fence()
    _merge((a_main(1, (0, 1, 2), XB[5] - HS, HS, state), rows_cost(5, 3)), (b_pre(0), PRE_COST),
           (w_terms(1, range(3), all_kb), 3 * KH * KB_COST))
    in_wait(0, H_IN)
    in_wait(1, K_IN, V_IN)
    in_start(0, WO_IN)
    in_start(1, H_IN)
    fence()
    a_last(1)
    a_heads(0)
    a_heads(1)
    _merge((b_filter(0), NC), (b_signal(0), NC), (b_pre(1), PRE_COST))

    def after_first(stream, *fns):
        yield next(stream)
        for fn in fns:
            fn()
        yield from stream

    def late(stream, cost):
        yield cost
        yield from stream

    for s in range(2, NG):
        in_wait(s - 1, H_IN)
        in_wait(s, K_IN, V_IN)
        in_wait(s - 2, WO_IN)
        if s >= 3:
            in_wait(s - 3, Q_IN)
        if s % 2 == 1 and s + 1 < NG:
            in_wait(s + 1, *W_IN)
            in_wait(s + 2, *W_IN)
        in_start(s, H_IN)
        in_start(s - 1, WO_IN)
        in_start(s - 2, Q_IN)
        if s + 1 < NG:
            in_start(s + 1, K_IN, V_IN)
        else:
            in_start(s, WO_IN)
        if s % 2 == 0 and s + 2 < NG:
            in_start(s + 2, *W_IN)
            in_start(s + 3, *W_IN)
        fence()
        fns = [] if s == 2 else [lambda s=s: a_last(s - 1)]
        if s % 2 == 0 and s > 2:
            fns += [lambda s=s: a_heads(s - 2), lambda s=s: a_heads(s - 1)]
        streams = [(a_main(s), MAIN_COST), (b_mac(s - 2), MAC_RATE * MAC_COST), (b_pre(s), PRE_COST),
                   (after_first(b_filter(s - 1), *fns), NC), (b_signal(s - 1), NC),
                   (late(a_norm(s - 2), NORM_COST / 2), 3 * NORM_COST / 2), (late(a_mix(s - 2), NG / 2), 3 * NG / 2)]
        if s >= 3:
            streams.append((b_post(s - 3), NC))
        if s % 2 == 1 and s + 1 < NG:
            streams.append((w_terms(s // 2 + 1, range(3), all_kb), 3 * KH * KB_COST))
        _merge(*streams)
        if s >= 3:
            ob_copy(s - 3).start()

    g5, g6, g7 = NG - 3, NG - 2, NG - 1
    in_start(g6, Q_IN)
    in_start(g7, Q_IN)
    in_wait(g5, Q_IN)
    in_wait(g6, WO_IN)
    in_wait(g7, WO_IN, H_IN)
    fence()
    SEC_COST = RO // (2 * RA) * KH * 7
    TERMS_COST = RO * KH / (2 * RP)
    mac = b_mac(g6)
    _merge((after_first(b_filter(g7), lambda: a_last(g7), lambda: a_heads(g6), lambda: a_heads(g7)), NC),
           (b_signal(g7), NC), (b_post(g5), NC),
           (late(a_norm(g6, True), NORM_COST / 3), 4 * NORM_COST / 3), (late(a_norm(g7, True), NORM_COST / 3), 4 * NORM_COST / 3),
           (late(a_mix(g6), NG / 3), 4 * NG / 3), (late(a_mix(g7), NG / 3), 4 * NG / 3),
           (_take(mac, MAC_COST / 4), MAC_COST / 4))
    ob_copy(g5).start()
    fence()
    _merge((a_out_plain(), NG * NG), (m_terms(), KH * KH * KB_COST), (p_terms(0), (RO - 2 * RA) * KH / (2 * RP)))
    fence()
    _merge((a_out(0), SEC_COST - KH * 7), (mac, MAC_COST * 3 / 4), (p_terms(1), TERMS_COST))
    mac = b_mac(g7)
    fence()
    _merge((a_out(1), SEC_COST), (p_terms(2), TERMS_COST), (_take(mac, MAC_COST / 2), MAC_COST / 2))
    fence()
    _merge((a_out(2), SEC_COST), (p_terms(3), TERMS_COST), (mac, MAC_COST / 2))
    in_wait(g6, Q_IN)
    in_wait(g7, Q_IN)
    fence()
    out = a_out(3)
    for g in (g6, g7):
        _merge((b_post(g), NC), (_take(out, SEC_COST * 3 // 8), SEC_COST * 3 // 8))
        ob_copy(g).start()
    _merge((out, 1))
    for g in range(NG):
        ob_copy(g).wait()
    for i in range(S // (2 * RA) - 1):
        oa_copy(i).wait()
    for n in range(NG):
        last_copy(n).wait()


@jax.jit
def pallas_concat_heads__linear_attn_block__ssm_conv_h3__prompt_kernel(
    A_x: jax.Array,
    A_wqkv: jax.Array,
    A_wo: jax.Array,
    B_q: jax.Array,
    B_k: jax.Array,
    B_v: jax.Array,
    B_shift_k: jax.Array,
    B_ssm_k: jax.Array,
    B_ssm_D: jax.Array,
):
    hbm = pl.BlockSpec(memory_space=pl.ANY)
    out = pl.pallas_call(
        _kernel,
        out_shape=jax.ShapeDtypeStruct((S, 2 * D), BF16),
        in_specs=[hbm] * 11,
        out_specs=hbm,
        scratch_shapes=[
            pltpu.VMEM((S, D), BF16),
            pltpu.VMEM((2, 7, KH, HS // 2, CG), BF16),
            pltpu.VMEM((NG, 3, NG, CG, CG), BF16),
            pltpu.VMEM((2, 3, 7, KH, CG, CG), BF16),
            pltpu.VMEM((NG, CG, D), BF16),
            pltpu.VMEM((NG, S, CG), BF16),
            pltpu.VMEM((NG, S, CG), BF16),
            pltpu.VMEM((NG, S, CG), BF16),
            pltpu.VMEM((NG, CG, S), BF16),
            pltpu.VMEM((NG, KS + 1, 8, CG), F32),
            pltpu.VMEM((S + 8, CG), F32),
            pltpu.VMEM((4, S, CG), BF16),
            pltpu.VMEM((2, NC, 3 * T, CG), F32),
            pltpu.VMEM((2, NC, 3 * T, CG), F32),
            pltpu.VMEM((2, NC, 2 * T, CG), BF16),
            pltpu.VMEM((2, HS, CG), BF16),
            pltpu.VMEM((2, HS, CG), BF16),
            pltpu.VMEM((NG, 2, 8, CG), F32),
            pltpu.VMEM((NG, 2, CG, CG), F32),
            pltpu.VMEM((2, 8, CG), F32),
            pltpu.VMEM((2, 8 * CG // DH, CG), BF16),
            pltpu.VMEM((2, CG, CG), BF16),
            pltpu.VMEM((NG, 2, HS, CG), BF16),
            pltpu.VMEM((2, 7, KH, RO // 2, CG), BF16),
            pltpu.VMEM((NG, NG, CG, CG), BF16),
            pltpu.VMEM((KH, 7, KH, CG, CG), BF16),
            pltpu.VMEM((NG, S, CG), BF16),
            pltpu.VMEM((S, D), BF16),
            pltpu.VMEM(_FWD.shape, BF16),
            pltpu.VMEM(_INV.shape, BF16),
            pltpu.VMEM((KS, D), BF16),
            pltpu.VMEM((2 * NG, CG), BF16),
            pltpu.SemaphoreType.DMA((len(XB) - 1,)),
            pltpu.SemaphoreType.DMA((NG, 8)),
            pltpu.SemaphoreType.DMA((4,)),
            pltpu.SemaphoreType.DMA((NG,)),
            pltpu.SemaphoreType.DMA((S // (2 * RA),)),
            pltpu.SemaphoreType.REGULAR,
        ],
        compiler_params=pltpu.CompilerParams(vmem_limit_bytes=100 * 1024 * 1024),
    )(A_x.reshape(S, D), A_wqkv.reshape(NG, CG, 3 * D), A_wo, B_q.reshape(S, D), B_k.reshape(S, D),
      B_v.reshape(S, D), B_ssm_k, B_shift_k.T, B_ssm_D.reshape(NG, CG), _FWD, _INV)
    return out.reshape(1, S, 2 * D)
```
